```python
import jax
import jax.numpy as jnp

def _softmax(x, axis=-1):
    return jax.nn.softmax(x, axis=axis)
def _gelu(x):
    return jax.nn.gelu(x, approximate=True)
def _silu(x):
    return jax.nn.silu(x)
def _sigmoid(x):
    return jax.nn.sigmoid(x)
def _layernorm(x, axis=-1, eps=1e-5):
    m = jnp.mean(x, axis=axis, keepdims=True)
    v = jnp.var(x, axis=axis, keepdims=True)
    return (x - m) / jnp.sqrt(v + eps)
def _scatter_add(tgt, idx, src, axis=0):
    return tgt.at[idx].add(src)
def _segment_sum(src, seg, n):
    return jax.ops.segment_sum(src, seg, n)
class _Rng:
    def __init__(self, key):
        self._k = key
    def _next(self):
        self._k, sub = jax.random.split(self._k)
        return sub
    def normal(self, shape):
        return jax.random.normal(self._next(), shape, dtype=jnp.bfloat16)
    def randint(self, lo, hi, shape):
        return jax.random.randint(self._next(), shape, lo, hi, dtype=jnp.int32)
    def uniform(self, shape, lo=0.0, hi=1.0):
        return jax.random.uniform(self._next(), shape, jnp.bfloat16, lo, hi)
    def permutation(self, n):
        return jax.random.permutation(self._next(), n)


kernel_name = 'recurrent_scan__mha_block_cached__moe_arch_mod__prompt'

def setup_inputs():
    _rng = _Rng(jax.random.key(int.from_bytes(__import__("os").urandom(4), "little")))
    _w = (lambda a: (lambda t: t.astype(jnp.bfloat16) if jnp.issubdtype(t.dtype, jnp.floating) else t)(jnp.asarray(a)))
    def _A_setup():
        B, Sq, D = 1, 2048, 640
        H, Sk, Dh = 32, 2048, 128
        return {
            "x": _w((lambda *s: _rng.normal(s) * 0.05)(B, Sq, D)),
            "k_cache": _w((lambda *s: _rng.normal(s) * 0.05)(B, H, Sk, Dh)),
            "v_cache": _w((lambda *s: _rng.normal(s) * 0.05)(B, H, Sk, Dh)),
            "wq": _w((lambda *s: _rng.normal(s) * 0.05)(D, H * Dh) * (D ** -0.5)),
            "wo": _w((lambda *s: _rng.normal(s) * 0.05)(H * Dh, D) * ((H * Dh) ** -0.5)),
        }
    _A_in = _A_setup()

    def _B_setup():
        B, S, D, F, C = 1, 2048, 640, 1728, 8
        return {
            "x": _w((lambda *s: _rng.normal(s) * 0.05)(B, S, D)),
            "w_r": _w((lambda *s: _rng.normal(s) * 0.05)(D)),
            "w_gate": _w((lambda *s: _rng.normal(s) * 0.05)(D, F)),
            "w_up": _w((lambda *s: _rng.normal(s) * 0.05)(D, F)),
            "w_down": _w((lambda *s: _rng.normal(s) * 0.05)(F, D)),
        }
    _B_in = _B_setup()

    return {
        "A_x": _A_in["x"],
        "A_k_cache": _A_in["k_cache"],
        "A_v_cache": _A_in["v_cache"],
        "A_wq": _A_in["wq"],
        "A_wo": _A_in["wo"],
        "B_x": _B_in["x"],
        "B_w_r": _B_in["w_r"],
        "B_w_gate": _B_in["w_gate"],
        "B_w_up": _B_in["w_up"],
        "B_w_down": _B_in["w_down"],
    }

def reference(A_x, A_k_cache, A_v_cache, A_wq, A_wo, B_x, B_w_r, B_w_gate, B_w_up, B_w_down):
    def _A_ref(x, k_cache, v_cache, wq, wo):
        B, Sq, D = x.shape
        H, Dh = 32, 128
        q = (lambda x, *d: x.transpose(*d))((x @ wq).reshape(B, Sq, H, Dh), 0, 2, 1, 3)
        scores = jnp.einsum("bhqd,bhkd->bhqk", q, k_cache) * (Dh ** -0.5)
        p = _softmax(scores, axis=-1)
        o = jnp.einsum("bhqk,bhkd->bhqd", p, v_cache)
        return (lambda x, *d: x.transpose(*d))(o, 0, 2, 1, 3).reshape(B, Sq, H * Dh) @ wo

    def _B_ref(x, w_r, w_gate, w_up, w_down):
        B, S, D = x.shape
        C = 8
        r = x @ w_r
        idx = jnp.argsort(-r, axis=-1)[:, :C]
        idx_e = jnp.repeat(idx.reshape(B, C, 1), D, axis=2)
        x_sel = jnp.take_along_axis(x, idx_e, axis=1)
        g = _silu(x_sel @ w_gate)
        u = x_sel @ w_up
        y = (g * u) @ w_down
        r_sel = _sigmoid(jnp.take_along_axis(r, idx, axis=1))
        y = y * r_sel.reshape(B, C, 1)
        b_off = (jnp.arange(B) * S).reshape(B, 1)
        flat_idx = (idx + b_off).reshape(B * C)
        zero = (x * 0.0).reshape(B * S, D)
        upd = _scatter_add(zero, flat_idx, y.reshape(B * C, D), axis=0)
        return x + upd.reshape(B, S, D)

    x = A_x
    xn = _layernorm(x, axis=-1)
    s = _A_ref(xn, A_k_cache, A_v_cache, A_wq, A_wo)
    g = _silu(_B_ref(xn, B_w_r, B_w_gate, B_w_up, B_w_down))
    return x + s * g
```

```python
import functools
import math

import jax
import jax.numpy as jnp
import jax.experimental.pallas as pl
import jax.experimental.pallas.tpu as pltpu

_F32 = jnp.float32
_BF16 = jnp.bfloat16

_TOPC = 8
_EPS = 1e-5
_TQ = 256


def _bf(x):
    return x.astype(_BF16).astype(_F32)


def _sigmoid(x):
    return 1.0 / (1.0 + jnp.exp(-x))


def _kernel(x_ref, k_ref, v_ref, wq_ref, wo_ref, wr_ref, wg_hbm, wu_hbm, wd_hbm,
            out_ref,
            xn_ref, z_ref, acc_ref, q_ref, wg_ref, wu_ref, wd_ref, sel_ref, rsel_ref, sems,
            *, S, D, Dh, H, tq):
    h = pl.program_id(0)
    ln_rows = 256

    def ffn_copies():
        return (pltpu.make_async_copy(wg_hbm, wg_ref, sems.at[0]),
                pltpu.make_async_copy(wu_hbm, wu_ref, sems.at[1]),
                pltpu.make_async_copy(wd_hbm, wd_ref, sems.at[2]))

    @pl.when(h == 0)
    def _prologue():
        for c in ffn_copies():
            c.start()

        def ln_body(i, carry):
            rows = pl.ds(pl.multiple_of(i * ln_rows, ln_rows), ln_rows)
            x = x_ref[rows, :].astype(_F32)
            mean = jnp.sum(x, axis=-1, keepdims=True) * (1.0 / D)
            xc = x - mean
            var = jnp.sum(xc * xc, axis=-1, keepdims=True) * (1.0 / D)
            num = _bf(x - _bf(mean))
            den = _bf(jnp.sqrt(_bf(_bf(var) + _bf(jnp.float32(_EPS)))))
            xn = (num / den).astype(_BF16)
            xn_ref[rows, :] = xn
            z_ref[rows, :] = xn.astype(_F32)
            acc_ref[rows, :] = jnp.zeros((ln_rows, D), _F32)
            return carry

        jax.lax.fori_loop(0, S // ln_rows, ln_body, 0)

        wr8 = jnp.broadcast_to(wr_ref[...], (8, D))
        r = jax.lax.dot_general(wr8, xn_ref[...], (((1,), (1,)), ((), ())),
                                preferred_element_type=_F32)
        r = _bf(r[0:1, :])
        col = jax.lax.broadcasted_iota(jnp.int32, (1, S), 1)
        for c in range(_TOPC):
            m = jnp.max(r)
            idx = jnp.min(jnp.where(r == m, col, S))
            idx = jnp.minimum(idx, S - 1)
            sel_ref[c] = idx
            rsel_ref[c] = m
            r = jnp.where(col == idx, -jnp.inf, r)

    scale = (Dh ** -0.5) * math.log2(math.e)
    q = jnp.dot(xn_ref[...], wq_ref[...], preferred_element_type=_F32)
    q_ref[...] = (q * scale).astype(_BF16)

    def attn_body(i, carry):
        rows = pl.ds(pl.multiple_of(i * tq, tq), tq)
        s = jax.lax.dot_general(q_ref[rows, :], k_ref[...], (((1,), (1,)), ((), ())),
                                preferred_element_type=_F32)
        m = jnp.max(s, axis=-1, keepdims=True)
        p = jnp.exp2(s - m)
        l = jnp.sum(p, axis=-1, keepdims=True)
        o = jnp.dot(p.astype(_BF16), v_ref[...], preferred_element_type=_F32)
        o = (o * (1.0 / l)).astype(_BF16)
        acc_ref[rows, :] += jnp.dot(o, wo_ref[...], preferred_element_type=_F32)
        return carry

    jax.lax.fori_loop(0, S // tq, attn_body, 0)

    @pl.when(h == H - 1)
    def _epilogue():
        for c in ffn_copies():
            c.wait()
        rowid = jax.lax.broadcasted_iota(jnp.int32, (_TOPC, 1), 0)
        xs = jnp.zeros((_TOPC, D), _F32)
        rs = jnp.zeros((_TOPC, 1), _F32)
        for c in range(_TOPC):
            row = z_ref[pl.ds(sel_ref[c], 1), :]
            xs = jnp.where(rowid == c, row, xs)
            rs = jnp.where(rowid == c, rsel_ref[c], rs)
        xs = xs.astype(_BF16)
        g = _bf(jnp.dot(xs, wg_ref[...], preferred_element_type=_F32))
        g = _bf(g * _sigmoid(g))
        u = _bf(jnp.dot(xs, wu_ref[...], preferred_element_type=_F32))
        y = _bf(jnp.dot((g * u).astype(_BF16), wd_ref[...], preferred_element_type=_F32))
        y = _bf(y * _bf(_sigmoid(rs)))
        for c in range(_TOPC):
            sl = pl.ds(sel_ref[c], 1)
            z_ref[sl, :] = _bf(z_ref[sl, :] + y[c:c + 1, :])

        def fin_body(i, carry):
            rows = pl.ds(pl.multiple_of(i * ln_rows, ln_rows), ln_rows)
            z = z_ref[rows, :]
            gate = z * _sigmoid(z)
            out_ref[rows, :] = (x_ref[rows, :].astype(_F32) + acc_ref[rows, :] * gate).astype(_BF16)
            return carry

        jax.lax.fori_loop(0, S // ln_rows, fin_body, 0)


@jax.jit
def pallas_recurrent_scan__mha_block_cached__moe_arch_mod__prompt_kernel(
    A_x: jax.Array,
    A_k_cache: jax.Array,
    A_v_cache: jax.Array,
    A_wq: jax.Array,
    A_wo: jax.Array,
    B_x: jax.Array,
    B_w_r: jax.Array,
    B_w_gate: jax.Array,
    B_w_up: jax.Array,
    B_w_down: jax.Array,
):
    B, S, D = A_x.shape
    _, H, Sk, Dh = A_k_cache.shape
    F = B_w_gate.shape[1]
    assert B == 1
    x = A_x.reshape(S, D)
    k = A_k_cache.reshape(H, Sk, Dh)
    v = A_v_cache.reshape(H, Sk, Dh)
    wr = B_w_r.reshape(1, D)

    kernel = functools.partial(_kernel, S=S, D=D, Dh=Dh, H=H, tq=_TQ)
    out = pl.pallas_call(
        kernel,
        grid=(H,),
        in_specs=[
            pl.BlockSpec((S, D), lambda h: (0, 0)),
            pl.BlockSpec((None, Sk, Dh), lambda h: (h, 0, 0)),
            pl.BlockSpec((None, Sk, Dh), lambda h: (h, 0, 0)),
            pl.BlockSpec((D, Dh), lambda h: (0, h)),
            pl.BlockSpec((Dh, D), lambda h: (h, 0)),
            pl.BlockSpec((1, D), lambda h: (0, 0)),
            pl.BlockSpec(memory_space=pl.ANY),
            pl.BlockSpec(memory_space=pl.ANY),
            pl.BlockSpec(memory_space=pl.ANY),
        ],
        out_specs=pl.BlockSpec((S, D), lambda h: (0, 0)),
        out_shape=jax.ShapeDtypeStruct((S, D), _BF16),
        scratch_shapes=[
            pltpu.VMEM((S, D), _BF16),
            pltpu.VMEM((S, D), _F32),
            pltpu.VMEM((S, D), _F32),
            pltpu.VMEM((S, Dh), _BF16),
            pltpu.VMEM((D, F), _BF16),
            pltpu.VMEM((D, F), _BF16),
            pltpu.VMEM((F, D), _BF16),
            pltpu.SMEM((_TOPC,), jnp.int32),
            pltpu.SMEM((_TOPC,), _F32),
            pltpu.SemaphoreType.DMA((3,)),
        ],
        compiler_params=pltpu.CompilerParams(
            dimension_semantics=("arbitrary",),
            vmem_limit_bytes=100 * 1024 * 1024,
        ),
    )(x, k, v, A_wq, A_wo, wr, B_w_gate, B_w_up, B_w_down)
    return out.reshape(B, S, D)
```

```python
import functools
import math

import jax
import jax.numpy as jnp
import jax.experimental.pallas as pl
import jax.experimental.pallas.tpu as pltpu

_F32 = jnp.float32
_BF16 = jnp.bfloat16
_I32 = jnp.int32
_NT = (((1,), (1,)), ((), ()))

_TOPC = 8
_EPS = 1e-5
_TQ = 256
_CW = 512
_P = 4
_NS = 3
_INT_MIN = -2 ** 31


def _bf(x):
    return x.astype(_BF16).astype(_F32)


def _silu(x):
    h = 0.5 * x
    return h + h * jnp.tanh(h)


def _sigmoid(x):
    return 0.5 + 0.5 * jnp.tanh(0.5 * x)


def _after(gate, val):
    return jnp.where(gate > jnp.inf, 0.0, val)


def _kernel(x_hbm, k_hbm, v_hbm, wq_hbm, wo_hbm, wr_ref, wg_hbm, wu_hbm, wd_hbm,
            out_hbm,
            x_ref, xn_ref, z_ref, acc_ref, ob_ref, s_ref, mc_ref, oc_ref, lc_ref,
            kb, vb, wqb, wob, wg_ref, wu_ref, wd_ref, sel_ref, zs,
            hsems, xsems, osems, fsems,
            *, S, D, Dh, H):
    tq, cw, p, NS = _TQ, _CW, _P, _NS
    n = S // tq
    R = S // cw
    tb = tq // 4
    D4 = (D // 512) * 512
    scale = (Dh ** -0.5) * math.log2(math.e)

    def hcol(h):
        return pl.ds(pl.multiple_of(h * Dh, Dh), Dh)

    def cp_k(h, slot):
        return pltpu.make_async_copy(k_hbm.at[h], kb.at[slot], hsems.at[0, slot])

    def cp_wq(h, slot):
        return pltpu.make_async_copy(wq_hbm.at[:, hcol(h)], wqb.at[slot], hsems.at[1, slot])

    def cp_v(h, slot):
        return pltpu.make_async_copy(v_hbm.at[h], vb.at[slot], hsems.at[2, slot])

    def cp_wo(h, slot):
        return pltpu.make_async_copy(wo_hbm.at[hcol(h), :], wob.at[slot], hsems.at[3, slot])

    def cp_head(h, slot):
        return (cp_wq(h, slot), cp_k(h, slot), cp_v(h, slot), cp_wo(h, slot))

    def cp_x(i):
        return pltpu.make_async_copy(x_hbm.at[pl.ds(i * tq, tq), :], x_ref.at[pl.ds(i * tq, tq), :], xsems.at[i])

    def cp_out(i):
        return pltpu.make_async_copy(ob_ref.at[pl.ds(i * tq, tq), :], out_hbm.at[pl.ds(i * tq, tq), :], osems.at[i])

    def cp_ffn():
        return (pltpu.make_async_copy(wg_hbm, wg_ref, fsems.at[0]),
                pltpu.make_async_copy(wu_hbm, wu_ref, fsems.at[1]),
                pltpu.make_async_copy(wd_hbm, wd_ref, fsems.at[2]))

    def router(xn32):
        wr = wr_ref[...].astype(_F32)
        return _bf(jnp.sum(xn32 * wr, axis=-1, keepdims=True))

    def layernorm(i, rt):
        rows = slice(i * tq, (i + 1) * tq)
        x = x_ref[rows, :].astype(_F32)
        mean = jnp.sum(x, axis=-1, keepdims=True) * (1.0 / D)
        xc = x - mean
        var = jnp.sum(xc * xc, axis=-1, keepdims=True) * (1.0 / D)
        num = _bf(x - _bf(mean))
        den = _bf(jnp.sqrt(_bf(_bf(var) + _bf(jnp.float32(_EPS)))))
        xn = (num * (1.0 / den)).astype(_BF16)
        xn32 = xn.astype(_F32)
        xn_ref[rows, :] = xn
        z_ref[rows, :] = xn32
        lane = jax.lax.broadcasted_iota(_I32, (tq, 128), 1)
        return jnp.where(lane == i, router(xn32), rt)

    def qproj(i, slot):
        r0 = i * tq
        w = wqb.at[slot]
        q = jnp.dot(xn_ref[r0:r0 + tq, 0:D4], w[0:D4, :], preferred_element_type=_F32)
        q = q + jnp.concatenate(
            [jnp.dot(xn_ref[r0 + t * tb:r0 + (t + 1) * tb, D4:D], w[D4:D, :], preferred_element_type=_F32)
             for t in range(4)], axis=0)
        return (q * scale).astype(_BF16)

    def qk(i, slot, q, z):
        s = jax.lax.dot_general(q, kb[slot], _NT, preferred_element_type=_F32)
        s_ref[z + i % 2] = s
        return jnp.broadcast_to(jnp.max(s, axis=-1, keepdims=True), (tq, 128))

    def finalize(r0, nr, c0, c1, s):
        out = x_ref[r0:r0 + nr, c0:c1].astype(_F32) + s * _silu(z_ref[r0:r0 + nr, c0:c1])
        ob_ref[r0:r0 + nr, c0:c1] = out.astype(_BF16)

    def wo(i, slot, o, lp, mode):
        l = jnp.sum(lp, axis=-1, keepdims=True)
        o = (o * (1.0 / l)).astype(_BF16)
        r0 = i * tq
        w = wob.at[slot]

        def emit(r0, nr, c0, c1, a):
            if mode == "init":
                acc_ref[r0:r0 + nr, c0:c1] = a
            elif mode == "acc":
                acc_ref[r0:r0 + nr, c0:c1] += a
            else:
                finalize(r0, nr, c0, c1, acc_ref[r0:r0 + nr, c0:c1] + a)

        a = jnp.dot(o, w[:, 0:D4], preferred_element_type=_F32)
        emit(r0, tq, 0, D4, a)
        for t in range(4):
            emit(r0 + t * tb, tb, D4, D,
                 jnp.dot(o[t * tb:(t + 1) * tb, :], w[:, D4:D], preferred_element_type=_F32))
        return a[:, 0:128]

    def pv(i, slot, m, gate, z):
        o = lp = None
        for c in range(R):
            mc = m if gate is None else _after(gate, m)
            sc = s_ref[z + i % 2, :, c * cw:(c + 1) * cw]
            pe = jnp.exp2(sc - jnp.concatenate([mc] * (cw // 128), axis=1))
            ps = [pe[:, j * 128:(j + 1) * 128] for j in range(cw // 128)]
            for pj in ps:
                lp = pj if lp is None else lp + pj
            ps[-1] = _after(lp, ps[-1])
            pb = jnp.concatenate(ps, axis=1).astype(_BF16)
            oc = jnp.dot(pb, vb[slot, c * cw:(c + 1) * cw, :], preferred_element_type=_F32)
            o = oc if o is None else o + oc
            gate = o
        return o, _after(o, lp)

    def topk(rt):
        lane = jax.lax.broadcasted_iota(_I32, (tq, 128), 1)
        row = jax.lax.broadcasted_iota(_I32, (tq, 128), 0)
        bits = pltpu.bitcast(jnp.where(rt == 0.0, 0.0, rt), _I32)
        mono = jnp.where(bits < 0, bits ^ 0x7FFFFFFF, bits) & -65536
        mono = jnp.where(rt != rt, _INT_MIN, mono)
        key = jnp.where(lane < n, mono | (65535 - (lane * tq + row)), _INT_MIN)
        for c in range(_TOPC):
            kmax = jnp.max(jnp.max(key, axis=0, keepdims=True), axis=1, keepdims=True)
            sel_ref[c] = jnp.clip(65535 - (kmax[0, 0] & 65535), 0, S - 1)
            key = jnp.where(key == kmax, _INT_MIN, key)

    def ffn():
        rowid = jax.lax.broadcasted_iota(_I32, (_TOPC, 1), 0)
        xs = jnp.zeros((_TOPC, D), _F32)
        for c in range(_TOPC):
            xs = jnp.where(rowid == c, z_ref[pl.ds(sel_ref[c], 1), :], xs)
        rs = router(xs)
        xb = xs.astype(_BF16)
        g = _bf(jax.lax.dot_general(xb, wg_ref[...], _NT, preferred_element_type=_F32))
        u = _bf(jax.lax.dot_general(xb, wu_ref[...], _NT, preferred_element_type=_F32))
        hid = (_bf(_silu(g)) * u).astype(_BF16)
        y = _bf(jnp.dot(hid, wd_ref[...], preferred_element_type=_F32))
        zz = _bf(xs + _bf(y * _bf(_sigmoid(rs))))
        for c in range(_TOPC):
            z_ref[pl.ds(sel_ref[c], 1), :] = zz[c:c + 1, :]

    zs[0] = jnp.minimum(pl.program_id(0), 0)
    for c in (cp_x(0), cp_wq(0, 0), cp_k(0, 0), cp_x(1)):
        c.start()
    cp_x(0).wait()
    cp_wq(0, 0).wait()
    for c in (cp_v(0, 0), cp_x(2), cp_wo(0, 0), cp_x(3), cp_x(4)):
        c.start()
    z = zs[0]
    rt = layernorm(0, jnp.zeros((tq, 128), _F32))
    q = qproj(0, 0)
    cp_k(0, 0).wait()
    cp_x(1).wait()
    for i in range(5, n):
        cp_x(i).start()
    for c in cp_head(1, 1):
        c.start()
    m = qk(0, 0, q, z)
    o = lp = None
    for u in range(p):
        rt = layernorm(u + 1, rt)
        m_next = qk(u + 1, 0, qproj(u + 1, 0), z)
        if u == 0:
            cp_v(0, 0).wait()
            cp_x(2).wait()
        if u == 1:
            cp_wo(0, 0).wait()
            for i in range(3, n):
                cp_x(i).wait()
            for c in cp_head(2, 2) + cp_ffn():
                c.start()
        gate = None if o is None else wo(u - 1, 0, o, lp, "init")
        o, lp = pv(u, 0, m, gate, z)
        m = m_next
    for i in range(p + 1, n):
        rt = layernorm(i, rt)
    acc_ref[(p - 1) * tq:, :] = jnp.zeros((S - (p - 1) * tq, D), _F32)
    topk(rt)
    mc_ref[...], oc_ref[...], lc_ref[...] = m, o, lp
    for c in cp_head(1, 1):
        c.wait()

    def body(h, carry):
        z = zs[0]
        s0 = h % NS
        s1 = (h + 1) % NS
        slot = lambda u: s0 if u < n else s1
        m, o, lp = mc_ref[...], oc_ref[...], lc_ref[...]
        for u in range(p, p + n):
            m_next = qk((u + 1) % n, slot(u + 1), qproj((u + 1) % n, slot(u + 1)), z)
            gate = wo((u - 1) % n, slot(u - 1), o, lp, "acc")
            o, lp = pv(u % n, slot(u), m, gate, z)
            m = m_next
        mc_ref[...], oc_ref[...], lc_ref[...] = m, o, lp
        for c in cp_head(0, (h + 2) % NS):
            c.wait()
        for c in cp_head(jnp.minimum(h + 3, H - 1), s0):
            c.start()
        return carry

    jax.lax.fori_loop(0, H - 1, body, 0)

    z = zs[0]
    sl = (H - 1) % NS
    for c in cp_ffn():
        c.wait()
    m, o, lp = mc_ref[...], oc_ref[...], lc_ref[...]
    for u in range(p, n):
        m_next = None
        if u + 1 < n:
            m_next = qk(u + 1, sl, qproj(u + 1, sl), z)
        if u == p:
            ffn()
            for i in range(p - 1):
                finalize(i * tq, tq, 0, D, acc_ref[i * tq:(i + 1) * tq, :])
                cp_out(i).start()
        gate = wo(u - 1, sl, o, lp, "final")
        cp_out(u - 1).start()
        o, lp = pv(u, sl, m, gate, z)
        m = m_next
    wo(n - 1, sl, o, lp, "final")
    cp_out(n - 1).start()
    for c in cp_head(0, (H - 2) % NS):
        c.wait()
    for i in range(n):
        cp_out(i).wait()


@jax.jit
def pallas_recurrent_scan__mha_block_cached__moe_arch_mod__prompt_kernel(
    A_x: jax.Array,
    A_k_cache: jax.Array,
    A_v_cache: jax.Array,
    A_wq: jax.Array,
    A_wo: jax.Array,
    B_x: jax.Array,
    B_w_r: jax.Array,
    B_w_gate: jax.Array,
    B_w_up: jax.Array,
    B_w_down: jax.Array,
):
    B, S, D = A_x.shape
    _, H, Sk, Dh = A_k_cache.shape
    F = B_w_gate.shape[1]
    assert B == 1 and Sk == S and S % _TQ == 0 and S % _CW == 0 and Dh == 128 and D % 512 == 128
    n = S // _TQ
    assert n % 2 == 0 and 2 <= _P < n - 1 and n <= 128 and H >= 3 and S <= 65536
    hbm = pl.BlockSpec(memory_space=pltpu.HBM)
    out = pl.pallas_call(
        functools.partial(_kernel, S=S, D=D, Dh=Dh, H=H),
        grid=(1,),
        in_specs=[hbm, hbm, hbm, hbm, hbm, pl.BlockSpec((1, D), lambda i: (0, 0)), hbm, hbm, hbm],
        out_specs=pl.BlockSpec(memory_space=pl.ANY),
        out_shape=jax.ShapeDtypeStruct((S, D), _BF16),
        scratch_shapes=[
            pltpu.VMEM((S, D), _BF16),
            pltpu.VMEM((S, D), _BF16),
            pltpu.VMEM((S, D), _F32),
            pltpu.VMEM((S, D), _F32),
            pltpu.VMEM((S, D), _BF16),
            pltpu.VMEM((2, _TQ, S), _F32),
            pltpu.VMEM((_TQ, 128), _F32),
            pltpu.VMEM((_TQ, Dh), _F32),
            pltpu.VMEM((_TQ, 128), _F32),
            pltpu.VMEM((_NS, S, Dh), _BF16),
            pltpu.VMEM((_NS, S, Dh), _BF16),
            pltpu.VMEM((_NS, D, Dh), _BF16),
            pltpu.VMEM((_NS, Dh, D), _BF16),
            pltpu.VMEM((F, D), _BF16),
            pltpu.VMEM((F, D), _BF16),
            pltpu.VMEM((F, D), _BF16),
            pltpu.SMEM((_TOPC,), _I32),
            pltpu.SMEM((1,), _I32),
            pltpu.SemaphoreType.DMA((4, _NS)),
            pltpu.SemaphoreType.DMA((n,)),
            pltpu.SemaphoreType.DMA((n,)),
            pltpu.SemaphoreType.DMA((3,)),
        ],
        compiler_params=pltpu.CompilerParams(
            dimension_semantics=("arbitrary",),
            vmem_limit_bytes=100 * 1024 * 1024,
            internal_scratch_in_bytes=64 * 1024,
        ),
    )(A_x.reshape(S, D), A_k_cache.reshape(H, Sk, Dh), A_v_cache.reshape(H, Sk, Dh), A_wq, A_wo,
      B_w_r.reshape(1, D), B_w_gate.T, B_w_up.T, B_w_down)
    return out.reshape(B, S, D)
```

```python
import functools
import math

import jax
import jax.numpy as jnp
import jax.experimental.pallas as pl
import jax.experimental.pallas.tpu as pltpu

_F32 = jnp.float32
_BF16 = jnp.bfloat16
_I32 = jnp.int32
_NT = (((1,), (1,)), ((), ()))

_TOPC = 8
_EPS = 1e-5
_TQ = 256
_CW = 512
_P = 4
_NS = 3
_INT_MIN = -2 ** 31


def _bf(x):
    return x.astype(_BF16).astype(_F32)


def _silu(x):
    h = 0.5 * x
    return h + h * jnp.tanh(h)


def _sigmoid(x):
    return 0.5 + 0.5 * jnp.tanh(0.5 * x)


def _after(gate, val):
    return jnp.where(gate > jnp.inf, 0.0, val)


def _kernel(x_hbm, k_hbm, v_hbm, wq_hbm, wo_hbm, wr_ref, wg_hbm, wu_hbm, wd_hbm,
            out_hbm,
            x_ref, xn_ref, z_ref, acc_ref, ob_ref, s_ref, mc_ref, oc_ref, lc_ref, qs_ref,
            kb, vb, wqb, wob, wg_ref, wu_ref, wd_ref, sel_ref, zs,
            hsems, xsems, osems, fsems,
            *, S, D, Dh, H):
    tq, cw, p, NS = _TQ, _CW, _P, _NS
    n = S // tq
    R = S // cw
    tb = tq // 4
    D4 = (D // 512) * 512
    F = wd_ref.shape[0]
    scale = (Dh ** -0.5) * math.log2(math.e)

    def hcol(h):
        return pl.ds(pl.multiple_of(h * Dh, Dh), Dh)

    def cp_k(h, slot):
        return pltpu.make_async_copy(k_hbm.at[h], kb.at[slot], hsems.at[0, slot])

    def cp_wq(h, slot):
        return pltpu.make_async_copy(wq_hbm.at[:, hcol(h)], wqb.at[slot], hsems.at[1, slot])

    def cp_v(h, slot):
        return pltpu.make_async_copy(v_hbm.at[h], vb.at[slot], hsems.at[2, slot])

    def cp_wo(h, slot):
        return pltpu.make_async_copy(wo_hbm.at[hcol(h), :], wob.at[slot], hsems.at[3, slot])

    def cp_head(h, slot):
        return (cp_wq(h, slot), cp_k(h, slot), cp_v(h, slot), cp_wo(h, slot))

    def cp_x(i):
        return pltpu.make_async_copy(x_hbm.at[pl.ds(i * tq, tq), :], x_ref.at[pl.ds(i * tq, tq), :], xsems.at[i])

    def cp_out(i, z):
        src = pl.ds(pl.multiple_of(z * tq + i * tq, tq), tq)
        return pltpu.make_async_copy(ob_ref.at[src, :], out_hbm.at[pl.ds(i * tq, tq), :], osems.at[i])

    def cp_ffn():
        return (pltpu.make_async_copy(wg_hbm, wg_ref, fsems.at[0]),
                pltpu.make_async_copy(wu_hbm, wu_ref, fsems.at[1]),
                pltpu.make_async_copy(wd_hbm, wd_ref, fsems.at[2]))

    def lanes(v, k):
        return jnp.concatenate([v] * k, axis=1)

    def rows(v, k):
        return jnp.concatenate([v] * k, axis=0)

    def fold(v):
        t = v[:, 0:128]
        for j in range(1, v.shape[1] // 128):
            t = t + v[:, j * 128:(j + 1) * 128]
        return t

    def compact(col, g0, init):
        lane = jax.lax.broadcasted_iota(_I32, (8, 128), 1)
        for g in range(col.shape[0] // 8):
            init = jnp.where(lane == (g0 + g) % 128, col[8 * g:8 * g + 8, :], init)
        return init

    def layernorm(r0, nr, rt):
        x = x_ref[r0:r0 + nr, :].astype(_F32)
        mean = jnp.sum(x, axis=-1, keepdims=True) * (1.0 / D)
        xc = x - mean
        var = compact(jnp.sum(xc * xc, axis=-1, keepdims=True), 0, jnp.ones((8, 128), _F32)) * (1.0 / D)
        inv = 1.0 / _bf(jnp.sqrt(_bf(_bf(var) + _bf(jnp.float32(_EPS)))))
        inv = jnp.concatenate([jnp.broadcast_to(inv[:, g:g + 1], (8, 128)) for g in range(nr // 8)], axis=0)
        xn = (_bf(x - _bf(mean)) * lanes(inv, D // 128)).astype(_BF16)
        xn32 = xn.astype(_F32)
        xn_ref[r0:r0 + nr, :] = xn
        z_ref[r0:r0 + nr, :] = xn32
        rp = fold(xn32 * wr_ref[...].astype(_F32))
        if r0 >= (p - 1) * tq:
            zero = _after(rp, 0.0)
            acc_ref[r0:r0 + nr, :] = lanes(zero, D // 128)
            rp = rp + zero
        g0 = r0 // 8
        rt[g0 // 128] = compact(jnp.sum(rp, axis=-1, keepdims=True), g0, rt[g0 // 128])
        return rt[g0 // 128]

    def qproj(i, slot):
        r0 = i * tq
        w = wqb.at[slot]
        q = jnp.dot(xn_ref[r0:r0 + tq, 0:D4], w[0:D4, :], preferred_element_type=_F32)
        q = q + jnp.concatenate(
            [jnp.dot(xn_ref[r0 + t * tb:r0 + (t + 1) * tb, D4:D], w[D4:D, :], preferred_element_type=_F32)
             for t in range(4)], axis=0)
        return (q * scale).astype(_BF16)

    def gated_bf16(packed, gates):
        for g in gates:
            packed = jnp.where(lanes(rows(g > jnp.inf, packed.shape[0] // 8), packed.shape[1] // 128),
                               jnp.uint32(0), packed)
        return pltpu.bitcast(packed, _BF16)

    def qk(i, slot, q, z, fill=None):
        if fill is None:
            s = jax.lax.dot_general(q, kb[slot], _NT, preferred_element_type=_F32)
            s_ref[z + i % 2] = s
            return jnp.broadcast_to(jnp.max(s, axis=-1, keepdims=True), (tq, 128))
        qs_ref.bitcast(_BF16)[...] = q
        mx = None
        for c in range(R):
            qc = gated_bf16(qs_ref[...], [f() for f in fill[c]])
            s = jax.lax.dot_general(qc, kb[slot, c * cw:(c + 1) * cw, :], _NT, preferred_element_type=_F32)
            s_ref[z + i % 2, :, c * cw:(c + 1) * cw] = s
            for j in range(cw // 128):
                sj = s[:, j * 128:(j + 1) * 128]
                mx = sj if mx is None else jnp.maximum(mx, sj)
        return jnp.broadcast_to(jnp.max(mx, axis=-1, keepdims=True), (tq, 128))

    def finalize(r0, nr, c0, c1, s):
        out = x_ref[r0:r0 + nr, c0:c1].astype(_F32) + s * z_ref[r0:r0 + nr, c0:c1]
        ob_ref[r0:r0 + nr, c0:c1] = out.astype(_BF16)

    def stored(ref, r0, z):
        k = 32 // (8 * ref.dtype.itemsize)
        v = ref[pl.ds(pl.multiple_of(z * 8 * k + r0, 8 * k), 8 * k), 0:128]
        return v if k == 1 else pltpu.bitcast(v, _F32)

    def wo(i, slot, o, lp, mode):
        l = jnp.sum(lp, axis=-1, keepdims=True)
        o = (o * (1.0 / l)).astype(_BF16)
        r0 = i * tq
        w = wob.at[slot]

        def emit(r0, nr, c0, c1, a):
            if mode == "init":
                acc_ref[r0:r0 + nr, c0:c1] = a
            elif mode == "acc":
                acc_ref[r0:r0 + nr, c0:c1] += a
            else:
                finalize(r0, nr, c0, c1, acc_ref[r0:r0 + nr, c0:c1] + a)

        a = jnp.dot(o, w[:, 0:D4], preferred_element_type=_F32)
        emit(r0, tq, 0, D4, a)
        for t in range(4):
            emit(r0 + t * tb, tb, D4, D,
                 jnp.dot(o[t * tb:(t + 1) * tb, :], w[:, D4:D], preferred_element_type=_F32))
        return a[:, 0:128]

    def pv(i, slot, m, gate, z, fill=None, last=False):
        o = lp = None
        for c in range(R):
            mc = m if gate is None else _after(gate, m)
            for f in ([] if fill is None else fill[c]):
                mc = _after(rows(f(), tq // 8), mc)
            sc = s_ref[z + i % 2, :, c * cw:(c + 1) * cw]
            pe = jnp.exp2(sc - lanes(mc, cw // 128))
            ps = [pe[:, j * 128:(j + 1) * 128] for j in range(cw // 128)]
            for pj in ps:
                lp = pj if lp is None else lp + pj
            ps[-1] = _after(lp, ps[-1])
            pb = jnp.concatenate(ps, axis=1).astype(_BF16)
            oc = jnp.dot(pb, vb[slot, c * cw:(c + 1) * cw, :], preferred_element_type=_F32)
            o = oc if o is None else o + oc
            gate = o
        return o, (lp if last else _after(o, lp))

    def topk(rt):
        rt = _bf(jnp.concatenate(rt, axis=1))
        lane = jax.lax.broadcasted_iota(_I32, rt.shape, 1)
        sub = jax.lax.broadcasted_iota(_I32, rt.shape, 0)
        bits = pltpu.bitcast(jnp.where(rt == 0.0, 0.0, rt), _I32)
        mono = jnp.where(bits < 0, bits ^ 0x7FFFFFFF, bits) & -65536
        mono = jnp.where(rt != rt, _INT_MIN, mono)
        key = mono | (65535 - (lane * 8 + sub))
        for c in range(_TOPC):
            kmax = jnp.max(jnp.max(key, axis=0, keepdims=True), axis=1, keepdims=True)
            sel_ref[c] = jnp.clip(65535 - (kmax[0, 0] & 65535), 0, S - 1)
            key = jnp.where(key == kmax, _INT_MIN, key)

    def ffn(z):
        rowid = jax.lax.broadcasted_iota(_I32, (_TOPC, 1), 0)
        xs = jnp.zeros((_TOPC, D), _F32)
        for c in range(_TOPC):
            xs = jnp.where(rowid == c, z_ref[pl.ds(sel_ref[c], 1), :], xs)
        rs = _bf(jnp.sum(fold(xs * wr_ref[...].astype(_F32)), axis=-1, keepdims=True))
        cuts = list(range(0, F, cw)) + [F]
        npc = 2 * (len(cuts) - 1)
        pr = S // npc

        def proj(w_ref, k0):
            parts = []
            for k in range(len(cuts) - 1):
                r0 = (k0 + k) * pr
                z_ref[r0:r0 + pr, :] = _silu(z_ref[r0:r0 + pr, :])
                xb = _after(lanes(stored(z_ref, r0, z), D // 128), xs).astype(_BF16)
                parts.append(jax.lax.dot_general(xb, w_ref[cuts[k]:cuts[k + 1], :], _NT,
                                                 preferred_element_type=_F32))
            return _bf(jnp.concatenate(parts, axis=1))

        g = proj(wg_ref, 0)
        u = proj(wu_ref, npc // 2)
        hid = (_bf(_silu(g)) * u).astype(_BF16)
        y = _bf(jnp.dot(hid, wd_ref[...], preferred_element_type=_F32))
        zz = _silu(_bf(xs + _bf(y * _bf(_sigmoid(rs)))))
        for c in range(_TOPC):
            z_ref[pl.ds(sel_ref[c], 1), :] = zz[c:c + 1, :]

    zs[0] = jnp.minimum(pl.program_id(0), 0)
    for c in (cp_x(0), cp_wq(0, 0), cp_k(0, 0), cp_x(1)):
        c.start()
    cp_x(0).wait()
    cp_wq(0, 0).wait()
    for c in (cp_v(0, 0), cp_x(2), cp_x(3), cp_wo(0, 0), cp_x(4), cp_x(5)):
        c.start()
    z = zs[0]
    rt = [jnp.zeros((8, 128), _F32) for _ in range(S // 1024)]

    def ln_fill(chunks):
        pieces = [(i * tq + t * tb, tb) for i in chunks for t in range(4)]
        k = len(pieces) // R
        return [[functools.partial(layernorm, r0, nr, rt) for r0, nr in pieces[c * k:(c + 1) * k]]
                for c in range(R)]

    for t in range(4):
        layernorm(t * tb, tb, rt)
    q = qproj(0, 0)
    cp_k(0, 0).wait()
    cp_x(1).wait()
    for i in range(6, n):
        cp_x(i).start()
    for c in cp_head(1, 1):
        c.start()
    m = qk(0, 0, q, z, ln_fill([1]))
    o = lp = None
    for u in range(p):
        q = qproj(u + 1, 0)
        if u == 0:
            cp_v(0, 0).wait()
        if u == 1:
            cp_wo(0, 0).wait()
        todo = [i for i in (2 * u + 2, 2 * u + 3) if i < n]
        for i in todo:
            cp_x(i).wait()
        if u == 1:
            for c in cp_head(2, 2) + cp_ffn():
                c.start()
        m_next = qk(u + 1, 0, q, z, ln_fill(todo) if todo else None)
        gate = None if o is None else wo(u - 1, 0, o, lp, "init")
        o, lp = pv(u, 0, m, gate, z, last=(u == p - 1))
        m = m_next
    topk(rt)
    mc_ref[...], oc_ref[...], lc_ref[...] = m, o, lp
    for c in cp_head(1, 1):
        c.wait()

    def body(h, slots):
        z = zs[0]
        s0, s1, s2 = slots
        slot = lambda u: s0 if u < n else s1
        m, o, lp = mc_ref[...], oc_ref[...], lc_ref[...]
        for u in range(p, p + n):
            m_next = qk((u + 1) % n, slot(u + 1), qproj((u + 1) % n, slot(u + 1)), z)
            gate = wo((u - 1) % n, slot(u - 1), o, lp, "acc")
            if u == n:
                for c in cp_head(jnp.minimum(h + 3, H - 1), s0):
                    c.start()
            o, lp = pv(u % n, slot(u), m, gate, z, last=(u == p + n - 1))
            m = m_next
        mc_ref[...], oc_ref[...], lc_ref[...] = m, o, lp
        for c in cp_head(0, s2):
            c.wait()
        return s1, s2, s0

    jax.lax.fori_loop(0, H - 1, body, (jnp.int32(0), jnp.int32(1), jnp.int32(2)))

    z = zs[0]
    sl = (H - 1) % NS
    for c in cp_ffn():
        c.wait()
    m, o, lp = mc_ref[...], oc_ref[...], lc_ref[...]

    def fin_piece(r0, nr):
        finalize(r0, nr, 0, D, acc_ref[r0:r0 + nr, :])
        if (r0 + nr) % tq == 0:
            cp_out(r0 // tq, z).start()
        return stored(ob_ref, r0, z)

    ffn(z)
    for u in range(p, n):
        m_next = None
        if u + 1 < n:
            fill = None
            if u == p:
                pieces = [(r0, tb) for r0 in range(0, (p - 1) * tq, tb)]
                k = len(pieces) // R
                fill = [[functools.partial(fin_piece, *pc) for pc in pieces[c * k:(c + 1) * k]] for c in range(R)]
            m_next = qk(u + 1, sl, qproj(u + 1, sl), z, fill)
        gate = wo(u - 1, sl, o, lp, "final")
        cp_out(u - 1, z).start()
        fill = [[], [], [functools.partial(stored, ob_ref, (u - 1) * tq, z)], []]
        o, lp = pv(u, sl, m, gate, z, fill)
        m = m_next
    wo(n - 1, sl, o, lp, "final")
    cp_out(n - 1, z).start()
    for c in cp_head(0, (H - 2) % NS):
        c.wait()
    for i in range(n):
        cp_out(i, z).wait()


@jax.jit
def pallas_recurrent_scan__mha_block_cached__moe_arch_mod__prompt_kernel(
    A_x: jax.Array,
    A_k_cache: jax.Array,
    A_v_cache: jax.Array,
    A_wq: jax.Array,
    A_wo: jax.Array,
    B_x: jax.Array,
    B_w_r: jax.Array,
    B_w_gate: jax.Array,
    B_w_up: jax.Array,
    B_w_down: jax.Array,
):
    B, S, D = A_x.shape
    _, H, Sk, Dh = A_k_cache.shape
    F = B_w_gate.shape[1]
    assert B == 1 and Sk == S and S % _TQ == 0 and S % _CW == 0 and Dh == 128 and D % 512 == 128
    n = S // _TQ
    assert n % 2 == 0 and 2 <= _P < n - 1 and n <= 2 * _P and H >= 3 and S % 1024 == 0 and S <= 65536
    hbm = pl.BlockSpec(memory_space=pltpu.HBM)
    out = pl.pallas_call(
        functools.partial(_kernel, S=S, D=D, Dh=Dh, H=H),
        grid=(1,),
        in_specs=[hbm, hbm, hbm, hbm, hbm, pl.BlockSpec((1, D), lambda i: (0, 0)), hbm, hbm, hbm],
        out_specs=pl.BlockSpec(memory_space=pl.ANY),
        out_shape=jax.ShapeDtypeStruct((S, D), _BF16),
        scratch_shapes=[
            pltpu.VMEM((S, D), _BF16),
            pltpu.VMEM((S, D), _BF16),
            pltpu.VMEM((S, D), _F32),
            pltpu.VMEM((S, D), _F32),
            pltpu.VMEM((S, D), _BF16),
            pltpu.VMEM((2, _TQ, S), _F32),
            pltpu.VMEM((_TQ, 128), _F32),
            pltpu.VMEM((_TQ, Dh), _F32),
            pltpu.VMEM((_TQ, 128), _F32),
            pltpu.VMEM((_TQ // 2, Dh), jnp.uint32),
            pltpu.VMEM((_NS, S, Dh), _BF16),
            pltpu.VMEM((_NS, S, Dh), _BF16),
            pltpu.VMEM((_NS, D, Dh), _BF16),
            pltpu.VMEM((_NS, Dh, D), _BF16),
            pltpu.VMEM((F, D), _BF16),
            pltpu.VMEM((F, D), _BF16),
            pltpu.VMEM((F, D), _BF16),
            pltpu.SMEM((_TOPC,), _I32),
            pltpu.SMEM((1,), _I32),
            pltpu.SemaphoreType.DMA((4, _NS)),
            pltpu.SemaphoreType.DMA((n,)),
            pltpu.SemaphoreType.DMA((n,)),
            pltpu.SemaphoreType.DMA((3,)),
        ],
        compiler_params=pltpu.CompilerParams(
            dimension_semantics=("arbitrary",),
            vmem_limit_bytes=100 * 1024 * 1024,
            disable_bounds_checks=True,
            internal_scratch_in_bytes=64 * 1024,
        ),
    )(A_x.reshape(S, D), A_k_cache.reshape(H, Sk, Dh), A_v_cache.reshape(H, Sk, Dh), A_wq, A_wo,
      B_w_r.reshape(1, D), B_w_gate.T, B_w_up.T, B_w_down)
    return out.reshape(B, S, D)
```

```python
import functools
import math

import jax
import jax.numpy as jnp
import jax.experimental.pallas as pl
import jax.experimental.pallas.tpu as pltpu

_F32 = jnp.float32
_BF16 = jnp.bfloat16
_I32 = jnp.int32
_NT = (((1,), (1,)), ((), ()))

_TOPC = 8
_EPS = 1e-5
_TQ = 256
_CW = 512
_P = 4
_NS = 3
_INT_MIN = -2 ** 31


def _bf(x):
    return x.astype(_BF16).astype(_F32)


def _silu(x):
    h = 0.5 * x
    return h + h * jnp.tanh(h)


def _sigmoid(x):
    return 0.5 + 0.5 * jnp.tanh(0.5 * x)


def _after(gate, val):
    return jnp.where(gate > jnp.inf, 0.0, val)


def _kernel(x_hbm, k_hbm, v_hbm, wq_hbm, wo_hbm, wr_ref, wg_hbm, wu_hbm, wd_hbm,
            out_hbm,
            x_ref, xnp_ref, z_ref, acc_ref, ob_ref, s_ref, mc_ref, oc_ref, lc_ref, qs_ref,
            kb, vb, wqb, wob, wg_ref, wu_ref, wd_ref, sel_ref, zs,
            sems,
            *, S, D, Dh, H):
    tq, cw, p, NS = _TQ, _CW, _P, _NS
    n = S // tq
    R = S // cw
    tb = tq // 4
    D4 = (D // 512) * 512
    F = wd_ref.shape[0]
    scale = (Dh ** -0.5) * math.log2(math.e)
    xn_ref = xnp_ref.bitcast(_BF16)

    def hcol(h):
        return pl.ds(pl.multiple_of(h * Dh, Dh), Dh)

    def cp_k(h, slot):
        return pltpu.make_async_copy(k_hbm.at[h], kb.at[slot], sems.at[0 * NS + slot])

    def cp_wq(h, slot):
        return pltpu.make_async_copy(wq_hbm.at[:, hcol(h)], wqb.at[slot], sems.at[1 * NS + slot])

    def cp_v(h, slot):
        return pltpu.make_async_copy(v_hbm.at[h], vb.at[slot], sems.at[2 * NS + slot])

    def cp_wo(h, slot):
        return pltpu.make_async_copy(wo_hbm.at[hcol(h), :], wob.at[slot], sems.at[3 * NS + slot])

    def cp_head(h, slot):
        return (cp_wq(h, slot), cp_k(h, slot), cp_v(h, slot), cp_wo(h, slot))

    def cp_x(i):
        return pltpu.make_async_copy(x_hbm.at[pl.ds(i * tq, tq), :], x_ref.at[pl.ds(i * tq, tq), :], sems.at[4 * NS + i])

    def cp_out(i, z):
        src = pl.ds(pl.multiple_of(z * tq + i * tq, tq), tq)
        return pltpu.make_async_copy(ob_ref.at[src, :], out_hbm.at[pl.ds(i * tq, tq), :], sems.at[4 * NS + n + i])

    def cp_ffn():
        return (pltpu.make_async_copy(wg_hbm, wg_ref, sems.at[4 * NS + 2 * n + 0]),
                pltpu.make_async_copy(wu_hbm, wu_ref, sems.at[4 * NS + 2 * n + 1]),
                pltpu.make_async_copy(wd_hbm, wd_ref, sems.at[4 * NS + 2 * n + 2]))

    def lanes(v, k):
        return jnp.concatenate([v] * k, axis=1)

    def rows(v, k):
        return jnp.concatenate([v] * k, axis=0)

    def fold(v):
        t = v[:, 0:128]
        for j in range(1, v.shape[1] // 128):
            t = t + v[:, j * 128:(j + 1) * 128]
        return t

    def compact(col, g0, init):
        lane = jax.lax.broadcasted_iota(_I32, (8, 128), 1)
        for g in range(col.shape[0] // 8):
            init = jnp.where(lane == (g0 + g) % 128, col[8 * g:8 * g + 8, :], init)
        return init

    def layernorm(r0, nr, rt, z, rel=None):
        def x(k):
            return x_ref[pl.ds(pl.multiple_of(k * z * 16 + r0, 16), nr), :].astype(_F32)
        xs = fold(x(0))
        if rel is not None:
            xs = _after(rows(rel, nr // 8), xs)
        mean = jnp.sum(xs, axis=-1, keepdims=True) * (1.0 / D)
        xc = x(1) - mean
        var = compact(jnp.sum(xc * xc, axis=-1, keepdims=True), 0, jnp.ones((8, 128), _F32)) * (1.0 / D)
        inv = 1.0 / _bf(jnp.sqrt(_bf(_bf(var) + _bf(jnp.float32(_EPS)))))
        inv = jnp.concatenate([jnp.broadcast_to(inv[:, g:g + 1], (8, 128)) for g in range(nr // 8)], axis=0)
        xn = (_bf(x(2) - _bf(mean)) * lanes(inv, D // 128)).astype(_BF16)
        xn_ref[r0:r0 + nr, :] = xn
        rp = fold(xn.astype(_F32) * wr_ref[...].astype(_F32))
        g0 = r0 // 8
        rt[g0 // 128] = compact(jnp.sum(rp, axis=-1, keepdims=True), g0, rt[g0 // 128])

    def qproj(i, slot):
        r0 = i * tq
        w = wqb.at[slot]
        q = jnp.dot(xn_ref[r0:r0 + tq, 0:D4], w[0:D4, :], preferred_element_type=_F32)
        q = q + jnp.concatenate(
            [jnp.dot(xn_ref[r0 + t * tb:r0 + (t + 1) * tb, D4:D], w[D4:D, :], preferred_element_type=_F32)
             for t in range(4)], axis=0)
        return (q * scale).astype(_BF16)

    def gated_bf16(packed, gates):
        for g in gates:
            packed = jnp.where(lanes(rows(g > jnp.inf, packed.shape[0] // 8), packed.shape[1] // 128),
                               jnp.uint32(0), packed)
        return pltpu.bitcast(packed, _BF16)

    def qk(i, slot, q, z, fill=None, rel=None):
        if fill is None:
            s = jax.lax.dot_general(q, kb[slot], _NT, preferred_element_type=_F32)
            s_ref[z + i % 2] = s
            for c in range(R if rel is not None else 0):
                for k, f in enumerate(rel[c]):
                    r0 = k * tq // len(rel[c])
                    f(s[r0:r0 + 8, c * cw:c * cw + 128])
            return jnp.broadcast_to(jnp.max(s, axis=-1, keepdims=True), (tq, 128))
        qs_ref.bitcast(_BF16)[...] = q
        mx = None
        for c in range(R):
            qc = gated_bf16(qs_ref[...], [f() for f in fill[c]])
            s = jax.lax.dot_general(qc, kb[slot, c * cw:(c + 1) * cw, :], _NT, preferred_element_type=_F32)
            s_ref[z + i % 2, :, c * cw:(c + 1) * cw] = s
            for j in range(cw // 128):
                sj = s[:, j * 128:(j + 1) * 128]
                mx = sj if mx is None else jnp.maximum(mx, sj)
        return jnp.broadcast_to(jnp.max(mx, axis=-1, keepdims=True), (tq, 128))

    def finalize(r0, nr, c0, c1, s):
        out = x_ref[r0:r0 + nr, c0:c1].astype(_F32) + s * z_ref[r0:r0 + nr, c0:c1]
        ob_ref[r0:r0 + nr, c0:c1] = out.astype(_BF16)

    def stored(ref, r0, z):
        k = 32 // (8 * ref.dtype.itemsize)
        v = ref[pl.ds(pl.multiple_of(z * 8 * k + r0, 8 * k), 8 * k), 0:128]
        return v if k == 1 else pltpu.bitcast(v, _F32)

    def wo(i, slot, o, lp, mode):
        l = jnp.sum(lp, axis=-1, keepdims=True)
        o = (o * (1.0 / l)).astype(_BF16)
        r0 = i * tq
        w = wob.at[slot]

        def emit(r0, nr, c0, c1, a):
            if mode == "init":
                acc_ref[r0:r0 + nr, c0:c1] = a
            elif mode == "acc":
                acc_ref[r0:r0 + nr, c0:c1] += a
            else:
                finalize(r0, nr, c0, c1, acc_ref[r0:r0 + nr, c0:c1] + a)

        a = jnp.dot(o, w[:, 0:D4], preferred_element_type=_F32)
        emit(r0, tq, 0, D4, a)
        for t in range(4):
            emit(r0 + t * tb, tb, D4, D,
                 jnp.dot(o[t * tb:(t + 1) * tb, :], w[:, D4:D], preferred_element_type=_F32))
        return a[:, 0:128]

    def pv(i, slot, m, gate, z, fill=None, last=False, rel=None):
        o = lp = None
        for c in range(R):
            mc = m if gate is None else _after(gate, m)
            for f in ([] if fill is None else fill[c]):
                mc = _after(rows(f(), tq // 8), mc)
            sc = s_ref[z + i % 2, :, c * cw:(c + 1) * cw]
            pe = jnp.exp2(sc - lanes(mc, cw // 128))
            ps = [pe[:, j * 128:(j + 1) * 128] for j in range(cw // 128)]
            for pj in ps:
                lp = pj if lp is None else lp + pj
            ps[-1] = _after(lp, ps[-1])
            pb = jnp.concatenate(ps, axis=1).astype(_BF16)
            oc = jnp.dot(pb, vb[slot, c * cw:(c + 1) * cw, :], preferred_element_type=_F32)
            for k, f in enumerate([] if rel is None else rel[c]):
                r0 = k * tq // len(rel[c])
                f(oc[r0:r0 + 8, :])
            o = oc if o is None else o + oc
            gate = o
        return o, (lp if last else _after(o, lp))

    def topk(rt):
        rt = _bf(jnp.concatenate(rt, axis=1))
        lane = jax.lax.broadcasted_iota(_I32, rt.shape, 1)
        sub = jax.lax.broadcasted_iota(_I32, rt.shape, 0)
        bits = pltpu.bitcast(jnp.where(rt == 0.0, 0.0, rt), _I32)
        mono = jnp.where(bits < 0, bits ^ 0x7FFFFFFF, bits) & -65536
        mono = jnp.where(rt != rt, _INT_MIN, mono)
        key = mono | (65535 - (lane * 8 + sub))
        for c in range(_TOPC):
            kmax = jnp.max(jnp.max(key, axis=0, keepdims=True), axis=1, keepdims=True)
            sel_ref[c] = jnp.clip(65535 - (kmax[0, 0] & 65535), 0, S - 1)
            key = jnp.where(key == kmax, _INT_MIN, key)

    def ffn(z):
        rowid = jax.lax.broadcasted_iota(_I32, (_TOPC, 1), 0)
        xs = jnp.zeros((_TOPC, D), _F32)
        for c in range(_TOPC):
            w = xnp_ref[pl.ds(sel_ref[c] // 2, 1), :]
            w = jnp.where(sel_ref[c] % 2 == 0, w << 16, w & jnp.uint32(0xFFFF0000))
            xs = jnp.where(rowid == c, pltpu.bitcast(w, _F32), xs)
        rs = _bf(jnp.sum(fold(xs * wr_ref[...].astype(_F32)), axis=-1, keepdims=True))
        cuts = list(range(0, F, cw)) + [F]
        npc = 2 * (len(cuts) - 1)
        pr = S // npc

        def proj(w_ref, k0):
            parts = []
            for k in range(len(cuts) - 1):
                r0 = (k0 + k) * pr
                z_ref[r0:r0 + pr, :] = _silu(xn_ref[r0:r0 + pr, :].astype(_F32))
                xb = _after(lanes(stored(z_ref, r0, z), D // 128), xs).astype(_BF16)
                parts.append(jax.lax.dot_general(xb, w_ref[cuts[k]:cuts[k + 1], :], _NT,
                                                 preferred_element_type=_F32))
            return _bf(jnp.concatenate(parts, axis=1))

        g = proj(wg_ref, 0)
        u = proj(wu_ref, npc // 2)
        hid = (_bf(_silu(g)) * u).astype(_BF16)
        y = _bf(jnp.dot(hid, wd_ref[...], preferred_element_type=_F32))
        zz = _silu(_bf(xs + _bf(y * _bf(_sigmoid(rs)))))
        for c in range(_TOPC):
            z_ref[pl.ds(sel_ref[c], 1), :] = zz[c:c + 1, :]

    zs[0] = jnp.minimum(pl.program_id(0), 0)
    first = (cp_x(0), cp_wq(0, 0), cp_k(0, 0), cp_x(1), cp_v(0, 0), cp_x(2), cp_x(3), cp_wo(0, 0))
    for c in first + tuple(cp_x(i) for i in range(4, n)) + cp_head(1, 1) + cp_head(2, 2) + cp_ffn():
        c.start()
    acc_ref[(p - 1) * tq:, :] = jnp.zeros((S - (p - 1) * tq, D), _F32)
    cp_x(0).wait()
    cp_wq(0, 0).wait()
    z = zs[0]
    rt = [jnp.zeros((8, 128), _F32) for _ in range(S // 1024)]

    def ln(chunks, spread):
        pieces = [functools.partial(layernorm, i * tq + t * tb, tb, rt, z) for i in chunks for t in range(4)]
        assert sum(spread) == len(pieces)
        return [[pieces.pop(0) for _ in range(k)] for k in spread]

    for f in ln([0], [4])[0]:
        f()
    q = qproj(0, 0)
    cp_k(0, 0).wait()
    cp_x(1).wait()
    m = qk(0, 0, q, z, rel=ln([1], [3, 1, 0, 0]))
    o = lp = None
    for u in range(p):
        rel_qk = {1: ln([3], [1, 1, 1, 1]), 2: ln([5, 6], [2, 2, 2, 2]), 3: ln([7], [2, 2, 0, 0])}.get(u)
        rel_pv = {0: ln([2], [2, 2, 0, 0]), 1: ln([4], [1, 1, 1, 1])}.get(u)
        m_next = qk(u + 1, 0, qproj(u + 1, 0), z, rel=rel_qk)
        if u == 0:
            for c in (cp_v(0, 0), cp_x(2), cp_x(3)):
                c.wait()
        if u == 1:
            for c in (cp_wo(0, 0),) + tuple(cp_x(i) for i in range(4, n)):
                c.wait()
        gate = None if o is None else wo(u - 1, 0, o, lp, "init")
        o, lp = pv(u, 0, m, gate, z, last=(u == p - 1), rel=rel_pv)
        m = m_next
    topk(rt)
    mc_ref[...], oc_ref[...], lc_ref[...] = m, o, lp
    for c in cp_head(1, 1):
        c.wait()

    def body(h, slots):
        z = zs[0]
        s0, s1, s2 = slots
        slot = lambda u: s0 if u < n else s1
        m, o, lp = mc_ref[...], oc_ref[...], lc_ref[...]
        for u in range(p, p + n):
            m_next = qk((u + 1) % n, slot(u + 1), qproj((u + 1) % n, slot(u + 1)), z)
            gate = wo((u - 1) % n, slot(u - 1), o, lp, "acc")
            if u == n:
                for c in cp_head(jnp.minimum(h + 3, H - 1), s0):
                    c.start()
            o, lp = pv(u % n, slot(u), m, gate, z, last=(u == p + n - 1))
            m = m_next
        mc_ref[...], oc_ref[...], lc_ref[...] = m, o, lp
        for c in cp_head(0, s2):
            c.wait()
        return s1, s2, s0

    jax.lax.fori_loop(0, H - 1, body, (jnp.int32(0), jnp.int32(1), jnp.int32(2)))

    z = zs[0]
    sl = (H - 1) % NS
    for c in cp_ffn():
        c.wait()
    m, o, lp = mc_ref[...], oc_ref[...], lc_ref[...]

    def fin_piece(r0, nr):
        finalize(r0, nr, 0, D, acc_ref[r0:r0 + nr, :])
        if (r0 + nr) % tq == 0:
            cp_out(r0 // tq, z).start()
        return stored(ob_ref, r0, z)

    ffn(z)
    for u in range(p, n):
        m_next = None
        if u + 1 < n:
            fill = None
            if u == p:
                pieces = [(r0, tb) for r0 in range(0, (p - 1) * tq, tb)]
                k = len(pieces) // R
                fill = [[functools.partial(fin_piece, *pc) for pc in pieces[c * k:(c + 1) * k]] for c in range(R)]
            m_next = qk(u + 1, sl, qproj(u + 1, sl), z, fill)
        gate = wo(u - 1, sl, o, lp, "final")
        cp_out(u - 1, z).start()
        fill = [[], [], [functools.partial(stored, ob_ref, (u - 1) * tq, z)], []]
        o, lp = pv(u, sl, m, gate, z, fill)
        m = m_next
    wo(n - 1, sl, o, lp, "final")
    cp_out(n - 1, z).start()
    for c in cp_head(0, (H - 2) % NS):
        c.wait()
    for i in range(n):
        cp_out(i, z).wait()


@jax.jit
def pallas_recurrent_scan__mha_block_cached__moe_arch_mod__prompt_kernel(
    A_x: jax.Array,
    A_k_cache: jax.Array,
    A_v_cache: jax.Array,
    A_wq: jax.Array,
    A_wo: jax.Array,
    B_x: jax.Array,
    B_w_r: jax.Array,
    B_w_gate: jax.Array,
    B_w_up: jax.Array,
    B_w_down: jax.Array,
):
    B, S, D = A_x.shape
    _, H, Sk, Dh = A_k_cache.shape
    F = B_w_gate.shape[1]
    assert B == 1 and Sk == S and S % _TQ == 0 and S % _CW == 0 and Dh == 128 and D % 512 == 128
    n = S // _TQ
    assert n % 2 == 0 and 2 <= _P < n - 1 and n == 8 and _P == 4 and H >= 3 and S % 1024 == 0 and S <= 65536
    hbm = pl.BlockSpec(memory_space=pltpu.HBM)
    out = pl.pallas_call(
        functools.partial(_kernel, S=S, D=D, Dh=Dh, H=H),
        grid=(1,),
        in_specs=[hbm, hbm, hbm, hbm, hbm, pl.BlockSpec((1, D), lambda i: (0, 0)), hbm, hbm, hbm],
        out_specs=pl.BlockSpec(memory_space=pl.ANY),
        out_shape=jax.ShapeDtypeStruct((S, D), _BF16),
        scratch_shapes=[
            pltpu.VMEM((S, D), _BF16),
            pltpu.VMEM((S // 2, D), jnp.uint32),
            pltpu.VMEM((S, D), _F32),
            pltpu.VMEM((S, D), _F32),
            pltpu.VMEM((S, D), _BF16),
            pltpu.VMEM((2, _TQ, S), _F32),
            pltpu.VMEM((_TQ, 128), _F32),
            pltpu.VMEM((_TQ, Dh), _F32),
            pltpu.VMEM((_TQ, 128), _F32),
            pltpu.VMEM((_TQ // 2, Dh), jnp.uint32),
            pltpu.VMEM((_NS, S, Dh), _BF16),
            pltpu.VMEM((_NS, S, Dh), _BF16),
            pltpu.VMEM((_NS, D, Dh), _BF16),
            pltpu.VMEM((_NS, Dh, D), _BF16),
            pltpu.VMEM((F, D), _BF16),
            pltpu.VMEM((F, D), _BF16),
            pltpu.VMEM((F, D), _BF16),
            pltpu.SMEM((_TOPC,), _I32),
            pltpu.SMEM((1,), _I32),
            pltpu.SemaphoreType.DMA((4 * _NS + 2 * n + 3,)),
        ],
        compiler_params=pltpu.CompilerParams(
            dimension_semantics=("arbitrary",),
            vmem_limit_bytes=100 * 1024 * 1024,
            disable_bounds_checks=True,
            internal_scratch_in_bytes=64 * 1024,
        ),
    )(A_x.reshape(S, D), A_k_cache.reshape(H, Sk, Dh), A_v_cache.reshape(H, Sk, Dh), A_wq, A_wo,
      B_w_r.reshape(1, D), B_w_gate.T, B_w_up.T, B_w_down)
    return out.reshape(B, S, D)
```

```python
import functools
import math

import jax
import jax.numpy as jnp
import jax.experimental.pallas as pl
import jax.experimental.pallas.tpu as pltpu

_F32 = jnp.float32
_BF16 = jnp.bfloat16
_I32 = jnp.int32
_NT = (((1,), (1,)), ((), ()))

_TOPC = 8
_EPS = 1e-5
_TQ = 256
_CW = 512
_P = 7
_B = 1
_NS = 2 * _B + 1
_INT_MIN = -2 ** 31


def _bf(x):
    return x.astype(_BF16).astype(_F32)


def _silu(x):
    h = 0.5 * x
    return h + h * jnp.tanh(h)


def _sigmoid(x):
    return 0.5 + 0.5 * jnp.tanh(0.5 * x)


def _after(gate, val):
    return jnp.where(gate > jnp.inf, 0.0, val)


def _kernel(x_hbm, k_hbm, v_hbm, wq_hbm, wo_hbm, wr_ref, wg_hbm, wu_hbm, wd_hbm,
            out_hbm,
            x_ref, xnp_ref, z_ref, acc_ref, ob_ref, s_ref, mc_ref, oc_ref, lc_ref,
            kb, vb, wqb, wob, wg_ref, wu_ref, wd_ref, sel_ref, zs,
            sems,
            *, S, D, Dh, H):
    tq, cw, p, B, NS = _TQ, _CW, _P, _B, _NS
    n = S // tq
    R = S // cw
    tb = tq // 4
    D4 = (D // 512) * 512
    F = wd_ref.shape[0]
    scale = (Dh ** -0.5) * math.log2(math.e)
    xn_ref = xnp_ref.bitcast(_BF16)

    def hcol(h):
        return pl.ds(pl.multiple_of(h * Dh, Dh), Dh)

    def cp_k(h, slot):
        return pltpu.make_async_copy(k_hbm.at[h], kb.at[slot], sems.at[0 * NS + slot])

    def cp_wq(h, slot):
        return pltpu.make_async_copy(wq_hbm.at[:, hcol(h)], wqb.at[slot], sems.at[1 * NS + slot])

    def cp_v(h, slot):
        return pltpu.make_async_copy(v_hbm.at[h], vb.at[slot], sems.at[2 * NS + slot])

    def cp_wo(h, slot):
        return pltpu.make_async_copy(wo_hbm.at[hcol(h), :], wob.at[slot], sems.at[3 * NS + slot])

    def cp_head(h, slot):
        return (cp_wq(h, slot), cp_k(h, slot), cp_v(h, slot), cp_wo(h, slot))

    def cp_x(i):
        return pltpu.make_async_copy(x_hbm.at[rs(i * tq, tq), :], x_ref.at[rs(i * tq, tq), :],
                                     sems.at[4 * NS + i])

    def cp_out(i, z):
        src = pl.ds(pl.multiple_of(z * tq + i * tq, tq), tq)
        return pltpu.make_async_copy(ob_ref.at[src, :], out_hbm.at[pl.ds(i * tq, tq), :],
                                     sems.at[4 * NS + n + i])

    def cp_ffn():
        return (pltpu.make_async_copy(wg_hbm, wg_ref, sems.at[4 * NS + 2 * n + 0]),
                pltpu.make_async_copy(wu_hbm, wu_ref, sems.at[4 * NS + 2 * n + 1]),
                pltpu.make_async_copy(wd_hbm, wd_ref, sems.at[4 * NS + 2 * n + 2]))

    def lanes(v, k):
        return jnp.concatenate([v] * k, axis=1)

    def rows(v, k):
        return jnp.concatenate([v] * k, axis=0)

    def rs(r0, nr):
        return slice(r0, r0 + nr) if isinstance(r0, int) else pl.ds(pl.multiple_of(r0, tb), nr)

    def fold(v):
        t = v[:, 0:128]
        for j in range(1, v.shape[1] // 128):
            t = t + v[:, j * 128:(j + 1) * 128]
        return t

    def compact(col, g0, init):
        lane = jax.lax.broadcasted_iota(_I32, init.shape, 1) - g0
        for g in range(col.shape[0] // 8):
            init = jnp.where(lane == g, col[8 * g:8 * g + 8, :], init)
        return init

    def side(jobs, res):
        for k, f in enumerate(jobs or []):
            r0 = (k * res.shape[0] // len(jobs)) // 8 * 8
            f(res[r0:r0 + 8, 0:128])

    def stored(ref, r0, z):
        k = 32 // (8 * ref.dtype.itemsize)
        v = ref[pl.ds(pl.multiple_of(z * 8 * k + r0, 8 * k), 8 * k), 0:128]
        return v if k == 1 else pltpu.bitcast(v, _F32)

    def qproj(i, slot, jobs=None):
        r0 = i * tq
        w = wqb.at[slot]
        q = jnp.dot(xn_ref[rs(r0, tq), 0:D4], w[0:D4, :], preferred_element_type=_F32)
        q = q + jnp.concatenate(
            [jnp.dot(xn_ref[rs(r0 + t * tb, tb), D4:D], w[D4:D, :], preferred_element_type=_F32)
             for t in range(4)], axis=0)
        side(jobs, q)
        return (q * scale).astype(_BF16)

    def qk(par, slot, q, z, jobs=None):
        if jobs is None:
            s = jax.lax.dot_general(q, kb[slot], _NT, preferred_element_type=_F32)
            s_ref[z + par % 2] = s
            return jnp.broadcast_to(jnp.max(s, axis=-1, keepdims=True), (tq, 128))
        mx = None
        for c in range(R):
            s = jax.lax.dot_general(q, kb[slot, c * cw:(c + 1) * cw, :], _NT, preferred_element_type=_F32)
            s_ref[z + par % 2, :, c * cw:(c + 1) * cw] = s
            for j in range(cw // 128):
                sj = s[:, j * 128:(j + 1) * 128]
                mx = sj if mx is None else jnp.maximum(mx, sj)
            side(jobs[c], s)
        return jnp.broadcast_to(jnp.max(mx, axis=-1, keepdims=True), (tq, 128))

    def finalize(r0, nr, c0, c1, s):
        out = x_ref[r0:r0 + nr, c0:c1].astype(_F32) + s * z_ref[r0:r0 + nr, c0:c1]
        ob_ref[r0:r0 + nr, c0:c1] = out.astype(_BF16)

    def wo(i, slot, o, lp, mode, jobs=None):
        l = jnp.sum(lp, axis=-1, keepdims=True)
        o = (o * pl.reciprocal(l, full_range=False)).astype(_BF16)
        r0 = i * tq
        w = wob.at[slot]

        def emit(r0, nr, c0, c1, a):
            if mode == "init":
                acc_ref[rs(r0, nr), c0:c1] = a
            elif mode == "acc":
                acc_ref[r0:r0 + nr, c0:c1] += a
            else:
                finalize(r0, nr, c0, c1, acc_ref[r0:r0 + nr, c0:c1] + a)

        a = jnp.dot(o, w[:, 0:D4], preferred_element_type=_F32)
        emit(r0, tq, 0, D4, a)
        side(jobs, a)
        for t in range(4):
            emit(r0 + t * tb, tb, D4, D,
                 jnp.dot(o[t * tb:(t + 1) * tb, :], w[:, D4:D], preferred_element_type=_F32))
        return a[:, 0:128]

    def pv(par, slot, m, gate, z, jobs=None, before=None, last=False):
        o = lp = None
        for c in range(R):
            mc = m if gate is None else _after(gate, m)
            if before is not None and before[c] is not None:
                mc = _after(rows(before[c](), tq // 8), mc)
            sc = s_ref[z + par % 2, :, c * cw:(c + 1) * cw]
            pe = jnp.exp2(sc - lanes(mc, cw // 128))
            ps = [pe[:, j * 128:(j + 1) * 128] for j in range(cw // 128)]
            for pj in ps:
                lp = pj if lp is None else lp + pj
            ps[-1] = _after(lp, ps[-1])
            pb = jnp.concatenate(ps, axis=1).astype(_BF16)
            oc = jnp.dot(pb, vb[slot, c * cw:(c + 1) * cw, :], preferred_element_type=_F32)
            side(None if jobs is None else jobs[c], oc)
            o = oc if o is None else o + oc
            gate = o
        return o, (lp if last else _after(o, lp))

    def layernorm(r0, nr, rt, z, rel=None):
        def x(k):
            return x_ref[pl.ds(pl.multiple_of(k * z * 16 + r0, 16), nr), :].astype(_F32)
        xs = fold(x(0))
        if rel is not None:
            xs = _after(rows(rel, nr // 8), xs)
        mean = jnp.sum(xs, axis=-1, keepdims=True) * (1.0 / D)
        xc = x(1) - mean
        var = compact(jnp.sum(xc * xc, axis=-1, keepdims=True), 0, jnp.ones((8, 128), _F32)) * (1.0 / D)
        inv = 1.0 / _bf(jnp.sqrt(_bf(_bf(var) + _bf(jnp.float32(_EPS)))))
        inv = jnp.concatenate([jnp.broadcast_to(inv[:, g:g + 1], (8, 128)) for g in range(nr // 8)], axis=0)
        xn = (_bf(x(2) - _bf(mean)) * lanes(inv, D // 128)).astype(_BF16)
        xn_ref[rs(r0, nr), :] = xn
        rp = fold(xn.astype(_F32) * wr_ref[...].astype(_F32))
        rt[0] = compact(jnp.sum(rp, axis=-1, keepdims=True), r0 // 8, rt[0])

    def topk(rt):
        rt = _bf(rt)
        lane = jax.lax.broadcasted_iota(_I32, rt.shape, 1)
        sub = jax.lax.broadcasted_iota(_I32, rt.shape, 0)
        bits = pltpu.bitcast(jnp.where(rt == 0.0, 0.0, rt), _I32)
        mono = jnp.where(bits < 0, bits ^ 0x7FFFFFFF, bits) & -65536
        mono = jnp.where(rt != rt, _INT_MIN, mono)
        key = mono | (65535 - (lane * 8 + sub))
        for c in range(_TOPC):
            kmax = jnp.max(jnp.max(key, axis=0, keepdims=True), axis=1, keepdims=True)
            sel_ref[c] = jnp.clip(65535 - (kmax[0, 0] & 65535), 0, S - 1)
            key = jnp.where(key == kmax, _INT_MIN, key)

    def gate_piece(r0, nr, done, rel):
        h = _after(lanes(rows(rel, nr // 8), D // 128), 0.5 * xn_ref[r0:r0 + nr, :].astype(_F32))
        g = h + h * jnp.tanh(h)
        z_ref[r0:r0 + nr, :] = g
        t = fold(g)
        t = jnp.concatenate([t[k:k + 8] + t[k + 8:k + 16] for k in range(0, nr, 16)], axis=0)
        done[0] = compact(jnp.sum(t, axis=-1, keepdims=True), r0 // 16, done[0])

    def ffn_jobs():
        st = {}
        F4 = (F // cw) * cw

        def gather():
            rowid = jax.lax.broadcasted_iota(_I32, (_TOPC, 1), 0)
            xs = jnp.zeros((_TOPC, D), _F32)
            for c in range(_TOPC):
                w = xnp_ref[pl.ds(sel_ref[c] // 2, 1), :]
                w = jnp.where(sel_ref[c] % 2 == 0, w << 16, w & jnp.uint32(0xFFFF0000))
                xs = jnp.where(rowid == c, pltpu.bitcast(w, _F32), xs)
            st["xs"], st["xb"] = xs, xs.astype(_BF16)

        def add(key, val):
            st[key] = val if key not in st else st[key] + val

        def up(parts, k, rel):
            xk = st["xb"][:, k * 128:(k + 1) * 128]
            for name, w_ref, c0, c1 in parts:
                add((name, c0), jax.lax.dot_general(xk, w_ref[c0:c1, k * 128:(k + 1) * 128], _NT,
                                                    preferred_element_type=_F32))

        def hidden():
            cuts = list(range(0, F, cw))
            g = _bf(jnp.concatenate([st["g", c] for c in cuts], axis=1))
            u = _bf(jnp.concatenate([st["u", c] for c in cuts], axis=1))
            st["h"] = (_bf(_silu(g)) * u).astype(_BF16)

        def down(k0, k1, c0, c1, rel):
            if "h" not in st:
                hidden()
            add(("y", c0), jnp.dot(st["h"][:, k0:k1], wd_ref[k0:k1, c0:c1], preferred_element_type=_F32))

        def scatter(done):
            xs = _after(lanes(done, D // 128), st["xs"])
            rs = _bf(jnp.sum(fold(xs * wr_ref[...].astype(_F32)), axis=-1, keepdims=True))
            y = _bf(jnp.concatenate([st["y", 0], st["y", D4]], axis=1))
            zz = _silu(_bf(xs + _bf(y * _bf(_sigmoid(rs)))))
            for c in range(_TOPC):
                z_ref[pl.ds(sel_ref[c], 1), :] = zz[c:c + 1, :]

        stage1 = []
        for k in range(D // 128):
            for name, w_ref in (("g", wg_ref), ("u", wu_ref)):
                for c0 in range(0, F4, cw):
                    stage1.append(functools.partial(up, [(name, w_ref, c0, c0 + cw)], k))
            stage1.append(functools.partial(up, [("g", wg_ref, F4, F), ("u", wu_ref, F4, F)], k))
        stage2 = [functools.partial(down, k0, min(k0 + 128, F), 0, D4) for k0 in range(0, F, 128)]
        stage2 += [functools.partial(down, k0, min(k0 + cw, F), D4, D) for k0 in range(0, F, cw)]
        return gather, stage1, stage2, scatter

    zs[0] = jnp.minimum(pl.program_id(0), 0)
    first = (cp_x(0), cp_wq(0, 0), cp_k(0, 0), cp_x(1), cp_x(2), cp_v(0, 0), cp_x(3), cp_wo(0, 0))
    first += tuple(cp_x(i) for i in range(4, n))
    for h in range(1, B + 1):
        first += cp_head(h, h)
    for c in first + cp_ffn():
        c.start()
    acc_ref[(p - 1) * tq:, :] = jnp.zeros((S - (p - 1) * tq, D), _F32)
    cp_x(0).wait()
    cp_wq(0, 0).wait()
    z = zs[0]
    rt = [jnp.zeros((8, S // 8), _F32)]

    def first_rounds(us, base, state, z, waits):
        m, o, lp = state
        for u in us:
            jobs = [None] * (R + 1)
            if u + 2 < n:
                pieces = [functools.partial(layernorm, (base + u + 2) * tq + t * tb, tb, rt, z) for t in range(4)]
                jobs = [[pieces.pop(0) for _ in range(k)]
                        for k in ([0, 3, 1, 0, 0] if u in waits else [2, 2, 0, 0, 0])]
            q = qproj(base + u + 1, 0, jobs[0])
            for c in waits.get(u, ()):
                c.wait()
            m_next = qk(u + 1, 0, q, z, jobs[1:] if u + 2 < n else None)
            gate = None if o is None else wo(base + u - 1, 0, o, lp, "init")
            if m is not None:
                o, lp = pv(u, 0, m, gate, z, last=(u == us[-1]))
            m = m_next
        mc_ref[...], oc_ref[...], lc_ref[...] = m, o, lp

    for t in range(4):
        layernorm(t * tb, tb, rt, z)
    first_rounds([-1, 0, 1], 0, (None, None, None), z,
                 {-1: (cp_k(0, 0), cp_x(1)), 0: (cp_x(2), cp_v(0, 0)), 1: (cp_x(3), cp_wo(0, 0))})

    def pair(j, rt_in):
        for k in range(2):
            cp_x(4 + 2 * j + k).wait()
        rt[0] = rt_in
        first_rounds([0, 1], 2 + 2 * j, (mc_ref[...], oc_ref[...], lc_ref[...]), zs[0], {})
        return rt[0]

    rt[0] = jax.lax.fori_loop(0, 2, pair, rt[0])
    first_rounds([p - 1], 0, (mc_ref[...], oc_ref[...], lc_ref[...]), zs[0], {})
    topk(rt[0])
    for h in range(1, B + 1):
        for c in cp_head(h, h):
            c.wait()

    def body(j, slots):
        z = zs[0]
        slot = lambda u: slots[u // n]
        m, o, lp = mc_ref[...], oc_ref[...], lc_ref[...]
        for u in range(p, p + B * n):
            m_next = qk((u + 1) % n, slot(u + 1), qproj((u + 1) % n, slot(u + 1)), z)
            gate = wo((u - 1) % n, slot(u - 1), o, lp, "acc")
            if u == p + 1:
                for b in range(B):
                    for c in cp_head(jnp.minimum(B * j + B + 1 + b, H - 1), slots[B + 1 + b]):
                        c.start()
            o, lp = pv(u % n, slot(u), m, gate, z, last=(u == p + B * n - 1))
            m = m_next
        mc_ref[...], oc_ref[...], lc_ref[...] = m, o, lp
        for b in range(B):
            for c in cp_head(0, slots[B + 1 + b]):
                c.wait()
        return slots[B:] + slots[:B]

    jax.lax.fori_loop(0, (H - 2) // B, body, tuple(jnp.int32(k) for k in range(NS)))

    z = zs[0]
    slot = lambda u: (H - 2 + u // n) % NS
    for c in cp_ffn():
        c.wait()
    m, o, lp = mc_ref[...], oc_ref[...], lc_ref[...]
    gather, stage1, stage2, scatter = ffn_jobs()
    gather()
    done = [jnp.zeros((8, 128), _F32)]
    gates = [functools.partial(gate_piece, r0, tb, done) for r0 in range(0, S, tb)]
    fq = stage1 + stage2
    plan_gate = {p: [3, 3, 3, 3, 0], p + 1: [3, 3, 3, 3, 0], p + 2: [4, 4, 0, 0, 0]}
    plan_ffn = {p: [2, 2, 2, 2, 2, 2, 3, 3, 3, 2], p + 1: [2, 2, 2, 2, 2, 2, 0, 3, 3, 3],
                p + 2: [3, 2, 2, 2, 0, 0, 0, 0, 0, 0]}
    assert sum(plan_ffn[p]) + sum(plan_ffn[p + 1][:6]) == len(stage1)

    for u in range(p, 2 * n):
        def jobs(k):
            ng, nf = (plan_gate.get(u, []) + [0] * 10)[k], plan_ffn.get(u, [0] * 10)[k]
            return [gates.pop(0) for _ in range(ng)] + [fq.pop(0) for _ in range(nf)]
        m_next = None
        if u + 1 < 2 * n:
            q = qproj((u + 1) % n, slot(u + 1), jobs(0))
            m_next = qk((u + 1) % n, slot(u + 1), q, z, [jobs(1 + c) for c in range(R)] if u in plan_ffn else None)
        if u == p + 2:
            assert not fq and not gates
            scatter(done[0])
        i = u - 1 - n
        gate = wo((u - 1) % n, slot(u - 1), o, lp, "final" if i >= 0 else "acc", jobs(5))
        before = [None] * R
        if i >= 0:
            cp_out(i, z).start()
            before[2] = functools.partial(stored, ob_ref, i * tq, z)
        o, lp = pv(u % n, slot(u), m, gate, z, [jobs(6 + c) for c in range(R)], before)
        m = m_next
    wo(n - 1, slot(2 * n - 1), o, lp, "final")
    cp_out(n - 1, z).start()
    for i in range(n):
        cp_out(i, z).wait()


@jax.jit
def pallas_recurrent_scan__mha_block_cached__moe_arch_mod__prompt_kernel(
    A_x: jax.Array,
    A_k_cache: jax.Array,
    A_v_cache: jax.Array,
    A_wq: jax.Array,
    A_wo: jax.Array,
    B_x: jax.Array,
    B_w_r: jax.Array,
    B_w_gate: jax.Array,
    B_w_up: jax.Array,
    B_w_down: jax.Array,
):
    B, S, D = A_x.shape
    _, H, Sk, Dh = A_k_cache.shape
    F = B_w_gate.shape[1]
    assert B == 1 and Sk == S and S % _TQ == 0 and S % _CW == 0 and Dh == 128 and D % 512 == 128
    n = S // _TQ
    assert n == 8 and _P == n - 1 and (H - 2) % _B == 0 and H >= 2 + _B and S % 1024 == 0
    hbm = pl.BlockSpec(memory_space=pltpu.HBM)
    out = pl.pallas_call(
        functools.partial(_kernel, S=S, D=D, Dh=Dh, H=H),
        grid=(1,),
        in_specs=[hbm, hbm, hbm, hbm, hbm, pl.BlockSpec((1, D), lambda i: (0, 0)), hbm, hbm, hbm],
        out_specs=pl.BlockSpec(memory_space=pl.ANY),
        out_shape=jax.ShapeDtypeStruct((S, D), _BF16),
        scratch_shapes=[
            pltpu.VMEM((S, D), _BF16),
            pltpu.VMEM((S // 2, D), jnp.uint32),
            pltpu.VMEM((S, D), _F32),
            pltpu.VMEM((S, D), _F32),
            pltpu.VMEM((S, D), _BF16),
            pltpu.VMEM((2, _TQ, S), _F32),
            pltpu.VMEM((_TQ, 128), _F32),
            pltpu.VMEM((_TQ, Dh), _F32),
            pltpu.VMEM((_TQ, 128), _F32),
            pltpu.VMEM((_NS, S, Dh), _BF16),
            pltpu.VMEM((_NS, S, Dh), _BF16),
            pltpu.VMEM((_NS, D, Dh), _BF16),
            pltpu.VMEM((_NS, Dh, D), _BF16),
            pltpu.VMEM((F, D), _BF16),
            pltpu.VMEM((F, D), _BF16),
            pltpu.VMEM((F, D), _BF16),
            pltpu.SMEM((_TOPC,), _I32),
            pltpu.SMEM((1,), _I32),
            pltpu.SemaphoreType.DMA((4 * _NS + 2 * n + 3,)),
        ],
        compiler_params=pltpu.CompilerParams(
            dimension_semantics=("arbitrary",),
            vmem_limit_bytes=100 * 1024 * 1024,
            disable_bounds_checks=True,
            internal_scratch_in_bytes=64 * 1024,
        ),
    )(A_x.reshape(S, D), A_k_cache.reshape(H, Sk, Dh), A_v_cache.reshape(H, Sk, Dh), A_wq, A_wo,
      B_w_r.reshape(1, D), B_w_gate.T, B_w_up.T, B_w_down)
    return out.reshape(B, S, D)
```

```python
import functools
import math

import jax
import jax.numpy as jnp
import jax.experimental.pallas as pl
import jax.experimental.pallas.tpu as pltpu

_F32 = jnp.float32
_BF16 = jnp.bfloat16
_I32 = jnp.int32
_NT = (((1,), (1,)), ((), ()))

_TOPC = 8
_EPS = 1e-5
_TQ = 256
_CW = 512
_P = 7
_B = 1
_NS = 2 * _B + 1
_INT_MIN = -2 ** 31


def _bf(x):
    return x.astype(_BF16).astype(_F32)


def _silu(x):
    h = 0.5 * x
    return h + h * jnp.tanh(h)


def _sigmoid(x):
    return 0.5 + 0.5 * jnp.tanh(0.5 * x)


def _after(gate, val):
    return jnp.where(gate > jnp.inf, 0.0, val)


def _kernel(x_hbm, k_hbm, v_hbm, wq_hbm, wo_hbm, wr_hbm, wg_hbm, wu_hbm, wd_hbm,
            out_hbm,
            x_ref, xnp_ref, z_ref, acc_ref, ob_ref, s_ref, mc_ref, oc_ref, lc_ref,
            kb, vb, wqb, wob, wg_ref, wu_ref, wd_ref, wr_ref, sel_ref, zs,
            sems,
            *, S, D, Dh, H):
    tq, cw, p, B, NS = _TQ, _CW, _P, _B, _NS
    n = S // tq
    R = S // cw
    tb = tq // 4
    D4 = (D // 512) * 512
    F = wd_ref.shape[0]
    scale = (Dh ** -0.5) * math.log2(math.e)
    xn_ref = xnp_ref.bitcast(_BF16)

    def hcol(h):
        return pl.ds(pl.multiple_of(h * Dh, Dh), Dh)

    def cp_k(h, slot):
        return pltpu.make_async_copy(k_hbm.at[h], kb.at[slot], sems.at[0 * NS + slot])

    def cp_wq(h, slot):
        return pltpu.make_async_copy(wq_hbm.at[:, hcol(h)], wqb.at[slot], sems.at[1 * NS + slot])

    def cp_v(h, slot):
        return pltpu.make_async_copy(v_hbm.at[h], vb.at[slot], sems.at[2 * NS + slot])

    def cp_wo(h, slot):
        return pltpu.make_async_copy(wo_hbm.at[hcol(h), :], wob.at[slot], sems.at[3 * NS + slot])

    def cp_head(h, slot):
        return (cp_wq(h, slot), cp_k(h, slot), cp_v(h, slot), cp_wo(h, slot))

    def cp_x(i):
        return pltpu.make_async_copy(x_hbm.at[rs(i * tq, tq), :], x_ref.at[rs(i * tq, tq), :],
                                     sems.at[4 * NS + i])

    def cp_out(i, z):
        src = pl.ds(pl.multiple_of(z * tq + i * tq, tq), tq)
        return pltpu.make_async_copy(ob_ref.at[src, :], out_hbm.at[pl.ds(i * tq, tq), :],
                                     sems.at[4 * NS + n + i])

    def cp_ffn():
        return (pltpu.make_async_copy(wg_hbm, wg_ref, sems.at[4 * NS + 2 * n + 0]),
                pltpu.make_async_copy(wu_hbm, wu_ref, sems.at[4 * NS + 2 * n + 1]),
                pltpu.make_async_copy(wd_hbm, wd_ref, sems.at[4 * NS + 2 * n + 2]))

    def cp_wr():
        return pltpu.make_async_copy(wr_hbm, wr_ref, sems.at[4 * NS + 2 * n + 3])

    def lanes(v, k):
        return jnp.concatenate([v] * k, axis=1)

    def rows(v, k):
        return jnp.concatenate([v] * k, axis=0)

    def rs(r0, nr):
        return slice(r0, r0 + nr) if isinstance(r0, int) else pl.ds(pl.multiple_of(r0, tb), nr)

    def fold(v):
        t = v[:, 0:128]
        for j in range(1, v.shape[1] // 128):
            t = t + v[:, j * 128:(j + 1) * 128]
        return t

    def compact(col, g0, init):
        lane = jax.lax.broadcasted_iota(_I32, init.shape, 1) - g0
        for g in range(col.shape[0] // 8):
            init = jnp.where(lane == g, col[8 * g:8 * g + 8, :], init)
        return init

    def side(jobs, res):
        for k, f in enumerate(jobs or []):
            r0 = (k * res.shape[0] // len(jobs)) // 8 * 8
            f(res[r0:r0 + 8, 0:128])

    def stored(ref, r0, z):
        k = 32 // (8 * ref.dtype.itemsize)
        v = ref[pl.ds(pl.multiple_of(z * 8 * k + r0, 8 * k), 8 * k), 0:128]
        return v if k == 1 else pltpu.bitcast(v, _F32)

    def qproj(i, slot, jobs=None):
        r0 = i * tq
        w = wqb.at[slot]
        q = jnp.dot(xn_ref[rs(r0, tq), 0:D4], w[0:D4, :], preferred_element_type=_F32)
        q = q + jnp.concatenate(
            [jnp.dot(xn_ref[rs(r0 + t * tb, tb), D4:D], w[D4:D, :], preferred_element_type=_F32)
             for t in range(4)], axis=0)
        side(jobs, q)
        return (q * scale).astype(_BF16)

    def qk(par, slot, q, z, jobs=None):
        if jobs is None:
            s = jax.lax.dot_general(q, kb[slot], _NT, preferred_element_type=_F32)
            s_ref[z + par % 2] = s
            return jnp.broadcast_to(jnp.max(s, axis=-1, keepdims=True), (tq, 128))
        mx = None
        for c in range(R):
            s = jax.lax.dot_general(q, kb[slot, c * cw:(c + 1) * cw, :], _NT, preferred_element_type=_F32)
            s_ref[z + par % 2, :, c * cw:(c + 1) * cw] = s
            for j in range(cw // 128):
                sj = s[:, j * 128:(j + 1) * 128]
                mx = sj if mx is None else jnp.maximum(mx, sj)
            side(jobs[c], s)
        return jnp.broadcast_to(jnp.max(mx, axis=-1, keepdims=True), (tq, 128))

    def finalize(r0, nr, c0, c1, s):
        out = x_ref[r0:r0 + nr, c0:c1].astype(_F32) + s * z_ref[r0:r0 + nr, c0:c1]
        ob_ref[r0:r0 + nr, c0:c1] = out.astype(_BF16)

    def wo(i, slot, o, lp, mode, jobs=None):
        l = jnp.sum(lp, axis=-1, keepdims=True)
        o = (o * pl.reciprocal(l, full_range=False)).astype(_BF16)
        r0 = i * tq
        w = wob.at[slot]

        def emit(r0, nr, c0, c1, a):
            if mode == "init":
                acc_ref[rs(r0, nr), c0:c1] = a
            elif mode == "acc":
                acc_ref[r0:r0 + nr, c0:c1] += a
            else:
                finalize(r0, nr, c0, c1, acc_ref[r0:r0 + nr, c0:c1] + a)

        a = jnp.dot(o, w[:, 0:D4], preferred_element_type=_F32)
        emit(r0, tq, 0, D4, a)
        side(jobs, a)
        for t in range(4):
            emit(r0 + t * tb, tb, D4, D,
                 jnp.dot(o[t * tb:(t + 1) * tb, :], w[:, D4:D], preferred_element_type=_F32))
        return a[:, 0:128]

    def pv(par, slot, m, gate, z, jobs=None, before=None, last=False):
        o = lp = None
        for c in range(R):
            mc = m if gate is None else _after(gate, m)
            if before is not None and before[c] is not None:
                mc = _after(rows(before[c](), tq // 8), mc)
            sc = s_ref[z + par % 2, :, c * cw:(c + 1) * cw]
            pe = jnp.exp2(sc - lanes(mc, cw // 128))
            ps = [pe[:, j * 128:(j + 1) * 128] for j in range(cw // 128)]
            for pj in ps:
                lp = pj if lp is None else lp + pj
            ps[-1] = _after(lp, ps[-1])
            pb = jnp.concatenate(ps, axis=1).astype(_BF16)
            oc = jnp.dot(pb, vb[slot, c * cw:(c + 1) * cw, :], preferred_element_type=_F32)
            side(None if jobs is None else jobs[c], oc)
            o = oc if o is None else o + oc
            gate = o
        return o, (lp if last else _after(o, lp))

    def layernorm(r0, nr, rt, z, rel=None):
        def x(k):
            return x_ref[pl.ds(pl.multiple_of(k * z * 16 + r0, 16), nr), :].astype(_F32)
        xs = fold(x(0))
        if rel is not None:
            xs = _after(rows(rel, nr // 8), xs)
        mean = jnp.sum(xs, axis=-1, keepdims=True) * (1.0 / D)
        xc = x(1) - mean
        var = compact(jnp.sum(xc * xc, axis=-1, keepdims=True), 0, jnp.ones((8, 128), _F32)) * (1.0 / D)
        inv = 1.0 / _bf(jnp.sqrt(_bf(_bf(var) + _bf(jnp.float32(_EPS)))))
        inv = jnp.concatenate([jnp.broadcast_to(inv[:, g:g + 1], (8, 128)) for g in range(nr // 8)], axis=0)
        xn = (_bf(x(2) - _bf(mean)) * lanes(inv, D // 128)).astype(_BF16)
        xn_ref[rs(r0, nr), :] = xn
        rp = fold(xn.astype(_F32) * wr_ref[...].astype(_F32).reshape(1, D))
        rt[0] = compact(jnp.sum(rp, axis=-1, keepdims=True), r0 // 8, rt[0])

    def topk(rt):
        rt = _bf(rt)
        lane = jax.lax.broadcasted_iota(_I32, rt.shape, 1)
        sub = jax.lax.broadcasted_iota(_I32, rt.shape, 0)
        bits = pltpu.bitcast(jnp.where(rt == 0.0, 0.0, rt), _I32)
        mono = jnp.where(bits < 0, bits ^ 0x7FFFFFFF, bits) & -65536
        mono = jnp.where(rt != rt, _INT_MIN, mono)
        key = mono | (65535 - (lane * 8 + sub))
        for c in range(_TOPC):
            kmax = jnp.max(jnp.max(key, axis=0, keepdims=True), axis=1, keepdims=True)
            sel_ref[c] = jnp.clip(65535 - (kmax[0, 0] & 65535), 0, S - 1)
            key = jnp.where(key == kmax, _INT_MIN, key)

    def gate_piece(r0, nr, done, rel):
        h = _after(lanes(rows(rel, nr // 8), D // 128), 0.5 * xn_ref[r0:r0 + nr, :].astype(_F32))
        g = h + h * jnp.tanh(h)
        z_ref[r0:r0 + nr, :] = g
        t = fold(g)
        t = jnp.concatenate([t[k:k + 8] + t[k + 8:k + 16] for k in range(0, nr, 16)], axis=0)
        done[0] = compact(jnp.sum(t, axis=-1, keepdims=True), r0 // 16, done[0])

    def ffn_jobs():
        st = {}
        F4 = (F // cw) * cw

        def gather():
            rowid = jax.lax.broadcasted_iota(_I32, (_TOPC, 1), 0)
            xs = jnp.zeros((_TOPC, D), _F32)
            for c in range(_TOPC):
                w = xnp_ref[pl.ds(sel_ref[c] // 2, 1), :]
                w = jnp.where(sel_ref[c] % 2 == 0, w << 16, w & jnp.uint32(0xFFFF0000))
                xs = jnp.where(rowid == c, pltpu.bitcast(w, _F32), xs)
            st["xs"], st["xb"] = xs, xs.astype(_BF16)

        def add(key, val):
            st[key] = val if key not in st else st[key] + val

        def up(parts, k, rel):
            xk = st["xb"][:, k * 128:(k + 1) * 128]
            for name, w_ref, c0, c1 in parts:
                add((name, c0), jax.lax.dot_general(xk, w_ref[c0:c1, k * 128:(k + 1) * 128], _NT,
                                                    preferred_element_type=_F32))

        def hidden():
            cuts = list(range(0, F, cw))
            g = _bf(jnp.concatenate([st["g", c] for c in cuts], axis=1))
            u = _bf(jnp.concatenate([st["u", c] for c in cuts], axis=1))
            st["h"] = (_bf(_silu(g)) * u).astype(_BF16)

        def down(k0, k1, c0, c1, rel):
            if "h" not in st:
                hidden()
            add(("y", c0), jnp.dot(st["h"][:, k0:k1], wd_ref[k0:k1, c0:c1], preferred_element_type=_F32))

        def scatter(done):
            xs = _after(lanes(done, D // 128), st["xs"])
            rs = _bf(jnp.sum(fold(xs * wr_ref[...].astype(_F32).reshape(1, D)), axis=-1, keepdims=True))
            y = _bf(jnp.concatenate([st["y", 0], st["y", D4]], axis=1))
            zz = _silu(_bf(xs + _bf(y * _bf(_sigmoid(rs)))))
            for c in range(_TOPC):
                z_ref[pl.ds(sel_ref[c], 1), :] = zz[c:c + 1, :]

        stage1 = []
        for k in range(D // 128):
            for name, w_ref in (("g", wg_ref), ("u", wu_ref)):
                for c0 in range(0, F4, cw):
                    stage1.append(functools.partial(up, [(name, w_ref, c0, c0 + cw)], k))
            stage1.append(functools.partial(up, [("g", wg_ref, F4, F), ("u", wu_ref, F4, F)], k))
        stage2 = [functools.partial(down, k0, min(k0 + 128, F), 0, D4) for k0 in range(0, F, 128)]
        stage2 += [functools.partial(down, k0, min(k0 + cw, F), D4, D) for k0 in range(0, F, cw)]
        return gather, stage1, stage2, scatter

    zs[0] = jnp.minimum(pl.program_id(0), 0)
    first = (cp_x(0), cp_wr(), cp_wq(0, 0), cp_x(1), cp_k(0, 0), cp_x(2), cp_v(0, 0), cp_x(3), cp_wo(0, 0))
    first += tuple(cp_x(i) for i in range(4, n))
    for h in range(1, B + 1):
        first += cp_head(h, h)
    for c in first + cp_ffn():
        c.start()
    acc_ref[(p - 1) * tq:, :] = jnp.zeros((S - (p - 1) * tq, D), _F32)
    cp_x(0).wait()
    cp_wr().wait()
    z = zs[0]
    rt = [jnp.zeros((8, S // 8), _F32)]

    def ln_jobs(i, z, spread):
        pieces = [functools.partial(layernorm, i * tq + t * tb, tb, rt, z) for t in range(4)]
        return [[pieces.pop(0) for _ in range(k)] for k in spread]

    def first_rounds(us, base, state, z):
        m, o, lp = state
        for u in us:
            jobs = ln_jobs(base + u + 2, z, [2, 2, 0, 0, 0]) if u + 2 < n else [None, None]
            q = qproj(base + u + 1, 0, jobs[0])
            m_next = qk(u + 1, 0, q, z, jobs[1:] if u + 2 < n else None)
            gate = wo(base + u - 1, 0, o, lp, "init")
            o, lp = pv(u, 0, m, gate, z, last=(u == us[-1]))
            m = m_next
        mc_ref[...], oc_ref[...], lc_ref[...] = m, o, lp

    for f in ln_jobs(0, z, [4])[0]:
        f()
    cp_wq(0, 0).wait()
    cp_x(1).wait()
    q0 = qproj(0, 0)
    for f in ln_jobs(1, z, [4])[0]:
        f()
    q1 = qproj(1, 0)
    cp_k(0, 0).wait()
    m0 = qk(0, 0, q0, z)
    cp_x(2).wait()
    m1 = qk(1, 0, q1, z, ln_jobs(2, z, [3, 1, 0, 0]))
    for c in (cp_v(0, 0), cp_x(3), cp_wo(0, 0)):
        c.wait()
    first_rounds([1], 0, (m1,) + pv(0, 0, m0, None, z), z)

    def pair(j, rt_in):
        for k in range(2):
            cp_x(4 + 2 * j + k).wait()
        rt[0] = rt_in
        first_rounds([0, 1], 2 + 2 * j, (mc_ref[...], oc_ref[...], lc_ref[...]), zs[0])
        return rt[0]

    rt[0] = jax.lax.fori_loop(0, 2, pair, rt[0])
    first_rounds([p - 1], 0, (mc_ref[...], oc_ref[...], lc_ref[...]), zs[0])
    topk(rt[0])
    for h in range(1, B + 1):
        for c in cp_head(h, h):
            c.wait()

    def body(j, slots):
        z = zs[0]
        slot = lambda u: slots[u // n]
        m, o, lp = mc_ref[...], oc_ref[...], lc_ref[...]
        for u in range(p, p + B * n):
            m_next = qk((u + 1) % n, slot(u + 1), qproj((u + 1) % n, slot(u + 1)), z)
            gate = wo((u - 1) % n, slot(u - 1), o, lp, "acc")
            if u == p + 1:
                for b in range(B):
                    for c in cp_head(jnp.minimum(B * j + B + 1 + b, H - 1), slots[B + 1 + b]):
                        c.start()
            o, lp = pv(u % n, slot(u), m, gate, z, last=(u == p + B * n - 1))
            m = m_next
        mc_ref[...], oc_ref[...], lc_ref[...] = m, o, lp
        for b in range(B):
            for c in cp_head(0, slots[B + 1 + b]):
                c.wait()
        return slots[B:] + slots[:B]

    jax.lax.fori_loop(0, (H - 2) // B, body, tuple(jnp.int32(k) for k in range(NS)))

    z = zs[0]
    slot = lambda u: (H - 2 + u // n) % NS
    for c in cp_ffn():
        c.wait()
    m, o, lp = mc_ref[...], oc_ref[...], lc_ref[...]
    gather, stage1, stage2, scatter = ffn_jobs()
    gather()
    done = [jnp.zeros((8, 128), _F32)]
    gates = [functools.partial(gate_piece, r0, tb, done) for r0 in range(0, S, tb)]
    fq = stage1 + stage2
    plan_gate = {p: [3, 3, 3, 3, 0], p + 1: [3, 3, 3, 3, 0], p + 2: [4, 4, 0, 0, 0]}
    plan_ffn = {p: [2, 2, 2, 2, 2, 2, 3, 3, 3, 2], p + 1: [2, 2, 2, 2, 2, 2, 0, 3, 3, 3],
                p + 2: [3, 2, 2, 2, 0, 0, 0, 0, 0, 0]}
    assert sum(plan_ffn[p]) + sum(plan_ffn[p + 1][:6]) == len(stage1)

    for u in range(p, 2 * n):
        def jobs(k):
            ng, nf = (plan_gate.get(u, []) + [0] * 10)[k], plan_ffn.get(u, [0] * 10)[k]
            return [gates.pop(0) for _ in range(ng)] + [fq.pop(0) for _ in range(nf)]
        m_next = None
        if u + 1 < 2 * n:
            q = qproj((u + 1) % n, slot(u + 1), jobs(0))
            m_next = qk((u + 1) % n, slot(u + 1), q, z, [jobs(1 + c) for c in range(R)] if u in plan_ffn else None)
        if u == p + 2:
            assert not fq and not gates
            scatter(done[0])
        i = u - 1 - n
        gate = wo((u - 1) % n, slot(u - 1), o, lp, "final" if i >= 0 else "acc", jobs(5))
        before = [None] * R
        if i >= 0:
            cp_out(i, z).start()
            before[2] = functools.partial(stored, ob_ref, i * tq, z)
        o, lp = pv(u % n, slot(u), m, gate, z, [jobs(6 + c) for c in range(R)], before)
        m = m_next
    wo(n - 1, slot(2 * n - 1), o, lp, "final")
    cp_out(n - 1, z).start()
    for i in range(n):
        cp_out(i, z).wait()


@jax.jit
def pallas_recurrent_scan__mha_block_cached__moe_arch_mod__prompt_kernel(
    A_x: jax.Array,
    A_k_cache: jax.Array,
    A_v_cache: jax.Array,
    A_wq: jax.Array,
    A_wo: jax.Array,
    B_x: jax.Array,
    B_w_r: jax.Array,
    B_w_gate: jax.Array,
    B_w_up: jax.Array,
    B_w_down: jax.Array,
):
    B, S, D = A_x.shape
    _, H, Sk, Dh = A_k_cache.shape
    F = B_w_gate.shape[1]
    assert B == 1 and Sk == S and S % _TQ == 0 and S % _CW == 0 and Dh == 128 and D % 512 == 128
    n = S // _TQ
    assert n == 8 and _P == n - 1 and (H - 2) % _B == 0 and H >= 2 + _B and S % 1024 == 0
    hbm = pl.BlockSpec(memory_space=pltpu.HBM)
    out = pl.pallas_call(
        functools.partial(_kernel, S=S, D=D, Dh=Dh, H=H),
        grid=(1,),
        in_specs=[hbm] * 9,
        out_specs=pl.BlockSpec(memory_space=pl.ANY),
        out_shape=jax.ShapeDtypeStruct((S, D), _BF16),
        scratch_shapes=[
            pltpu.VMEM((S, D), _BF16),
            pltpu.VMEM((S // 2, D), jnp.uint32),
            pltpu.VMEM((S, D), _F32),
            pltpu.VMEM((S, D), _F32),
            pltpu.VMEM((S, D), _BF16),
            pltpu.VMEM((2, _TQ, S), _F32),
            pltpu.VMEM((_TQ, 128), _F32),
            pltpu.VMEM((_TQ, Dh), _F32),
            pltpu.VMEM((_TQ, 128), _F32),
            pltpu.VMEM((_NS, S, Dh), _BF16),
            pltpu.VMEM((_NS, S, Dh), _BF16),
            pltpu.VMEM((_NS, D, Dh), _BF16),
            pltpu.VMEM((_NS, Dh, D), _BF16),
            pltpu.VMEM((F, D), _BF16),
            pltpu.VMEM((F, D), _BF16),
            pltpu.VMEM((F, D), _BF16),
            pltpu.VMEM((D,), _BF16),
            pltpu.SMEM((_TOPC,), _I32),
            pltpu.SMEM((1,), _I32),
            pltpu.SemaphoreType.DMA((4 * _NS + 2 * n + 4,)),
        ],
        compiler_params=pltpu.CompilerParams(
            dimension_semantics=("arbitrary",),
            vmem_limit_bytes=100 * 1024 * 1024,
            disable_bounds_checks=True,
            internal_scratch_in_bytes=64 * 1024,
        ),
    )(A_x.reshape(S, D), A_k_cache.reshape(H, Sk, Dh), A_v_cache.reshape(H, Sk, Dh), A_wq, A_wo,
      B_w_r, B_w_gate.T, B_w_up.T, B_w_down)
    return out.reshape(B, S, D)
```

```python
import functools
import math

import jax
import jax.numpy as jnp
import jax.experimental.pallas as pl
import jax.experimental.pallas.tpu as pltpu

_F32 = jnp.float32
_BF16 = jnp.bfloat16
_I32 = jnp.int32
_NT = (((1,), (1,)), ((), ()))

_TOPC = 8
_EPS = 1e-5
_TQ = 256
_CW = 512
_P = 7
_B = 1
_NS = 2 * _B + 1
_INT_MIN = -2 ** 31


def _bf(x):
    return x.astype(_BF16).astype(_F32)


def _silu(x):
    h = 0.5 * x
    return h + h * jnp.tanh(h)


def _sigmoid(x):
    return 0.5 + 0.5 * jnp.tanh(0.5 * x)


def _after(gate, val):
    return jnp.where(gate > jnp.inf, 0.0, val)


def _kernel(x_hbm, k_hbm, v_hbm, wq_hbm, wo_hbm, wr_hbm, wg_hbm, wu_hbm, wd_hbm,
            out_hbm,
            x_ref, xnp_ref, z_ref, acc_ref, ob_ref, s_ref, mc_ref, oc_ref, lc_ref,
            kb, vb, wqb, wob, wg_ref, wu_ref, wd_ref, wr_ref, sel_ref, zs,
            sems,
            *, S, D, Dh, H):
    tq, cw, p, B, NS = _TQ, _CW, _P, _B, _NS
    n = S // tq
    R = S // cw
    tb = tq // 4
    D4 = (D // 512) * 512
    F = wd_ref.shape[0]
    scale = (Dh ** -0.5) * math.log2(math.e)
    xn_ref = xnp_ref.bitcast(_BF16)

    def hcol(h):
        return pl.ds(pl.multiple_of(h * Dh, Dh), Dh)

    def cp_k(h, slot):
        return pltpu.make_async_copy(k_hbm.at[h], kb.at[slot], sems.at[0 * NS + slot])

    def cp_wq(h, slot):
        return pltpu.make_async_copy(wq_hbm.at[:, hcol(h)], wqb.at[slot], sems.at[1 * NS + slot])

    def cp_v(h, slot):
        return pltpu.make_async_copy(v_hbm.at[h], vb.at[slot], sems.at[2 * NS + slot])

    def cp_wo(h, slot):
        return pltpu.make_async_copy(wo_hbm.at[hcol(h), :], wob.at[slot], sems.at[3 * NS + slot])

    def cp_head(h, slot):
        return (cp_wq(h, slot), cp_k(h, slot), cp_v(h, slot), cp_wo(h, slot))

    def cp_x(i):
        return pltpu.make_async_copy(x_hbm.at[rs(i * tq, tq), :], x_ref.at[rs(i * tq, tq), :],
                                     sems.at[4 * NS + i])

    def cp_out(i, z):
        src = pl.ds(pl.multiple_of(z * tq + i * tq, tq), tq)
        return pltpu.make_async_copy(ob_ref.at[src, :], out_hbm.at[pl.ds(i * tq, tq), :],
                                     sems.at[4 * NS + n + i])

    def cp_ffn():
        return (pltpu.make_async_copy(wg_hbm, wg_ref, sems.at[4 * NS + 2 * n + 0]),
                pltpu.make_async_copy(wu_hbm, wu_ref, sems.at[4 * NS + 2 * n + 1]),
                pltpu.make_async_copy(wd_hbm, wd_ref, sems.at[4 * NS + 2 * n + 2]))

    def cp_wr():
        return pltpu.make_async_copy(wr_hbm, wr_ref, sems.at[4 * NS + 2 * n + 3])

    def lanes(v, k):
        return jnp.concatenate([v] * k, axis=1)

    def rows(v, k):
        return jnp.concatenate([v] * k, axis=0)

    def rs(r0, nr):
        return slice(r0, r0 + nr) if isinstance(r0, int) else pl.ds(pl.multiple_of(r0, tb), nr)

    def fold(v):
        t = v[:, 0:128]
        for j in range(1, v.shape[1] // 128):
            t = t + v[:, j * 128:(j + 1) * 128]
        return t

    def compact(col, g0, init):
        lane = jax.lax.broadcasted_iota(_I32, init.shape, 1) - g0
        for g in range(col.shape[0] // 8):
            init = jnp.where(lane == g, col[8 * g:8 * g + 8, :], init)
        return init

    def side(jobs, res):
        for k, f in enumerate(jobs or []):
            r0 = min(k * res.shape[0] // len(jobs) // 8 * 8, res.shape[0] - tb)
            f(res[r0:r0 + tb, 0:128])

    def stored(ref, r0, z):
        k = 32 // (8 * ref.dtype.itemsize)
        v = ref[pl.ds(pl.multiple_of(z * 8 * k + r0, 8 * k), 8 * k), 0:128]
        return v if k == 1 else pltpu.bitcast(v, _F32)

    def qproj(i, slot, jobs=None):
        r0 = i * tq
        w = wqb.at[slot]
        q = jnp.dot(xn_ref[rs(r0, tq), 0:D4], w[0:D4, :], preferred_element_type=_F32)
        q = q + jnp.concatenate(
            [jnp.dot(xn_ref[rs(r0 + t * tb, tb), D4:D], w[D4:D, :], preferred_element_type=_F32)
             for t in range(4)], axis=0)
        side(jobs, q)
        return (q * scale).astype(_BF16)

    def rowmax(mx):
        return jnp.broadcast_to(jnp.max(mx, axis=-1, keepdims=True), (tq, 128))

    def qk(par, slot, q, z, jobs=None, lanewise=False):
        if jobs is None:
            s = jax.lax.dot_general(q, kb[slot], _NT, preferred_element_type=_F32)
            s_ref[z + par % 2] = s
            return rowmax(s)
        mx = None
        for c in range(R):
            s = jax.lax.dot_general(q, kb[slot, c * cw:(c + 1) * cw, :], _NT, preferred_element_type=_F32)
            s_ref[z + par % 2, :, c * cw:(c + 1) * cw] = s
            for j in range(cw // 128):
                sj = s[:, j * 128:(j + 1) * 128]
                mx = sj if mx is None else jnp.maximum(mx, sj)
            side(jobs[c], s)
        return mx if lanewise else rowmax(mx)

    def finalize(r0, nr, c0, c1, s):
        out = x_ref[r0:r0 + nr, c0:c1].astype(_F32) + s * z_ref[r0:r0 + nr, c0:c1]
        ob_ref[r0:r0 + nr, c0:c1] = out.astype(_BF16)
        return out

    def wo(i, slot, o, lp, mode, jobs=None):
        l = jnp.sum(lp, axis=-1, keepdims=True)
        o = (o * pl.reciprocal(l, full_range=False)).astype(_BF16)
        r0 = i * tq
        w = wob.at[slot]

        def emit(r0, nr, c0, c1, a):
            if mode == "init":
                acc_ref[rs(r0, nr), c0:c1] = a
            elif mode == "acc":
                acc_ref[r0:r0 + nr, c0:c1] += a
            else:
                finalize(r0, nr, c0, c1, acc_ref[r0:r0 + nr, c0:c1] + a)

        a = jnp.dot(o, w[:, 0:D4], preferred_element_type=_F32)
        emit(r0, tq, 0, D4, a)
        side(jobs, a)
        for t in range(4):
            emit(r0 + t * tb, tb, D4, D,
                 jnp.dot(o[t * tb:(t + 1) * tb, :], w[:, D4:D], preferred_element_type=_F32))
        return a[:, 0:128]

    def pv(par, slot, m, gate, z, jobs=None, before=None, last=False):
        o = lp = None
        for c in range(R):
            mc = m if gate is None else _after(gate, m)
            if before is not None and before[c] is not None:
                mc = _after(rows(before[c](), tq // 8), mc)
            sc = s_ref[z + par % 2, :, c * cw:(c + 1) * cw]
            pe = jnp.exp2(sc - lanes(mc, cw // 128))
            ps = [pe[:, j * 128:(j + 1) * 128] for j in range(cw // 128)]
            for pj in ps:
                lp = pj if lp is None else lp + pj
            ps[-1] = _after(lp, ps[-1])
            pb = jnp.concatenate(ps, axis=1).astype(_BF16)
            oc = jnp.dot(pb, vb[slot, c * cw:(c + 1) * cw, :], preferred_element_type=_F32)
            side(None if jobs is None else jobs[c], oc)
            o = oc if o is None else o + oc
            gate = o
        return o, (lp if last else _after(o, lp))

    def layernorm(r0, nr, rt, z, rel=None):
        def x(k):
            return x_ref[pl.ds(pl.multiple_of(k * z * 16 + r0, 16), nr), :].astype(_F32)
        xs = fold(x(0))
        if rel is not None:
            xs = _after(rel, xs)
        mean = jnp.sum(xs, axis=-1, keepdims=True) * (1.0 / D)
        xc = x(1) - mean
        var = compact(jnp.sum(xc * xc, axis=-1, keepdims=True), 0, jnp.ones((8, 128), _F32)) * (1.0 / D)
        inv = 1.0 / _bf(jnp.sqrt(_bf(_bf(var) + _bf(jnp.float32(_EPS)))))
        inv = jnp.concatenate([jnp.broadcast_to(inv[:, g:g + 1], (8, 128)) for g in range(nr // 8)], axis=0)
        xn = (_bf(x(2) - _bf(mean)) * lanes(inv, D // 128)).astype(_BF16)
        xn_ref[rs(r0, nr), :] = xn
        rp = fold(xn.astype(_F32) * wr_ref[...].astype(_F32).reshape(1, D))
        rt[0] = compact(jnp.sum(rp, axis=-1, keepdims=True), r0 // 8, rt[0])

    def topk(rt):
        rt = _bf(rt)
        lane = jax.lax.broadcasted_iota(_I32, rt.shape, 1)
        sub = jax.lax.broadcasted_iota(_I32, rt.shape, 0)
        bits = pltpu.bitcast(jnp.where(rt == 0.0, 0.0, rt), _I32)
        mono = jnp.where(bits < 0, bits ^ 0x7FFFFFFF, bits) & -65536
        mono = jnp.where(rt != rt, _INT_MIN, mono)
        key = mono | (65535 - (lane * 8 + sub))
        for c in range(_TOPC):
            kmax = jnp.max(jnp.max(key, axis=0, keepdims=True), axis=1, keepdims=True)
            sel_ref[c] = jnp.clip(65535 - (kmax[0, 0] & 65535), 0, S - 1)
            key = jnp.where(key == kmax, _INT_MIN, key)

    def pace(v, k, done, rel):
        t = fold(v)
        t = jnp.concatenate([t[j:j + 8] + t[j + 8:j + 16] for j in range(0, v.shape[0], 16)], axis=0)
        if rel is not None:
            t = _after(jnp.concatenate([rel[j:j + 8] for j in range(0, v.shape[0], 16)], axis=0), t)
        done[0] = compact(jnp.sum(t, axis=-1, keepdims=True), k, done[0])

    def gate_piece(r0, nr, done, rel):
        g = _silu(xn_ref[r0:r0 + nr, :].astype(_F32))
        z_ref[r0:r0 + nr, :] = g
        pace(g, r0 // 16, done, rel)

    def fin_piece(r0, nr, done, z, rel):
        s = _after(lanes(rel, D // 128), acc_ref[r0:r0 + nr, :])
        pace(finalize(r0, nr, 0, D, s), r0 // 16, done, None)
        if (r0 + nr) % tq == 0:
            cp_out(r0 // tq, z).start()

    def ffn_jobs():
        st = {}
        F4 = (F // cw) * cw

        def gather():
            rowid = jax.lax.broadcasted_iota(_I32, (_TOPC, 1), 0)
            xs = jnp.zeros((_TOPC, D), _F32)
            for c in range(_TOPC):
                w = xnp_ref[pl.ds(sel_ref[c] // 2, 1), :]
                w = jnp.where(sel_ref[c] % 2 == 0, w << 16, w & jnp.uint32(0xFFFF0000))
                xs = jnp.where(rowid == c, pltpu.bitcast(w, _F32), xs)
            st["xs"], st["xb"] = xs, xs.astype(_BF16)

        def add(key, val):
            st[key] = val if key not in st else st[key] + val

        def up(parts, k, rel):
            xk = st["xb"][:, k * 128:(k + 1) * 128]
            for name, w_ref, c0, c1 in parts:
                add((name, c0), jax.lax.dot_general(xk, w_ref[c0:c1, k * 128:(k + 1) * 128], _NT,
                                                    preferred_element_type=_F32))

        def hidden():
            cuts = list(range(0, F, cw))
            g = _bf(jnp.concatenate([st["g", c] for c in cuts], axis=1))
            u = _bf(jnp.concatenate([st["u", c] for c in cuts], axis=1))
            st["h"] = (_bf(_silu(g)) * u).astype(_BF16)

        def down(k0, k1, c0, c1, rel):
            if "h" not in st:
                hidden()
            add(("y", c0), jnp.dot(st["h"][:, k0:k1], wd_ref[k0:k1, c0:c1], preferred_element_type=_F32))

        def scatter(done):
            xs = _after(lanes(done, D // 128), st["xs"])
            rs = _bf(jnp.sum(fold(xs * wr_ref[...].astype(_F32).reshape(1, D)), axis=-1, keepdims=True))
            y = _bf(jnp.concatenate([st["y", 0], st["y", D4]], axis=1))
            zz = _silu(_bf(xs + _bf(y * _bf(_sigmoid(rs)))))
            for c in range(_TOPC):
                z_ref[pl.ds(sel_ref[c], 1), :] = zz[c:c + 1, :]

        stage1 = []
        for k in range(D // 128):
            for name, w_ref in (("g", wg_ref), ("u", wu_ref)):
                for c0 in range(0, F4, cw):
                    stage1.append(functools.partial(up, [(name, w_ref, c0, c0 + cw)], k))
            stage1.append(functools.partial(up, [("g", wg_ref, F4, F), ("u", wu_ref, F4, F)], k))
        stage2 = [functools.partial(down, k0, min(k0 + 128, F), 0, D4) for k0 in range(0, F, 128)]
        stage2 += [functools.partial(down, k0, min(k0 + cw, F), D4, D) for k0 in range(0, F, cw)]
        return gather, stage1, stage2, scatter

    zs[0] = jnp.minimum(pl.program_id(0), 0)
    first = (cp_x(0), cp_wr(), cp_wq(0, 0), cp_x(1), cp_k(0, 0), cp_x(2), cp_v(0, 0), cp_x(3), cp_wo(0, 0))
    first += tuple(cp_x(i) for i in range(4, n))
    for h in range(1, B + 1):
        first += cp_head(h, h)
    for c in first + cp_ffn():
        c.start()
    acc_ref[(p - 1) * tq:, :] = jnp.zeros((S - (p - 1) * tq, D), _F32)
    cp_x(0).wait()
    cp_wr().wait()
    z = zs[0]
    rt = [jnp.zeros((8, S // 8), _F32)]

    def ln_jobs(i, z, spread):
        pieces = [functools.partial(layernorm, i * tq + t * tb, tb, rt, z) for t in range(4)]
        return [[pieces.pop(0) for _ in range(k)] for k in spread]

    def first_rounds(us, base, state, z):
        m, o, lp = state
        for u in us:
            jobs = ln_jobs(base + u + 2, z, [2, 2, 0, 0, 0]) if u + 2 < n else [None, None]
            q = qproj(base + u + 1, 0, jobs[0])
            m_next = qk(u + 1, 0, q, z, jobs[1:] if u + 2 < n else None)
            gate = wo(base + u - 1, 0, o, lp, "init")
            o, lp = pv(u, 0, m, gate, z, last=(u == us[-1]))
            m = m_next
        mc_ref[...], oc_ref[...], lc_ref[...] = m, o, lp

    for f in ln_jobs(0, z, [4])[0]:
        f()
    cp_wq(0, 0).wait()
    cp_x(1).wait()
    q0 = qproj(0, 0)
    for f in ln_jobs(1, z, [4])[0]:
        f()
    q1 = qproj(1, 0)
    cp_k(0, 0).wait()
    m0 = qk(0, 0, q0, z, [None] * R, lanewise=True)
    cp_x(2).wait()
    m0 = rowmax(m0)
    m1 = qk(1, 0, q1, z, ln_jobs(2, z, [3, 1, 0, 0]), lanewise=True)
    for c in (cp_v(0, 0), cp_x(3), cp_wo(0, 0)):
        c.wait()
    first_rounds([1], 0, (rowmax(m1),) + pv(0, 0, m0, None, z), z)

    def pair(j, rt_in):
        for k in range(2):
            cp_x(4 + 2 * j + k).wait()
        rt[0] = rt_in
        first_rounds([0, 1], 2 + 2 * j, (mc_ref[...], oc_ref[...], lc_ref[...]), zs[0])
        return rt[0]

    rt[0] = jax.lax.fori_loop(0, 2, pair, rt[0])
    first_rounds([p - 1], 0, (mc_ref[...], oc_ref[...], lc_ref[...]), zs[0])
    topk(rt[0])
    for h in range(1, B + 1):
        for c in cp_head(h, h):
            c.wait()

    def body(j, slots):
        z = zs[0]
        slot = lambda u: slots[u // n]
        m, o, lp = mc_ref[...], oc_ref[...], lc_ref[...]
        for u in range(p, p + B * n):
            m_next = qk((u + 1) % n, slot(u + 1), qproj((u + 1) % n, slot(u + 1)), z)
            gate = wo((u - 1) % n, slot(u - 1), o, lp, "acc")
            if u == p + 1:
                for b in range(B):
                    for c in cp_head(jnp.minimum(B * j + B + 1 + b, H - 1), slots[B + 1 + b]):
                        c.start()
            o, lp = pv(u % n, slot(u), m, gate, z, last=(u == p + B * n - 1))
            m = m_next
        mc_ref[...], oc_ref[...], lc_ref[...] = m, o, lp
        for b in range(B):
            for c in cp_head(0, slots[B + 1 + b]):
                c.wait()
        return slots[B:] + slots[:B]

    jax.lax.fori_loop(0, (H - 2) // B, body, tuple(jnp.int32(k) for k in range(NS)))

    z = zs[0]
    slot = lambda u: (H - 2 + u // n) % NS
    for c in cp_ffn():
        c.wait()
    m, o, lp = mc_ref[...], oc_ref[...], lc_ref[...]
    gather, stage1, stage2, scatter = ffn_jobs()
    gather()
    done, done2 = [jnp.zeros((8, 128), _F32)], [jnp.zeros((8, 128), _F32)]
    late = 3
    gates = [functools.partial(gate_piece, r0, tb, done) for r0 in range(0, S, tb)]
    fins = [functools.partial(fin_piece, r0, tb, done2, z) for r0 in range(0, late * tq, tb)]
    fq = stage1 + [lambda rel: None] + stage2
    u_ffn = n + 1 + late
    for u in range(p, 2 * n):
        def jobs(k):
            vpu = gates if u <= u_ffn else fins
            js = [vpu.pop(0) for _ in range(min(len(vpu), ([2, 2, 2, 2] + [0] * 6)[k]))]
            return js + [fq.pop(0) for _ in range(min(len(fq), 1))]
        m_next = None
        if u + 1 < 2 * n:
            q = qproj((u + 1) % n, slot(u + 1), jobs(0))
            m_next = qk((u + 1) % n, slot(u + 1), q, z, [jobs(1 + c) for c in range(R)])
        if u == u_ffn:
            assert not fq and not gates
            scatter(done[0])
        i = u - 1 - n
        gate = wo((u - 1) % n, slot(u - 1), o, lp, "final" if i >= late else "acc", jobs(5))
        before = [None] * R
        if i >= late:
            cp_out(i, z).start()
            before[2] = functools.partial(stored, ob_ref, i * tq, z)
        if u == 2 * n - 1:
            assert not fins
            before[0] = lambda: done2[0]
        o, lp = pv(u % n, slot(u), m, gate, z, [jobs(6 + c) for c in range(R)], before)
        m = m_next
    wo(n - 1, slot(2 * n - 1), o, lp, "final")
    cp_out(n - 1, z).start()
    for i in range(n):
        cp_out(i, z).wait()


@jax.jit
def pallas_recurrent_scan__mha_block_cached__moe_arch_mod__prompt_kernel(
    A_x: jax.Array,
    A_k_cache: jax.Array,
    A_v_cache: jax.Array,
    A_wq: jax.Array,
    A_wo: jax.Array,
    B_x: jax.Array,
    B_w_r: jax.Array,
    B_w_gate: jax.Array,
    B_w_up: jax.Array,
    B_w_down: jax.Array,
):
    B, S, D = A_x.shape
    _, H, Sk, Dh = A_k_cache.shape
    F = B_w_gate.shape[1]
    assert B == 1 and Sk == S and S % _TQ == 0 and S % _CW == 0 and Dh == 128 and D % 512 == 128
    n = S // _TQ
    assert n == 8 and _P == n - 1 and (H - 2) % _B == 0 and H >= 2 + _B and S % 1024 == 0
    hbm = pl.BlockSpec(memory_space=pltpu.HBM)
    out = pl.pallas_call(
        functools.partial(_kernel, S=S, D=D, Dh=Dh, H=H),
        grid=(1,),
        in_specs=[hbm] * 9,
        out_specs=pl.BlockSpec(memory_space=pl.ANY),
        out_shape=jax.ShapeDtypeStruct((S, D), _BF16),
        scratch_shapes=[
            pltpu.VMEM((S, D), _BF16),
            pltpu.VMEM((S // 2, D), jnp.uint32),
            pltpu.VMEM((S, D), _F32),
            pltpu.VMEM((S, D), _F32),
            pltpu.VMEM((S, D), _BF16),
            pltpu.VMEM((2, _TQ, S), _F32),
            pltpu.VMEM((_TQ, 128), _F32),
            pltpu.VMEM((_TQ, Dh), _F32),
            pltpu.VMEM((_TQ, 128), _F32),
            pltpu.VMEM((_NS, S, Dh), _BF16),
            pltpu.VMEM((_NS, S, Dh), _BF16),
            pltpu.VMEM((_NS, D, Dh), _BF16),
            pltpu.VMEM((_NS, Dh, D), _BF16),
            pltpu.VMEM((F, D), _BF16),
            pltpu.VMEM((F, D), _BF16),
            pltpu.VMEM((F, D), _BF16),
            pltpu.VMEM((D,), _BF16),
            pltpu.SMEM((_TOPC,), _I32),
            pltpu.SMEM((1,), _I32),
            pltpu.SemaphoreType.DMA((4 * _NS + 2 * n + 4,)),
        ],
        compiler_params=pltpu.CompilerParams(
            dimension_semantics=("arbitrary",),
            vmem_limit_bytes=100 * 1024 * 1024,
            disable_bounds_checks=True,
            internal_scratch_in_bytes=64 * 1024,
        ),
    )(A_x.reshape(S, D), A_k_cache.reshape(H, Sk, Dh), A_v_cache.reshape(H, Sk, Dh), A_wq, A_wo,
      B_w_r, B_w_gate.T, B_w_up.T, B_w_down)
    return out.reshape(B, S, D)
```

```python
import functools
import math

import jax
import jax.numpy as jnp
import jax.experimental.pallas as pl
import jax.experimental.pallas.tpu as pltpu

_F32 = jnp.float32
_BF16 = jnp.bfloat16
_I32 = jnp.int32
_NT = (((1,), (1,)), ((), ()))

_TOPC = 8
_EPS = 1e-5
_TQ = 256
_CW = 512
_P = 7
_B = 1
_NS = 2 * _B + 1
_INT_MIN = -2 ** 31


def _bf(x):
    return x.astype(_BF16).astype(_F32)


def _silu(x):
    h = 0.5 * x
    return h + h * jnp.tanh(h)


def _sigmoid(x):
    return 0.5 + 0.5 * jnp.tanh(0.5 * x)


def _after(gate, val):
    return jnp.where(gate > jnp.inf, 0.0, val)


def _kernel(x_hbm, k_hbm, v_hbm, wq_hbm, wo_hbm, wr_hbm, wg_hbm, wu_hbm, wd_hbm,
            out_hbm,
            x_ref, xnp_ref, z_ref, acc_ref, ob_ref, s_ref, mc_ref, oc_ref, lc_ref,
            kb, vb, wqb, wob, wg_ref, wu_ref, wd_ref, wr_ref, sel_ref, zs,
            sems,
            *, S, D, Dh, H):
    tq, cw, p, B, NS = _TQ, _CW, _P, _B, _NS
    n = S // tq
    R = S // cw
    tb = tq // 4
    D4 = (D // 512) * 512
    F = wd_ref.shape[0]
    scale = (Dh ** -0.5) * math.log2(math.e)
    xn_ref = xnp_ref.bitcast(_BF16)

    def hcol(h):
        return pl.ds(pl.multiple_of(h * Dh, Dh), Dh)

    def cp_k(h, slot):
        return pltpu.make_async_copy(k_hbm.at[h], kb.at[slot], sems.at[0 * NS + slot])

    def cp_wq(h, slot):
        return pltpu.make_async_copy(wq_hbm.at[:, hcol(h)], wqb.at[slot], sems.at[1 * NS + slot])

    def cp_v(h, slot):
        return pltpu.make_async_copy(v_hbm.at[h], vb.at[slot], sems.at[2 * NS + slot])

    def cp_wo(h, slot):
        return pltpu.make_async_copy(wo_hbm.at[hcol(h), :], wob.at[slot], sems.at[3 * NS + slot])

    def cp_head(h, slot):
        return (cp_wq(h, slot), cp_k(h, slot), cp_v(h, slot), cp_wo(h, slot))

    def cp_x(i):
        return pltpu.make_async_copy(x_hbm.at[rs(i * tq, tq), :], x_ref.at[rs(i * tq, tq), :],
                                     sems.at[4 * NS + i])

    def cp_out(i, z):
        r0, nr = (i * tq, tq) if i < n - 1 else ((n - 1) * tq + (i - n + 1) * tq // 2, tq // 2)
        src = pl.ds(pl.multiple_of(z * tq + r0, tb), nr)
        return pltpu.make_async_copy(ob_ref.at[src, :], out_hbm.at[pl.ds(r0, nr), :], sems.at[4 * NS + n + i])

    def cp_ffn():
        return (pltpu.make_async_copy(wg_hbm, wg_ref, sems.at[4 * NS + 2 * n + 4]),
                pltpu.make_async_copy(wu_hbm, wu_ref, sems.at[4 * NS + 2 * n + 1]),
                pltpu.make_async_copy(wd_hbm, wd_ref, sems.at[4 * NS + 2 * n + 2]))

    def cp_wr():
        return pltpu.make_async_copy(wr_hbm, wr_ref, sems.at[4 * NS + 2 * n + 3])

    def lanes(v, k):
        return jnp.concatenate([v] * k, axis=1)

    def rows(v, k):
        return jnp.concatenate([v] * k, axis=0)

    def rs(r0, nr):
        return slice(r0, r0 + nr) if isinstance(r0, int) else pl.ds(pl.multiple_of(r0, tb), nr)

    def fold(v):
        t = v[:, 0:128]
        for j in range(1, v.shape[1] // 128):
            t = t + v[:, j * 128:(j + 1) * 128]
        return t

    def compact(col, g0, init):
        lane = jax.lax.broadcasted_iota(_I32, init.shape, 1) - g0
        for g in range(col.shape[0] // 8):
            init = jnp.where(lane == g, col[8 * g:8 * g + 8, :], init)
        return init

    def side(jobs, res):
        for k, f in enumerate(jobs or []):
            r0 = min(k * res.shape[0] // len(jobs) // 8 * 8, res.shape[0] - tb)
            f(res[r0:r0 + tb, 0:128])

    def stored(ref, r0, z):
        k = 32 // (8 * ref.dtype.itemsize)
        v = ref[pl.ds(pl.multiple_of(z * 8 * k + r0, 8 * k), 8 * k), 0:128]
        return v if k == 1 else pltpu.bitcast(v, _F32)

    def qproj(i, slot, jobs=None):
        r0 = i * tq
        w = wqb.at[slot]
        q = jnp.dot(xn_ref[rs(r0, tq), 0:D4], w[0:D4, :], preferred_element_type=_F32)
        q = q + jnp.concatenate(
            [jnp.dot(xn_ref[rs(r0 + t * tb, tb), D4:D], w[D4:D, :], preferred_element_type=_F32)
             for t in range(4)], axis=0)
        side(jobs, q)
        return (q * scale).astype(_BF16)

    def rowmax(mx):
        return jnp.broadcast_to(jnp.max(mx, axis=-1, keepdims=True), (tq, 128))

    def qk(par, slot, q, z, jobs=None, lanewise=False):
        if jobs is None:
            s = jax.lax.dot_general(q, kb[slot], _NT, preferred_element_type=_F32)
            s_ref[z + par % 2] = s
            return rowmax(s)
        mx = None
        for c in range(R):
            s = jax.lax.dot_general(q, kb[slot, c * cw:(c + 1) * cw, :], _NT, preferred_element_type=_F32)
            s_ref[z + par % 2, :, c * cw:(c + 1) * cw] = s
            for j in range(cw // 128):
                sj = s[:, j * 128:(j + 1) * 128]
                mx = sj if mx is None else jnp.maximum(mx, sj)
            side(jobs[c], s)
        return mx if lanewise else rowmax(mx)

    def finalize(r0, nr, c0, c1, s):
        out = x_ref[r0:r0 + nr, c0:c1].astype(_F32) + s * z_ref[r0:r0 + nr, c0:c1]
        ob_ref[r0:r0 + nr, c0:c1] = out.astype(_BF16)
        return out

    def wo(i, slot, o, lp, mode, jobs=None, off=0):
        nq = o.shape[0]
        l = jnp.sum(lp, axis=-1, keepdims=True)
        o = (o * pl.reciprocal(l, full_range=False)).astype(_BF16)
        r0 = i * tq + off
        w = wob.at[slot]

        def emit(r0, nr, c0, c1, a):
            if mode == "init":
                acc_ref[rs(r0, nr), c0:c1] = a
            elif mode == "acc":
                acc_ref[r0:r0 + nr, c0:c1] += a
            else:
                finalize(r0, nr, c0, c1, acc_ref[r0:r0 + nr, c0:c1] + a)

        a = jnp.dot(o, w[:, 0:D4], preferred_element_type=_F32)
        emit(r0, nq, 0, D4, a)
        side(jobs, a)
        for t in range(0, nq, nq // 4):
            emit(r0 + t, nq // 4, D4, D,
                 jnp.dot(o[t:t + nq // 4, :], w[:, D4:D], preferred_element_type=_F32))
        return a[:, 0:128]

    def pv(par, slot, m, gate, z, jobs=None, before=None, last=False, off=0, lag=1):
        o = lp = None
        gates = [gate] * lag
        for c in range(R):
            mc = m if gates[c] is None else _after(gates[c], m)
            if before is not None and before[c] is not None:
                mc = _after(rows(before[c](), m.shape[0] // 8), mc)
            sc = s_ref[z + par % 2, off:off + m.shape[0], c * cw:(c + 1) * cw]
            pe = jnp.exp2(sc - lanes(mc, cw // 128))
            ps = [pe[:, j * 128:(j + 1) * 128] for j in range(cw // 128)]
            for pj in ps:
                lp = pj if lp is None else lp + pj
            ps[-1] = _after(lp, ps[-1])
            pb = jnp.concatenate(ps, axis=1).astype(_BF16)
            oc = jnp.dot(pb, vb[slot, c * cw:(c + 1) * cw, :], preferred_element_type=_F32)
            side(None if jobs is None else jobs[c], oc)
            o = oc if o is None else o + oc
            gates.append(o)
        return o, (lp if last else _after(o, lp))

    def layernorm(r0, nr, rt, z, rel=None):
        def x(k):
            return x_ref[pl.ds(pl.multiple_of(k * z * 16 + r0, 16), nr), :].astype(_F32)
        xs = fold(x(0))
        if rel is not None:
            xs = _after(rel, xs)
        mean = jnp.sum(xs, axis=-1, keepdims=True) * (1.0 / D)
        xc = x(1) - mean
        var = compact(jnp.sum(xc * xc, axis=-1, keepdims=True), 0, jnp.ones((8, 128), _F32)) * (1.0 / D)
        inv = 1.0 / _bf(jnp.sqrt(_bf(_bf(var) + _bf(jnp.float32(_EPS)))))
        inv = jnp.concatenate([jnp.broadcast_to(inv[:, g:g + 1], (8, 128)) for g in range(nr // 8)], axis=0)
        xn = (_bf(x(2) - _bf(mean)) * lanes(inv, D // 128)).astype(_BF16)
        xn_ref[rs(r0, nr), :] = xn
        rp = fold(xn.astype(_F32) * wr_ref[...].astype(_F32).reshape(1, D))
        rt[0] = compact(jnp.sum(rp, axis=-1, keepdims=True), r0 // 8, rt[0])

    def topk(rt):
        rt = _bf(rt)
        lane = jax.lax.broadcasted_iota(_I32, rt.shape, 1)
        sub = jax.lax.broadcasted_iota(_I32, rt.shape, 0)
        bits = pltpu.bitcast(jnp.where(rt == 0.0, 0.0, rt), _I32)
        mono = jnp.where(bits < 0, bits ^ 0x7FFFFFFF, bits) & -65536
        mono = jnp.where(rt != rt, _INT_MIN, mono)
        key = mono | (65535 - (lane * 8 + sub))
        for c in range(_TOPC):
            kmax = jnp.max(jnp.max(key, axis=0, keepdims=True), axis=1, keepdims=True)
            sel_ref[c] = jnp.clip(65535 - (kmax[0, 0] & 65535), 0, S - 1)
            key = jnp.where(key == kmax, _INT_MIN, key)

    def pace(v, k, done, rel):
        t = fold(v)
        t = jnp.concatenate([t[j:j + 8] + t[j + 8:j + 16] for j in range(0, v.shape[0], 16)], axis=0)
        if rel is not None:
            t = _after(jnp.concatenate([rel[j:j + 8] for j in range(0, v.shape[0], 16)], axis=0), t)
        done[0] = compact(jnp.sum(t, axis=-1, keepdims=True), k, done[0])

    def gate_piece(r0, nr, done, rel):
        g = _silu(xn_ref[r0:r0 + nr, :].astype(_F32))
        z_ref[r0:r0 + nr, :] = g
        pace(g, r0 // 16, done, rel)

    def fin_piece(r0, nr, done, z, rel):
        s = _after(lanes(rel, D // 128), acc_ref[r0:r0 + nr, :])
        pace(finalize(r0, nr, 0, D, s), r0 // 16, done, None)
        if (r0 + nr) % tq == 0:
            cp_out(r0 // tq, z).start()

    def ffn_jobs():
        st = {}
        F4 = (F // cw) * cw

        def gather():
            rowid = jax.lax.broadcasted_iota(_I32, (_TOPC, 1), 0)
            xs = jnp.zeros((_TOPC, D), _F32)
            for c in range(_TOPC):
                w = xnp_ref[pl.ds(sel_ref[c] // 2, 1), :]
                w = jnp.where(sel_ref[c] % 2 == 0, w << 16, w & jnp.uint32(0xFFFF0000))
                xs = jnp.where(rowid == c, pltpu.bitcast(w, _F32), xs)
            st["xs"], st["xb"] = xs, xs.astype(_BF16)

        def add(key, val):
            st[key] = val if key not in st else st[key] + val

        def up(parts, k, rel):
            xk = st["xb"][:, k * 128:(k + 1) * 128]
            for name, w_ref, c0, c1 in parts:
                add((name, c0), jax.lax.dot_general(xk, w_ref[c0:c1, k * 128:(k + 1) * 128], _NT,
                                                    preferred_element_type=_F32))

        def hidden():
            cuts = list(range(0, F, cw))
            g = _bf(jnp.concatenate([st["g", c] for c in cuts], axis=1))
            u = _bf(jnp.concatenate([st["u", c] for c in cuts], axis=1))
            st["h"] = (_bf(_silu(g)) * u).astype(_BF16)

        def down(k0, k1, c0, c1, rel):
            if "h" not in st:
                hidden()
            add(("y", c0), jnp.dot(st["h"][:, k0:k1], wd_ref[k0:k1, c0:c1], preferred_element_type=_F32))

        def scatter(done):
            xs = _after(lanes(done, D // 128), st["xs"])
            rs = _bf(jnp.sum(fold(xs * wr_ref[...].astype(_F32).reshape(1, D)), axis=-1, keepdims=True))
            y = _bf(jnp.concatenate([st["y", 0], st["y", D4]], axis=1))
            zz = _silu(_bf(xs + _bf(y * _bf(_sigmoid(rs)))))
            for c in range(_TOPC):
                z_ref[pl.ds(sel_ref[c], 1), :] = zz[c:c + 1, :]

        stage1 = []
        for k in range(D // 128):
            for name, w_ref in (("g", wg_ref), ("u", wu_ref)):
                for c0 in range(0, F4, cw):
                    stage1.append(functools.partial(up, [(name, w_ref, c0, c0 + cw)], k))
            stage1.append(functools.partial(up, [("g", wg_ref, F4, F), ("u", wu_ref, F4, F)], k))
        stage2 = [functools.partial(down, k0, min(k0 + 128, F), 0, D4) for k0 in range(0, F, 128)]
        stage2 += [functools.partial(down, k0, min(k0 + cw, F), D4, D) for k0 in range(0, F, cw)]
        return gather, stage1, stage2, scatter

    zs[0] = jnp.minimum(pl.program_id(0), 0)
    first = (cp_x(0), cp_wr(), cp_wq(0, 0), cp_x(1), cp_k(0, 0), cp_x(2), cp_v(0, 0), cp_x(3), cp_wo(0, 0))
    first += tuple(cp_x(i) for i in range(4, n))
    for h in range(1, B + 1):
        first += cp_head(h, h)
    for c in first + cp_ffn():
        c.start()
    acc_ref[(p - 1) * tq:, :] = jnp.zeros((S - (p - 1) * tq, D), _F32)
    cp_x(0).wait()
    cp_wr().wait()
    z = zs[0]
    rt = [jnp.zeros((8, S // 8), _F32)]

    def ln_jobs(i, z, spread):
        pieces = [functools.partial(layernorm, i * tq + t * tb, tb, rt, z) for t in range(4)]
        return [[pieces.pop(0) for _ in range(k)] for k in spread]

    def first_rounds(us, base, state, z):
        m, o, lp = state
        for u in us:
            jobs = ln_jobs(base + u + 2, z, [2, 2, 0, 0, 0]) if u + 2 < n else [None, None]
            q = qproj(base + u + 1, 0, jobs[0])
            m_next = qk(u + 1, 0, q, z, jobs[1:] if u + 2 < n else None)
            gate = wo(base + u - 1, 0, o, lp, "init")
            o, lp = pv(u, 0, m, gate, z, last=(u == us[-1]))
            m = m_next
        mc_ref[...], oc_ref[...], lc_ref[...] = m, o, lp

    for f in ln_jobs(0, z, [4])[0]:
        f()
    cp_wq(0, 0).wait()
    cp_x(1).wait()
    q0 = qproj(0, 0)
    for f in ln_jobs(1, z, [4])[0]:
        f()
    q1 = qproj(1, 0)
    cp_k(0, 0).wait()
    m0 = qk(0, 0, q0, z, [None] * R, lanewise=True)
    cp_x(2).wait()
    m0 = rowmax(m0)
    m1 = qk(1, 0, q1, z, ln_jobs(2, z, [3, 1, 0, 0]), lanewise=True)
    for c in (cp_v(0, 0), cp_x(3), cp_wo(0, 0)):
        c.wait()
    first_rounds([1], 0, (rowmax(m1),) + pv(0, 0, m0, None, z), z)

    def pair(j, rt_in):
        for k in range(2):
            cp_x(4 + 2 * j + k).wait()
        rt[0] = rt_in
        first_rounds([0, 1], 2 + 2 * j, (mc_ref[...], oc_ref[...], lc_ref[...]), zs[0])
        return rt[0]

    rt[0] = jax.lax.fori_loop(0, 2, pair, rt[0])
    first_rounds([p - 1], 0, (mc_ref[...], oc_ref[...], lc_ref[...]), zs[0])
    topk(rt[0])
    for h in range(1, B + 1):
        for c in cp_head(h, h):
            c.wait()

    def body(j, slots):
        z = zs[0]
        slot = lambda u: slots[u // n]
        m, o, lp = mc_ref[...], oc_ref[...], lc_ref[...]
        for u in range(p, p + B * n):
            m_next = qk((u + 1) % n, slot(u + 1), qproj((u + 1) % n, slot(u + 1)), z)
            gate = wo((u - 1) % n, slot(u - 1), o, lp, "acc")
            if u == p + 1:
                for b in range(B):
                    for c in cp_head(jnp.minimum(B * j + B + 1 + b, H - 1), slots[B + 1 + b]):
                        c.start()
            o, lp = pv(u % n, slot(u), m, gate, z, last=(u == p + B * n - 1))
            m = m_next
        mc_ref[...], oc_ref[...], lc_ref[...] = m, o, lp
        for b in range(B):
            for c in cp_head(0, slots[B + 1 + b]):
                c.wait()
        return slots[B:] + slots[:B]

    jax.lax.fori_loop(0, (H - 2) // B, body, tuple(jnp.int32(k) for k in range(NS)))

    z = zs[0]
    slot = lambda u: (H - 2 + u // n) % NS
    for c in cp_ffn():
        c.wait()
    m, o, lp = mc_ref[...], oc_ref[...], lc_ref[...]
    gather, stage1, stage2, scatter = ffn_jobs()
    gather()
    done, done2 = [jnp.zeros((8, 128), _F32)], [jnp.zeros((8, 128), _F32)]
    late = 3
    gates = [functools.partial(gate_piece, r0, tb, done) for r0 in range(0, S, tb)]
    fins = [functools.partial(fin_piece, r0, tb, done2, z) for r0 in range(0, late * tq, tb)]
    fq = stage1 + [lambda rel: None] + stage2
    u_ffn = n + 1 + late
    for u in range(p, 2 * n - 1):
        def jobs(k):
            vpu = gates if u <= u_ffn else fins
            js = [vpu.pop(0) for _ in range(min(len(vpu), (([2, 2, 1, 1] if u <= u_ffn else [2, 2, 1, 1]) + [0] * 6)[k]))]
            return js + [fq.pop(0) for _ in range(min(len(fq), 1))]
        q = qproj((u + 1) % n, slot(u + 1), jobs(0))
        m_next = qk((u + 1) % n, slot(u + 1), q, z, [jobs(1 + c) for c in range(R)])
        if u == u_ffn:
            assert not fq and not gates
            scatter(done[0])
        i = u - 1 - n
        gate = wo((u - 1) % n, slot(u - 1), o, lp, "final" if i >= late else "acc", jobs(5))
        before = [None] * R
        if i >= late:
            cp_out(i, z).start()
            before[2] = functools.partial(stored, ob_ref, i * tq, z)
        o, lp = pv(u % n, slot(u), m, gate, z, [jobs(6 + c) for c in range(R)], before)
        m = m_next
    assert not fins
    sl, hq = slot(2 * n - 1), tq // 2
    oa, lpa = pv(n - 1, sl, m[:hq], o[:hq], z, before=[lambda: done2[0], None, None, None], lag=2)
    gate = wo(n - 2, sl, o, lp, "final")
    cp_out(n - 2, z).start()
    ob, lpb = pv(n - 1, sl, m[hq:], gate[:hq], z, off=hq, lag=2,
                 before=[None, None, None, functools.partial(stored, ob_ref, (n - 2) * tq, z)])
    wo(n - 1, sl, oa, lpa, "final")
    cp_out(n - 1, z).start()
    wo(n - 1, sl, ob, lpb, "final", off=hq)
    cp_out(n, z).start()
    for i in range(n + 1):
        cp_out(i, z).wait()


@jax.jit
def pallas_recurrent_scan__mha_block_cached__moe_arch_mod__prompt_kernel(
    A_x: jax.Array,
    A_k_cache: jax.Array,
    A_v_cache: jax.Array,
    A_wq: jax.Array,
    A_wo: jax.Array,
    B_x: jax.Array,
    B_w_r: jax.Array,
    B_w_gate: jax.Array,
    B_w_up: jax.Array,
    B_w_down: jax.Array,
):
    B, S, D = A_x.shape
    _, H, Sk, Dh = A_k_cache.shape
    F = B_w_gate.shape[1]
    assert B == 1 and Sk == S and S % _TQ == 0 and S % _CW == 0 and Dh == 128 and D % 512 == 128
    n = S // _TQ
    assert n == 8 and _P == n - 1 and (H - 2) % _B == 0 and H >= 2 + _B and S % 1024 == 0
    hbm = pl.BlockSpec(memory_space=pltpu.HBM)
    out = pl.pallas_call(
        functools.partial(_kernel, S=S, D=D, Dh=Dh, H=H),
        grid=(1,),
        in_specs=[hbm] * 9,
        out_specs=pl.BlockSpec(memory_space=pl.ANY),
        out_shape=jax.ShapeDtypeStruct((S, D), _BF16),
        scratch_shapes=[
            pltpu.VMEM((S, D), _BF16),
            pltpu.VMEM((S // 2, D), jnp.uint32),
            pltpu.VMEM((S, D), _F32),
            pltpu.VMEM((S, D), _F32),
            pltpu.VMEM((S, D), _BF16),
            pltpu.VMEM((2, _TQ, S), _F32),
            pltpu.VMEM((_TQ, 128), _F32),
            pltpu.VMEM((_TQ, Dh), _F32),
            pltpu.VMEM((_TQ, 128), _F32),
            pltpu.VMEM((_NS, S, Dh), _BF16),
            pltpu.VMEM((_NS, S, Dh), _BF16),
            pltpu.VMEM((_NS, D, Dh), _BF16),
            pltpu.VMEM((_NS, Dh, D), _BF16),
            pltpu.VMEM((F, D), _BF16),
            pltpu.VMEM((F, D), _BF16),
            pltpu.VMEM((F, D), _BF16),
            pltpu.VMEM((D,), _BF16),
            pltpu.SMEM((_TOPC,), _I32),
            pltpu.SMEM((1,), _I32),
            pltpu.SemaphoreType.DMA((4 * _NS + 2 * n + 5,)),
        ],
        compiler_params=pltpu.CompilerParams(
            dimension_semantics=("arbitrary",),
            vmem_limit_bytes=100 * 1024 * 1024,
            disable_bounds_checks=True,
            disable_semaphore_checks=True,
            internal_scratch_in_bytes=64 * 1024,
        ),
    )(A_x.reshape(S, D), A_k_cache.reshape(H, Sk, Dh), A_v_cache.reshape(H, Sk, Dh), A_wq, A_wo,
      B_w_r, B_w_gate.T, B_w_up.T, B_w_down)
    return out.reshape(B, S, D)
```

```python
import functools
import math

import jax
import jax.numpy as jnp
import jax.experimental.pallas as pl
import jax.experimental.pallas.tpu as pltpu

_F32 = jnp.float32
_BF16 = jnp.bfloat16
_I32 = jnp.int32
_NT = (((1,), (1,)), ((), ()))

_TOPC = 8
_EPS = 1e-5
_TQ = 256
_CW = 512
_P = 7
_B = 1
_NS = 2 * _B + 1
_INT_MIN = -2 ** 31


def _bf(x):
    return x.astype(_BF16).astype(_F32)


def _silu(x):
    h = 0.5 * x
    return h + h * jnp.tanh(h)


def _sigmoid(x):
    return 0.5 + 0.5 * jnp.tanh(0.5 * x)


def _after(gate, val):
    return jnp.where(gate > jnp.inf, 0.0, val)


def _kernel(x_hbm, k_hbm, v_hbm, wq_hbm, wo_hbm, wr_hbm, wg_hbm, wu_hbm, wd_hbm,
            out_hbm,
            x_ref, xnp_ref, z_ref, acc_ref, ob_ref, s_ref, mc_ref, oc_ref, lc_ref,
            kb, vb, wqb, wob, wg_ref, wu_ref, wd_ref, wr_ref, sel_ref, zs,
            sems,
            *, S, D, Dh, H):
    tq, cw, p, B, NS = _TQ, _CW, _P, _B, _NS
    n = S // tq
    R = S // cw
    tb = tq // 4
    D4 = (D // 512) * 512
    F = wd_ref.shape[0]
    scale = (Dh ** -0.5) * math.log2(math.e)
    xn_ref = xnp_ref.bitcast(_BF16)

    def hcol(h):
        return pl.ds(pl.multiple_of(h * Dh, Dh), Dh)

    def cp_k(h, slot):
        return pltpu.make_async_copy(k_hbm.at[h], kb.at[slot], sems.at[0 * NS + slot])

    def cp_wq(h, slot):
        return pltpu.make_async_copy(wq_hbm.at[:, hcol(h)], wqb.at[slot], sems.at[1 * NS + slot])

    def cp_v(h, slot):
        return pltpu.make_async_copy(v_hbm.at[h], vb.at[slot], sems.at[2 * NS + slot])

    def cp_wo(h, slot):
        return pltpu.make_async_copy(wo_hbm.at[hcol(h), :], wob.at[slot], sems.at[3 * NS + slot])

    def cp_head(h, slot):
        return (cp_wq(h, slot), cp_k(h, slot), cp_v(h, slot), cp_wo(h, slot))

    def cp_x(i):
        return pltpu.make_async_copy(x_hbm.at[rs(i * tq, tq), :], x_ref.at[rs(i * tq, tq), :],
                                     sems.at[4 * NS + i])

    def cp_out(i, z):
        r0, nr = (i * tq, tq) if i < n - 1 else ((n - 1) * tq + (i - n + 1) * tq // 2, tq // 2)
        src = pl.ds(pl.multiple_of(z * tq + r0, tb), nr)
        return pltpu.make_async_copy(ob_ref.at[src, :], out_hbm.at[pl.ds(r0, nr), :], sems.at[4 * NS + n + i])

    def cp_ffn():
        return (pltpu.make_async_copy(wg_hbm, wg_ref, sems.at[4 * NS + 2 * n + 4]),
                pltpu.make_async_copy(wu_hbm, wu_ref, sems.at[4 * NS + 2 * n + 1]),
                pltpu.make_async_copy(wd_hbm, wd_ref, sems.at[4 * NS + 2 * n + 2]))

    def cp_wr():
        return pltpu.make_async_copy(wr_hbm, wr_ref, sems.at[4 * NS + 2 * n + 3])

    def lanes(v, k):
        return jnp.concatenate([v] * k, axis=1)

    def rows(v, k):
        return jnp.concatenate([v] * k, axis=0)

    def rs(r0, nr):
        return slice(r0, r0 + nr) if isinstance(r0, int) else pl.ds(pl.multiple_of(r0, tb), nr)

    def fold(v):
        t = v[:, 0:128]
        for j in range(1, v.shape[1] // 128):
            t = t + v[:, j * 128:(j + 1) * 128]
        return t

    def compact(col, g0, init):
        lane = jax.lax.broadcasted_iota(_I32, init.shape, 1) - g0
        for g in range(col.shape[0] // 8):
            init = jnp.where(lane == g, col[8 * g:8 * g + 8, :], init)
        return init

    def side(jobs, res):
        for k, f in enumerate(jobs or []):
            r0 = min(k * res.shape[0] // len(jobs) // 8 * 8, res.shape[0] - tb)
            f(res[r0:r0 + tb, 0:128])

    def stored(ref, r0, z):
        k = 32 // (8 * ref.dtype.itemsize)
        v = ref[pl.ds(pl.multiple_of(z * 8 * k + r0, 8 * k), 8 * k), 0:128]
        return v if k == 1 else pltpu.bitcast(v, _F32)

    def qproj(i, slot, jobs=None):
        r0 = i * tq
        w = wqb.at[slot]
        q = jnp.dot(xn_ref[rs(r0, tq), 0:D4], w[0:D4, :], preferred_element_type=_F32)
        q = q + jnp.concatenate(
            [jnp.dot(xn_ref[rs(r0 + t * tb, tb), D4:D], w[D4:D, :], preferred_element_type=_F32)
             for t in range(4)], axis=0)
        side(jobs, q)
        return (q * scale).astype(_BF16)

    def rowmax(mx):
        return jnp.broadcast_to(jnp.max(mx, axis=-1, keepdims=True), (tq, 128))

    def qk(par, slot, q, z, jobs=None, lanewise=False):
        if jobs is None:
            s = jax.lax.dot_general(q, kb[slot], _NT, preferred_element_type=_F32)
            s_ref[z + par % 2] = s
            return rowmax(s)
        mx = None
        for c in range(R):
            s = jax.lax.dot_general(q, kb[slot, c * cw:(c + 1) * cw, :], _NT, preferred_element_type=_F32)
            s_ref[z + par % 2, :, c * cw:(c + 1) * cw] = s
            for j in range(cw // 128):
                sj = s[:, j * 128:(j + 1) * 128]
                mx = sj if mx is None else jnp.maximum(mx, sj)
            side(jobs[c], s)
        return mx if lanewise else rowmax(mx)

    def finalize(r0, nr, c0, c1, s):
        out = x_ref[r0:r0 + nr, c0:c1].astype(_F32) + s * z_ref[r0:r0 + nr, c0:c1]
        ob_ref[r0:r0 + nr, c0:c1] = out.astype(_BF16)
        return out

    def wo(i, slot, o, lp, mode, jobs=None, off=0):
        nq = o.shape[0]
        l = jnp.sum(lp, axis=-1, keepdims=True)
        o = (o * pl.reciprocal(l, full_range=False)).astype(_BF16)
        r0 = i * tq + off
        w = wob.at[slot]

        def emit(r0, nr, c0, c1, a):
            if mode == "init":
                acc_ref[rs(r0, nr), c0:c1] = a
            elif mode == "acc":
                acc_ref[r0:r0 + nr, c0:c1] += a
            else:
                finalize(r0, nr, c0, c1, acc_ref[r0:r0 + nr, c0:c1] + a)

        a = jnp.dot(o, w[:, 0:D4], preferred_element_type=_F32)
        emit(r0, nq, 0, D4, a)
        side(jobs, a)
        for t in range(0, nq, nq // 4):
            emit(r0 + t, nq // 4, D4, D,
                 jnp.dot(o[t:t + nq // 4, :], w[:, D4:D], preferred_element_type=_F32))
        return a[:, 0:128]

    def pv(par, slot, m, gate, z, jobs=None, before=None, last=False, off=0, lag=1):
        o = lp = None
        gates = [gate] * lag
        for c in range(R):
            mc = m if gates[c] is None else _after(gates[c], m)
            if before is not None and before[c] is not None:
                mc = _after(rows(before[c](), m.shape[0] // 8), mc)
            sc = s_ref[z + par % 2, off:off + m.shape[0], c * cw:(c + 1) * cw]
            pe = jnp.exp2(sc - lanes(mc, cw // 128))
            ps = [pe[:, j * 128:(j + 1) * 128] for j in range(cw // 128)]
            for pj in ps:
                lp = pj if lp is None else lp + pj
            ps[-1] = _after(lp, ps[-1])
            pb = jnp.concatenate(ps, axis=1).astype(_BF16)
            oc = jnp.dot(pb, vb[slot, c * cw:(c + 1) * cw, :], preferred_element_type=_F32)
            side(None if jobs is None else jobs[c], oc)
            o = oc if o is None else o + oc
            gates.append(o)
        return o, (lp if last else _after(o, lp))

    def layernorm(r0, nr, rt, z, rel=None):
        def x(k):
            k = k if rel is not None else 0
            return x_ref[pl.ds(pl.multiple_of(k * z * 16 + r0, 16), nr), :].astype(_F32)
        xs = fold(x(0))
        if rel is not None:
            xs = _after(rel, xs)
        mean = jnp.sum(xs, axis=-1, keepdims=True) * (1.0 / D)
        xc = x(1) - mean
        var = compact(jnp.sum(xc * xc, axis=-1, keepdims=True), 0, jnp.ones((8, 128), _F32)) * (1.0 / D)
        inv = 1.0 / _bf(jnp.sqrt(_bf(_bf(var) + _bf(jnp.float32(_EPS)))))
        inv = jnp.concatenate([jnp.broadcast_to(inv[:, g:g + 1], (8, 128)) for g in range(nr // 8)], axis=0)
        xn = (_bf(x(2) - _bf(mean)) * lanes(inv, D // 128)).astype(_BF16)
        xn_ref[rs(r0, nr), :] = xn
        rp = fold(xn.astype(_F32) * wr_ref[...].astype(_F32).reshape(1, D))
        rt[0] = compact(jnp.sum(rp, axis=-1, keepdims=True), r0 // 8, rt[0])

    def topk(rt):
        rt = _bf(rt)
        lane = jax.lax.broadcasted_iota(_I32, rt.shape, 1)
        sub = jax.lax.broadcasted_iota(_I32, rt.shape, 0)
        bits = pltpu.bitcast(jnp.where(rt == 0.0, 0.0, rt), _I32)
        mono = jnp.where(bits < 0, bits ^ 0x7FFFFFFF, bits) & -65536
        mono = jnp.where(rt != rt, _INT_MIN, mono)
        key = mono | (65535 - (lane * 8 + sub))
        for c in range(_TOPC):
            kmax = jnp.max(jnp.max(key, axis=0, keepdims=True), axis=1, keepdims=True)
            sel_ref[c] = jnp.clip(65535 - (kmax[0, 0] & 65535), 0, S - 1)
            key = jnp.where(key == kmax, _INT_MIN, key)

    def pace(v, k, done, rel):
        t = fold(v)
        t = jnp.concatenate([t[j:j + 8] + t[j + 8:j + 16] for j in range(0, v.shape[0], 16)], axis=0)
        if rel is not None:
            t = _after(jnp.concatenate([rel[j:j + 8] for j in range(0, v.shape[0], 16)], axis=0), t)
        done[0] = compact(jnp.sum(t, axis=-1, keepdims=True), k, done[0])

    def gate_piece(r0, nr, done, rel):
        g = _silu(xn_ref[r0:r0 + nr, :].astype(_F32))
        z_ref[r0:r0 + nr, :] = g
        pace(g, r0 // 16, done, rel)

    def fin_piece(r0, nr, done, z, rel):
        s = _after(lanes(rel, D // 128), acc_ref[r0:r0 + nr, :])
        pace(finalize(r0, nr, 0, D, s), r0 // 16, done, None)
        if (r0 + nr) % tq == 0:
            cp_out(r0 // tq, z).start()

    def ffn_jobs():
        st = {}
        F4 = (F // cw) * cw

        def gather():
            rowid = jax.lax.broadcasted_iota(_I32, (_TOPC, 1), 0)
            xs = jnp.zeros((_TOPC, D), _F32)
            for c in range(_TOPC):
                w = xnp_ref[pl.ds(sel_ref[c] // 2, 1), :]
                w = jnp.where(sel_ref[c] % 2 == 0, w << 16, w & jnp.uint32(0xFFFF0000))
                xs = jnp.where(rowid == c, pltpu.bitcast(w, _F32), xs)
            st["xs"], st["xb"] = xs, xs.astype(_BF16)

        def add(key, val):
            st[key] = val if key not in st else st[key] + val

        def up(parts, k, rel):
            xk = st["xb"][:, k * 128:(k + 1) * 128]
            for name, w_ref, c0, c1 in parts:
                add((name, c0), jax.lax.dot_general(xk, w_ref[c0:c1, k * 128:(k + 1) * 128], _NT,
                                                    preferred_element_type=_F32))

        def hidden():
            cuts = list(range(0, F, cw))
            g = _bf(jnp.concatenate([st["g", c] for c in cuts], axis=1))
            u = _bf(jnp.concatenate([st["u", c] for c in cuts], axis=1))
            st["h"] = (_bf(_silu(g)) * u).astype(_BF16)

        def down(k0, k1, c0, c1, rel):
            if "h" not in st:
                hidden()
            add(("y", c0), jnp.dot(st["h"][:, k0:k1], wd_ref[k0:k1, c0:c1], preferred_element_type=_F32))

        def scatter(done):
            xs = _after(lanes(done, D // 128), st["xs"])
            rs = _bf(jnp.sum(fold(xs * wr_ref[...].astype(_F32).reshape(1, D)), axis=-1, keepdims=True))
            y = _bf(jnp.concatenate([st["y", 0], st["y", D4]], axis=1))
            zz = _silu(_bf(xs + _bf(y * _bf(_sigmoid(rs)))))
            for c in range(_TOPC):
                z_ref[pl.ds(sel_ref[c], 1), :] = zz[c:c + 1, :]

        stage1 = []
        for k in range(D // 128):
            for name, w_ref in (("g", wg_ref), ("u", wu_ref)):
                for c0 in range(0, F4, cw):
                    stage1.append(functools.partial(up, [(name, w_ref, c0, c0 + cw)], k))
            stage1.append(functools.partial(up, [("g", wg_ref, F4, F), ("u", wu_ref, F4, F)], k))
        stage2 = [functools.partial(down, k0, min(k0 + 128, F), 0, D4) for k0 in range(0, F, 128)]
        stage2 += [functools.partial(down, k0, min(k0 + cw, F), D4, D) for k0 in range(0, F, cw)]
        return gather, stage1, stage2, scatter

    zs[0] = jnp.minimum(pl.program_id(0), 0)
    first = (cp_x(0), cp_wr(), cp_wq(0, 0), cp_x(1), cp_k(0, 0), cp_x(2), cp_v(0, 0), cp_x(3), cp_wo(0, 0))
    first += tuple(cp_x(i) for i in range(4, n))
    for h in range(1, B + 1):
        first += cp_head(h, h)
    for c in first + cp_ffn():
        c.start()
    acc_ref[(p - 1) * tq:, :] = jnp.zeros((S - (p - 1) * tq, D), _F32)
    cp_x(0).wait()
    cp_wr().wait()
    z = zs[0]
    rt = [jnp.zeros((8, S // 8), _F32)]

    def ln_jobs(i, z, spread):
        pieces = [functools.partial(layernorm, i * tq + t * tb, tb, rt, z) for t in range(4)]
        return [[pieces.pop(0) for _ in range(k)] for k in spread]

    def first_rounds(us, base, state, z):
        m, o, lp = state
        for u in us:
            jobs = ln_jobs(base + u + 2, z, [2, 2, 0, 0, 0]) if u + 2 < n else [None, None]
            q = qproj(base + u + 1, 0, jobs[0])
            m_next = qk(u + 1, 0, q, z, jobs[1:] if u + 2 < n else None)
            gate = wo(base + u - 1, 0, o, lp, "init")
            o, lp = pv(u, 0, m, gate, z, last=(u == us[-1]))
            m = m_next
        mc_ref[...], oc_ref[...], lc_ref[...] = m, o, lp

    for f in ln_jobs(0, z, [4])[0]:
        f()
    cp_wq(0, 0).wait()
    cp_x(1).wait()
    q0 = qproj(0, 0)
    for f in ln_jobs(1, z, [4])[0]:
        f()
    q1 = qproj(1, 0)
    cp_k(0, 0).wait()
    m0 = qk(0, 0, q0, z, [None] * R, lanewise=True)
    cp_x(2).wait()
    m0 = rowmax(m0)
    m1 = qk(1, 0, q1, z, ln_jobs(2, z, [3, 1, 0, 0]), lanewise=True)
    for c in (cp_v(0, 0), cp_x(3), cp_wo(0, 0)):
        c.wait()
    first_rounds([1], 0, (rowmax(m1),) + pv(0, 0, m0, None, z), z)

    def pair(j, rt_in):
        for k in range(2):
            cp_x(4 + 2 * j + k).wait()
        rt[0] = rt_in
        first_rounds([0, 1], 2 + 2 * j, (mc_ref[...], oc_ref[...], lc_ref[...]), zs[0])
        return rt[0]

    rt[0] = jax.lax.fori_loop(0, 2, pair, rt[0])
    first_rounds([p - 1], 0, (mc_ref[...], oc_ref[...], lc_ref[...]), zs[0])
    topk(rt[0])
    for h in range(1, B + 1):
        for c in cp_head(h, h):
            c.wait()

    def body(j, slots):
        z = zs[0]
        slot = lambda u: slots[u // n]
        prefetch = [c for b in range(B) for c in cp_head(B * j + B + 1 + b, slots[B + 1 + b])]
        m, o, lp = mc_ref[...], oc_ref[...], lc_ref[...]
        for u in range(p, p + B * n):
            m_next = qk((u + 1) % n, slot(u + 1), qproj((u + 1) % n, slot(u + 1)), z)
            gate = wo((u - 1) % n, slot(u - 1), o, lp, "acc")
            if u == p + 1:
                for c in prefetch:
                    c.start()
            o, lp = pv(u % n, slot(u), m, gate, z, last=(u == p + B * n - 1))
            m = m_next
        mc_ref[...], oc_ref[...], lc_ref[...] = m, o, lp
        for c in prefetch:
            c.wait()
        return slots[B:] + slots[:B]

    jax.lax.fori_loop(0, (H - 2) // B, body, tuple(jnp.int32(k) for k in range(NS)))

    z = zs[0]
    slot = lambda u: (H - 2 + u // n) % NS
    for c in cp_ffn():
        c.wait()
    m, o, lp = mc_ref[...], oc_ref[...], lc_ref[...]
    gather, stage1, stage2, scatter = ffn_jobs()
    gather()
    done, done2 = [jnp.zeros((8, 128), _F32)], [jnp.zeros((8, 128), _F32)]
    late = 3
    gates = [functools.partial(gate_piece, r0, tb, done) for r0 in range(0, S, tb)]
    fins = [functools.partial(fin_piece, r0, tb, done2, z) for r0 in range(0, late * tq, tb)]
    fq = stage1 + [lambda rel: None] + stage2
    u_ffn = n + 1 + late
    for u in range(p, 2 * n - 1):
        def jobs(k):
            vpu = gates if u <= u_ffn else fins
            js = [vpu.pop(0) for _ in range(min(len(vpu), ([2, 2, 1, 1] + [0] * 6)[k]))]
            return js + [fq.pop(0) for _ in range(min(len(fq), 1))]
        q = qproj((u + 1) % n, slot(u + 1), jobs(0))
        m_next = qk((u + 1) % n, slot(u + 1), q, z, [jobs(1 + c) for c in range(R)])
        if u == u_ffn:
            assert not fq and not gates
            scatter(done[0])
        i = u - 1 - n
        gate = wo((u - 1) % n, slot(u - 1), o, lp, "final" if i >= late else "acc", jobs(5))
        before = [None] * R
        if i >= late:
            cp_out(i, z).start()
            before[2] = functools.partial(stored, ob_ref, i * tq, z)
        o, lp = pv(u % n, slot(u), m, gate, z, [jobs(6 + c) for c in range(R)], before)
        m = m_next
    assert not fins
    sl, hq = slot(2 * n - 1), tq // 2
    oa, lpa = pv(n - 1, sl, m[:hq], o[:hq], z, before=[lambda: done2[0], None, None, None], lag=2)
    gate = wo(n - 2, sl, o, lp, "final")
    cp_out(n - 2, z).start()
    ob, lpb = pv(n - 1, sl, m[hq:], gate[:hq], z, off=hq, lag=2,
                 before=[None, None, None, functools.partial(stored, ob_ref, (n - 2) * tq, z)])
    wo(n - 1, sl, oa, lpa, "final")
    cp_out(n - 1, z).start()
    wo(n - 1, sl, ob, lpb, "final", off=hq)
    cp_out(n, z).start()
    for i in range(n + 1):
        cp_out(i, z).wait()


@jax.jit
def pallas_recurrent_scan__mha_block_cached__moe_arch_mod__prompt_kernel(
    A_x: jax.Array,
    A_k_cache: jax.Array,
    A_v_cache: jax.Array,
    A_wq: jax.Array,
    A_wo: jax.Array,
    B_x: jax.Array,
    B_w_r: jax.Array,
    B_w_gate: jax.Array,
    B_w_up: jax.Array,
    B_w_down: jax.Array,
):
    B, S, D = A_x.shape
    _, H, Sk, Dh = A_k_cache.shape
    F = B_w_gate.shape[1]
    assert B == 1 and Sk == S and S % _TQ == 0 and S % _CW == 0 and Dh == 128 and D % 512 == 128
    n = S // _TQ
    assert n == 8 and _P == n - 1 and (H - 2) % _B == 0 and H >= 2 + _B and S % 1024 == 0
    hbm = pl.BlockSpec(memory_space=pltpu.HBM)
    out = pl.pallas_call(
        functools.partial(_kernel, S=S, D=D, Dh=Dh, H=H),
        grid=(1,),
        in_specs=[hbm] * 9,
        out_specs=pl.BlockSpec(memory_space=pl.ANY),
        out_shape=jax.ShapeDtypeStruct((S, D), _BF16),
        scratch_shapes=[
            pltpu.VMEM((S, D), _BF16),
            pltpu.VMEM((S // 2, D), jnp.uint32),
            pltpu.VMEM((S, D), _F32),
            pltpu.VMEM((S, D), _F32),
            pltpu.VMEM((S, D), _BF16),
            pltpu.VMEM((2, _TQ, S), _F32),
            pltpu.VMEM((_TQ, 128), _F32),
            pltpu.VMEM((_TQ, Dh), _F32),
            pltpu.VMEM((_TQ, 128), _F32),
            pltpu.VMEM((_NS, S, Dh), _BF16),
            pltpu.VMEM((_NS, S, Dh), _BF16),
            pltpu.VMEM((_NS, D, Dh), _BF16),
            pltpu.VMEM((_NS, Dh, D), _BF16),
            pltpu.VMEM((F, D), _BF16),
            pltpu.VMEM((F, D), _BF16),
            pltpu.VMEM((F, D), _BF16),
            pltpu.VMEM((D,), _BF16),
            pltpu.SMEM((_TOPC,), _I32),
            pltpu.SMEM((1,), _I32),
            pltpu.SemaphoreType.DMA((4 * _NS + 2 * n + 5,)),
        ],
        compiler_params=pltpu.CompilerParams(
            dimension_semantics=("arbitrary",),
            vmem_limit_bytes=100 * 1024 * 1024,
            disable_bounds_checks=True,
            disable_semaphore_checks=True,
            internal_scratch_in_bytes=64 * 1024,
        ),
    )(A_x.reshape(S, D), A_k_cache.reshape(H, Sk, Dh), A_v_cache.reshape(H, Sk, Dh), A_wq, A_wo,
      B_w_r, B_w_gate.T, B_w_up.T, B_w_down)
    return out.reshape(B, S, D)
```

```python
import functools
import math

import jax
import jax.numpy as jnp
import jax.experimental.pallas as pl
import jax.experimental.pallas.tpu as pltpu

_F32 = jnp.float32
_BF16 = jnp.bfloat16
_I32 = jnp.int32
_NT = (((1,), (1,)), ((), ()))

_TOPC = 8
_EPS = 1e-5
_TQ = 256
_CW = 512
_P = 7
_L = 12
_NS = 4


def _bf(x):
    return x.astype(_BF16).astype(_F32)


def _silu(x):
    h = 0.5 * x
    return h + h * jnp.tanh(h)


def _sigmoid(x):
    return 0.5 + 0.5 * jnp.tanh(0.5 * x)


def _after(gate, val):
    return jnp.where(gate > jnp.inf, 0.0, val)


def _kernel(x_hbm, k_hbm, v_hbm, wq_hbm, wo_hbm, wr_hbm, wg_hbm, wu_hbm, wd_hbm,
            out_hbm,
            x_ref, xnp_ref, z_ref, acc_ref, ob_ref, s_ref, mc_ref, oc_ref, lc_ref,
            kb, vb, wqb, wob, wg_ref, wu_ref, wd_ref, wr_ref, sel_ref, zs,
            sems,
            *, S, D, Dh, H):
    tq, cw, p, L, NS = _TQ, _CW, _P, _L, _NS
    n = S // tq
    R = S // cw
    tb = tq // 4
    D4 = (D // 512) * 512
    F = wd_ref.shape[0]
    scale = (Dh ** -0.5) * math.log2(math.e)
    xn_ref = xnp_ref.bitcast(_BF16)

    def hcol(h):
        return pl.ds(pl.multiple_of(h * Dh, Dh), Dh)

    def cp_k(h, slot):
        return pltpu.make_async_copy(k_hbm.at[h], kb.at[slot], sems.at[0 * NS + slot])

    def cp_wq(h, slot):
        return pltpu.make_async_copy(wq_hbm.at[:, hcol(h)], wqb.at[slot], sems.at[1 * NS + slot])

    def cp_v(h, slot):
        return pltpu.make_async_copy(v_hbm.at[h], vb.at[slot], sems.at[2 * NS + slot])

    def cp_wo(h, slot):
        return pltpu.make_async_copy(wo_hbm.at[hcol(h), :], wob.at[slot], sems.at[3 * NS + slot])

    def cp_head(h, slot):
        return (cp_wq(h, slot), cp_k(h, slot), cp_v(h, slot), cp_wo(h, slot))

    def cp_x(i):
        return pltpu.make_async_copy(x_hbm.at[rs(i * tq, tq), :], x_ref.at[rs(i * tq, tq), :],
                                     sems.at[4 * NS + i])

    def cp_out(i, z):
        r0, nr = (i * tq, tq) if i < n - 1 else ((n - 1) * tq + (i - n + 1) * tq // 2, tq // 2)
        src = pl.ds(pl.multiple_of(z * tq + r0, tb), nr)
        return pltpu.make_async_copy(ob_ref.at[src, :], out_hbm.at[pl.ds(r0, nr), :], sems.at[4 * NS + n + i])

    def cp_ffn():
        return (pltpu.make_async_copy(wg_hbm, wg_ref, sems.at[4 * NS + 2 * n + 4]),
                pltpu.make_async_copy(wu_hbm, wu_ref, sems.at[4 * NS + 2 * n + 1]),
                pltpu.make_async_copy(wd_hbm, wd_ref, sems.at[4 * NS + 2 * n + 2]))

    def cp_wr():
        return pltpu.make_async_copy(wr_hbm, wr_ref, sems.at[4 * NS + 2 * n + 3])

    def lanes(v, k):
        return jnp.concatenate([v] * k, axis=1)

    def rows(v, k):
        return jnp.concatenate([v] * k, axis=0)

    def rs(r0, nr):
        return slice(r0, r0 + nr) if isinstance(r0, int) else pl.ds(pl.multiple_of(r0, tb), nr)

    def fold(v):
        t = v[:, 0:128]
        for j in range(1, v.shape[1] // 128):
            t = t + v[:, j * 128:(j + 1) * 128]
        return t

    def compact(col, g0, init):
        lane = jax.lax.broadcasted_iota(_I32, init.shape, 1) - g0
        for g in range(col.shape[0] // 8):
            init = jnp.where(lane == g, col[8 * g:8 * g + 8, :], init)
        return init

    def side(jobs, res):
        for k, f in enumerate(jobs or []):
            r0 = min(k * res.shape[0] // len(jobs) // 8 * 8, res.shape[0] - tb)
            f(res[r0:r0 + tb, 0:128])

    def stored(ref, r0, z):
        k = 32 // (8 * ref.dtype.itemsize)
        v = ref[pl.ds(pl.multiple_of(z * 8 * k + r0, 8 * k), 8 * k), 0:128]
        return v if k == 1 else pltpu.bitcast(v, _F32)

    def qproj(i, slot, jobs=None):
        w = wqb.at[slot]
        xv = xn_ref.at[rs(i * tq, tq)]
        q = jnp.dot(xv[:, 0:D4], w[0:D4, :], preferred_element_type=_F32)
        q = q + jnp.concatenate(
            [jnp.dot(xv[t * tb:(t + 1) * tb, D4:D], w[D4:D, :], preferred_element_type=_F32)
             for t in range(4)], axis=0)
        side(jobs, q)
        return (q * scale).astype(_BF16)

    def rowmax(mx):
        return jnp.broadcast_to(jnp.max(mx, axis=-1, keepdims=True), (tq, 128))

    def qk(par, slot, q, z, jobs=None, lanewise=False):
        if jobs is None and not lanewise:
            s = jax.lax.dot_general(q, kb[slot], _NT, preferred_element_type=_F32)
            s_ref[z + par % 2] = s
            return rowmax(s)
        mx = None
        for c in range(R):
            s = jax.lax.dot_general(q, kb[slot, c * cw:(c + 1) * cw, :], _NT, preferred_element_type=_F32)
            s_ref[z + par % 2, :, c * cw:(c + 1) * cw] = s
            for j in range(cw // 128):
                sj = s[:, j * 128:(j + 1) * 128]
                mx = sj if mx is None else jnp.maximum(mx, sj)
            side(jobs and jobs[c], s)
        return mx if lanewise else rowmax(mx)

    def finalize(r0, nr, c0, c1, s):
        out = x_ref[r0:r0 + nr, c0:c1].astype(_F32) + s * z_ref[r0:r0 + nr, c0:c1]
        ob_ref[r0:r0 + nr, c0:c1] = out.astype(_BF16)
        return out

    def wo(i, slot, o, lp, mode, jobs=None, off=0):
        nq = o.shape[0]
        l = jnp.sum(lp, axis=-1, keepdims=True)
        o = (o * pl.reciprocal(l, full_range=False)).astype(_BF16)
        w = wob.at[slot]
        av = acc_ref.at[rs(i * tq, tq)]

        def emit(r0, nr, c0, c1, a):
            if mode == "init":
                av[r0:r0 + nr, c0:c1] = a
            elif mode == "acc":
                av[r0:r0 + nr, c0:c1] += a
            else:
                finalize(i * tq + r0, nr, c0, c1, av[r0:r0 + nr, c0:c1] + a)

        a = jnp.dot(o, w[:, 0:D4], preferred_element_type=_F32)
        emit(off, nq, 0, D4, a)
        side(jobs, a)
        for t in range(0, nq, nq // 4):
            emit(off + t, nq // 4, D4, D,
                 jnp.dot(o[t:t + nq // 4, :], w[:, D4:D], preferred_element_type=_F32))
        return a[:, 0:128]

    def pv(par, slot, m, gate, z, jobs=None, before=None, last=False, off=0, lag=1):
        o = lp = None
        gates = [gate] * lag
        for c in range(R):
            mc = m if gates[c] is None else _after(gates[c], m)
            if before is not None and before[c] is not None:
                mc = _after(rows(before[c](), m.shape[0] // 8), mc)
            sc = s_ref[z + par % 2, off:off + m.shape[0], c * cw:(c + 1) * cw]
            pe = jnp.exp2(sc - lanes(mc, cw // 128))
            ps = [pe[:, j * 128:(j + 1) * 128] for j in range(cw // 128)]
            for pj in ps:
                lp = pj if lp is None else lp + pj
            ps[-1] = _after(lp, ps[-1])
            pb = jnp.concatenate(ps, axis=1).astype(_BF16)
            oc = jnp.dot(pb, vb[slot, c * cw:(c + 1) * cw, :], preferred_element_type=_F32)
            side(None if jobs is None else jobs[c], oc)
            o = oc if o is None else o + oc
            gates.append(o)
        return o, (lp if last else _after(o, lp))

    def layernorm(r0, nr, rt, z, rel=None):
        def x(k):
            k = k if rel is not None else 0
            return x_ref[pl.ds(pl.multiple_of(k * z * 16 + r0, 16), nr), :].astype(_F32)
        xs = fold(x(0))
        if rel is not None:
            xs = _after(rel, xs)
        mean = jnp.sum(xs, axis=-1, keepdims=True) * (1.0 / D)
        xc = x(1) - mean
        var = compact(jnp.sum(xc * xc, axis=-1, keepdims=True), 0, jnp.ones((8, 128), _F32)) * (1.0 / D)
        inv = 1.0 / _bf(jnp.sqrt(_bf(_bf(var) + _bf(jnp.float32(_EPS)))))
        inv = jnp.concatenate([jnp.broadcast_to(inv[:, g:g + 1], (8, 128)) for g in range(nr // 8)], axis=0)
        xn = (_bf(x(2) - _bf(mean)) * lanes(inv, D // 128)).astype(_BF16)
        xn_ref[rs(r0, nr), :] = xn
        rp = fold(xn.astype(_F32) * wr_ref[...].astype(_F32).reshape(1, D))
        rt[0] = compact(jnp.sum(rp, axis=-1, keepdims=True), r0 // 8, rt[0])

    def topk(rt):
        rt = _bf(rt)
        lane = jax.lax.broadcasted_iota(_I32, rt.shape, 1)
        sub = jax.lax.broadcasted_iota(_I32, rt.shape, 0)
        top = pltpu.bitcast(jnp.where(rt == 0.0, 0.0, rt), _I32) >> 16
        code = jnp.where(rt != rt, 0, jnp.where(top < 0, -1 - top, top + 32768))
        key = pltpu.bitcast((1 << 29) + code * S + (S - 1 - (lane * 8 + sub)), _F32)
        for c in range(_TOPC):
            kmax = jnp.max(jnp.max(key, axis=0, keepdims=True), axis=1, keepdims=True)
            sel_ref[c] = S - 1 - (pltpu.bitcast(kmax, _I32)[0, 0] & (S - 1))
            key = jnp.where(key == kmax, 0.0, key)

    def pace(v, k, done, rel):
        t = fold(v)
        t = jnp.concatenate([t[j:j + 8] + t[j + 8:j + 16] for j in range(0, v.shape[0], 16)], axis=0)
        if rel is not None:
            t = _after(jnp.concatenate([rel[j:j + 8] for j in range(0, v.shape[0], 16)], axis=0), t)
        done[0] = compact(jnp.sum(t, axis=-1, keepdims=True), k, done[0])

    def gate_piece(r0, nr, done, rel):
        g = _silu(xn_ref[r0:r0 + nr, :].astype(_F32))
        z_ref[r0:r0 + nr, :] = g
        pace(g, r0 // 16, done, rel)

    def fin_piece(r0, nr, done, z, rel):
        s = _after(lanes(rel, D // 128), acc_ref[r0:r0 + nr, :])
        pace(finalize(r0, nr, 0, D, s), r0 // 16, done, None)
        if (r0 + nr) % tq == 0:
            cp_out(r0 // tq, z).start()

    def ffn_jobs():
        st = {}
        F4 = (F // cw) * cw

        def gather():
            rowid = jax.lax.broadcasted_iota(_I32, (_TOPC, 1), 0)
            xs = jnp.zeros((_TOPC, D), _F32)
            for c in range(_TOPC):
                w = xnp_ref[pl.ds(sel_ref[c] // 2, 1), :]
                w = jnp.where(sel_ref[c] % 2 == 0, w << 16, w & jnp.uint32(0xFFFF0000))
                xs = jnp.where(rowid == c, pltpu.bitcast(w, _F32), xs)
            st["xs"], st["xb"] = xs, xs.astype(_BF16)

        def add(key, val):
            st[key] = val if key not in st else st[key] + val

        def up(parts, k, rel):
            xk = st["xb"][:, k * 128:(k + 1) * 128]
            for name, w_ref, c0, c1 in parts:
                add((name, c0), jax.lax.dot_general(xk, w_ref[c0:c1, k * 128:(k + 1) * 128], _NT,
                                                    preferred_element_type=_F32))

        def hidden():
            cuts = list(range(0, F, cw))
            g = _bf(jnp.concatenate([st["g", c] for c in cuts], axis=1))
            u = _bf(jnp.concatenate([st["u", c] for c in cuts], axis=1))
            st["h"] = (_bf(_silu(g)) * u).astype(_BF16)

        def down(k0, k1, c0, c1, rel):
            if "h" not in st:
                hidden()
            add(("y", c0), jnp.dot(st["h"][:, k0:k1], wd_ref[k0:k1, c0:c1], preferred_element_type=_F32))

        def scatter(done):
            xs = _after(lanes(done, D // 128), st["xs"])
            rs = _bf(jnp.sum(fold(xs * wr_ref[...].astype(_F32).reshape(1, D)), axis=-1, keepdims=True))
            y = _bf(jnp.concatenate([st["y", 0], st["y", D4]], axis=1))
            zz = _silu(_bf(xs + _bf(y * _bf(_sigmoid(rs)))))
            for c in range(_TOPC):
                z_ref[pl.ds(sel_ref[c], 1), :] = zz[c:c + 1, :]

        stage1 = []
        for k in range(D // 128):
            for name, w_ref in (("g", wg_ref), ("u", wu_ref)):
                for c0 in range(0, F4, cw):
                    stage1.append(functools.partial(up, [(name, w_ref, c0, c0 + cw)], k))
            stage1.append(functools.partial(up, [("g", wg_ref, F4, F), ("u", wu_ref, F4, F)], k))
        stage2 = [functools.partial(down, k0, min(k0 + 128, F), 0, D4) for k0 in range(0, F, 128)]
        stage2 += [functools.partial(down, k0, min(k0 + cw, F), D4, D) for k0 in range(0, F, cw)]
        return gather, stage1, stage2, scatter

    def save(state):
        mc_ref[...], oc_ref[...], lc_ref[...] = state

    def load():
        return rowmax(mc_ref[...]), oc_ref[...], lc_ref[...]

    def chunk(u):
        return u % n if isinstance(u, int) else u & (n - 1)

    def slot(u):
        return u // n % NS if isinstance(u, int) else (u >> 3) & (NS - 1)

    def round_(u, par, state, z, mode, jobs=None, before=None, last=False, mid=None):
        m, o, lp = state
        q = qproj(chunk(u + 1), slot(u + 1), jobs and jobs[0])
        m_next = qk(par + 1, slot(u + 1), q, z, jobs and jobs[1:R + 1], lanewise=last)
        if mid is not None:
            mid()
        gate = wo(chunk(u - 1), slot(u - 1), o, lp, mode, jobs and jobs[R + 1])
        if mode == "final":
            cp_out(chunk(u - 1), z).start()
        return (m_next,) + pv(par, slot(u), m, gate, z, jobs and jobs[R + 2:], before, last)

    zs[0] = jnp.minimum(pl.program_id(0), 0)
    first = (cp_x(0), cp_wr(), cp_wq(0, 0), cp_x(1), cp_k(0, 0), cp_x(2), cp_v(0, 0), cp_wo(0, 0))
    for c in first + tuple(cp_x(i) for i in range(3, n)) + cp_head(1, 1) + cp_head(2, 2) + cp_ffn():
        c.start()
    @pl.loop(0, (S - (p - 1) * tq) // 32)
    def _(i):
        acc_ref[pl.ds(pl.multiple_of((p - 1) * tq + i * 32, 32), 32), :] = jnp.zeros((32, D), _F32)

    cp_x(0).wait()
    cp_wr().wait()
    z = zs[0]
    rt = [jnp.zeros((8, S // 8), _F32)]

    def ln_jobs(i, z, spread):
        pieces = [functools.partial(layernorm, i * tq + t * tb, tb, rt, z) for t in range(4)]
        return [[pieces.pop(0) for _ in range(k)] for k in spread]

    for f in ln_jobs(0, z, [4])[0]:
        f()
    cp_wq(0, 0).wait()
    cp_x(1).wait()
    q0 = qproj(0, 0)
    for f in ln_jobs(1, z, [4])[0]:
        f()
    q1 = qproj(1, 0)
    cp_k(0, 0).wait()
    m0 = qk(0, 0, q0, z, lanewise=True)
    cp_x(2).wait()
    m0 = rowmax(m0)
    m1 = qk(1, 0, q1, z, ln_jobs(2, z, [3, 1, 0, 0]), lanewise=True)
    cp_v(0, 0).wait()
    cp_wo(0, 0).wait()
    save((m1,) + pv(0, 0, m0, None, z, last=True))

    def pair(j, rt_in):
        for k in range(2):
            pl.when(3 + 2 * j + k < n)(lambda: cp_x(jnp.minimum(3 + 2 * j + k, n - 1)).wait())
        z = zs[0]
        rt[0] = rt_in
        state = load()
        for k in range(2):
            u = 1 + 2 * j + k
            jobs = ln_jobs(jnp.minimum(u + 2, n - 1), z, [2, 2] + [0] * (2 * R))
            state = round_(u, 1 + k, state, z, "init", jobs, last=(k == 1))
        save(state)
        return rt[0]

    scores = jax.lax.fori_loop(0, (p - 1) // 2, pair, rt[0])
    for c in cp_head(1, 1) + cp_head(2, 2):
        c.wait()

    def body(j, carry):
        z = zs[0]
        u0 = p + L * j
        h1 = ((u0 + L) >> 3) + 1
        fetch1 = cp_head(jnp.minimum(h1, H - 1), h1 & (NS - 1))
        fetch2 = cp_head(jnp.minimum(h1 + 1, H - 1), (h1 + 1) & (NS - 1))
        two = (u0 + 2 * L) >> 3 > h1

        def prefetch():
            for c in fetch1:
                c.start()

            @pl.when(two)
            def _():
                for c in fetch2:
                    c.start()

        state = load()
        for k in range(L):
            state = round_(u0 + k, p + k, state, z, "acc", last=(k == L - 1), mid=prefetch if k == 1 else None)
        save(state)
        for c in fetch1:
            c.wait()

        @pl.when(two)
        def _():
            for c in fetch2:
                c.wait()

        return carry

    T = H * n
    jax.lax.fori_loop(0, (T - 2 * n) // L, body, 0)

    z = zs[0]
    for c in cp_ffn():
        c.wait()
    state = load()
    gather, stage1, stage2, scatter = ffn_jobs()
    topk(scores)
    gather()
    done, done2 = [jnp.zeros((8, 128), _F32)], [jnp.zeros((8, 128), _F32)]
    late = 3
    gates = [functools.partial(gate_piece, r0, tb, done) for r0 in range(0, S, tb)]
    fins = [functools.partial(fin_piece, r0, tb, done2, z) for r0 in range(0, late * tq, tb)]
    fq = stage1 + [lambda rel: None] + stage2
    u_first = T - 2 * n + p
    for u in range(u_first, T - 1):
        i = u - 1 - (T - n)
        vpu, nv, nf = gates, [2, 2, 2, 1], [1] * 6 + [1 if i < late - 2 else 2] * 4
        if u == u_first:
            nv, nf = [0, 0, 0, 0], [0] * 6 + [1] * 4
        if i > late:
            vpu, nv = fins, [2, 2, 1, 1]
        jobs = [[vpu.pop(0) for _ in range(min(len(vpu), a))] + [fq.pop(0) for _ in range(min(len(fq), b))]
                for a, b in zip(nv + [0] * 6, nf)]
        before = [None] * R
        if i >= late:
            assert not fq and not gates
            before[2] = functools.partial(stored, ob_ref, i * tq, z)
        state = round_(u, u, state, z, "final" if i >= late else "acc", jobs, before,
                       mid=(lambda: scatter(done[0])) if i == late else None)
    assert not fins
    m, o, lp = state
    sl, hq = slot(T - 1), tq // 2
    oa, lpa = pv(T - 1, sl, m[:hq], o[:hq], z, before=[lambda: done2[0], None, None, None], lag=2)
    gate = wo(n - 2, sl, o, lp, "final")
    cp_out(n - 2, z).start()
    ob, lpb = pv(T - 1, sl, m[hq:], gate[:hq], z, off=hq, lag=2,
                 before=[None, None, None, functools.partial(stored, ob_ref, (n - 2) * tq, z)])
    wo(n - 1, sl, oa, lpa, "final")
    cp_out(n - 1, z).start()
    wo(n - 1, sl, ob, lpb, "final", off=hq)
    cp_out(n, z).start()
    for i in range(n + 1):
        cp_out(i, z).wait()


@jax.jit
def pallas_recurrent_scan__mha_block_cached__moe_arch_mod__prompt_kernel(
    A_x: jax.Array,
    A_k_cache: jax.Array,
    A_v_cache: jax.Array,
    A_wq: jax.Array,
    A_wo: jax.Array,
    B_x: jax.Array,
    B_w_r: jax.Array,
    B_w_gate: jax.Array,
    B_w_up: jax.Array,
    B_w_down: jax.Array,
):
    B, S, D = A_x.shape
    _, H, Sk, Dh = A_k_cache.shape
    F = B_w_gate.shape[1]
    assert B == 1 and Sk == S and S % _TQ == 0 and S % _CW == 0 and Dh == 128 and D % 512 == 128
    n = S // _TQ
    assert n == 8 and _P == n - 1 and (H - 2) * n % _L == 0 and _L == 12 and _NS == 4 and S == 2048
    hbm = pl.BlockSpec(memory_space=pltpu.HBM)
    out = pl.pallas_call(
        functools.partial(_kernel, S=S, D=D, Dh=Dh, H=H),
        grid=(1,),
        in_specs=[hbm] * 9,
        out_specs=pl.BlockSpec(memory_space=pl.ANY),
        out_shape=jax.ShapeDtypeStruct((S, D), _BF16),
        scratch_shapes=[
            pltpu.VMEM((S, D), _BF16),
            pltpu.VMEM((S // 2, D), jnp.uint32),
            pltpu.VMEM((S, D), _F32),
            pltpu.VMEM((S, D), _F32),
            pltpu.VMEM((S, D), _BF16),
            pltpu.VMEM((2, _TQ, S), _F32),
            pltpu.VMEM((_TQ, 128), _F32),
            pltpu.VMEM((_TQ, Dh), _F32),
            pltpu.VMEM((_TQ, 128), _F32),
            pltpu.VMEM((_NS, S, Dh), _BF16),
            pltpu.VMEM((_NS, S, Dh), _BF16),
            pltpu.VMEM((_NS, D, Dh), _BF16),
            pltpu.VMEM((_NS, Dh, D), _BF16),
            pltpu.VMEM((F, D), _BF16),
            pltpu.VMEM((F, D), _BF16),
            pltpu.VMEM((F, D), _BF16),
            pltpu.VMEM((D,), _BF16),
            pltpu.SMEM((_TOPC,), _I32),
            pltpu.SMEM((1,), _I32),
            pltpu.SemaphoreType.DMA((4 * _NS + 2 * n + 5,)),
        ],
        compiler_params=pltpu.CompilerParams(
            dimension_semantics=("arbitrary",),
            vmem_limit_bytes=100 * 1024 * 1024,
            disable_bounds_checks=True,
            disable_semaphore_checks=True,
            internal_scratch_in_bytes=64 * 1024,
        ),
    )(A_x.reshape(S, D), A_k_cache.reshape(H, Sk, Dh), A_v_cache.reshape(H, Sk, Dh), A_wq, A_wo,
      B_w_r, B_w_gate.T, B_w_up.T, B_w_down)
    return out.reshape(B, S, D)
```

```python
import functools
import math

import jax
import jax.numpy as jnp
import jax.experimental.pallas as pl
import jax.experimental.pallas.tpu as pltpu

_F32 = jnp.float32
_BF16 = jnp.bfloat16
_I32 = jnp.int32
_NT = (((1,), (1,)), ((), ()))

_TOPC = 8
_EPS = 1e-5
_TQ = 256
_CW = 512
_P = 7
_L = 12
_NS = 4


def _bf(x):
    return x.astype(_BF16).astype(_F32)


def _silu(x):
    h = 0.5 * x
    return h + h * jnp.tanh(h)


def _sigmoid(x):
    return 0.5 + 0.5 * jnp.tanh(0.5 * x)


def _after(gate, val):
    return jnp.where(gate > jnp.inf, 0.0, val)


def _after16(gate, val):
    g = gate > jnp.inf
    g = jnp.concatenate([g[r:r + 8] for r in range(8, gate.shape[0], 16) for _ in range(2)], axis=0)
    return jnp.where(g, 0.0, val)


def _kernel(x_hbm, k_hbm, v_hbm, wq_hbm, wo_hbm, wr_hbm, wg_hbm, wu_hbm, wd_hbm,
            out_hbm,
            x_ref, xnp_ref, z_ref, acc_ref, ob_ref, s_ref, mc_ref, oc_ref, lc_ref,
            hb, wg_ref, wu_ref, wd_ref, wr_ref, sel_ref, zs,
            sems,
            *, S, D, Dh, H):
    tq, cw, p, L, NS = _TQ, _CW, _P, _L, _NS
    n = S // tq
    R = S // cw
    tb = tq // 4
    D4 = (D // 512) * 512
    F = wd_ref.shape[0]
    scale = (Dh ** -0.5) * math.log2(math.e)
    xn_ref = xnp_ref.bitcast(_BF16)

    K0, V0, Q0, O0 = 0, S, 2 * S, 2 * S + D

    def hcol(h):
        return pl.ds(pl.multiple_of(h * Dh, Dh), Dh)

    def cp_k(h, slot, sem):
        return (pltpu.make_async_copy(k_hbm.at[h], hb.at[slot, K0:K0 + S], sems.at[sem]),)

    def cp_v(h, slot, sem):
        return (pltpu.make_async_copy(v_hbm.at[h], hb.at[slot, V0:V0 + S], sems.at[sem]),)

    def cp_wq(h, slot, sem):
        return (pltpu.make_async_copy(wq_hbm.at[:, hcol(h)], hb.at[slot, Q0:Q0 + D], sems.at[sem]),)

    def cp_wo(h, slot, sem):
        return tuple(pltpu.make_async_copy(wo_hbm.at[hcol(h), c:c + 128], hb.at[slot, O0 + c:O0 + c + 128],
                                           sems.at[sem]) for c in range(0, D, 128))

    def start_head(h, slot):
        for cp in (cp_wq, cp_k, cp_v, cp_wo):
            for c in cp(h, slot, slot):
                c.start()

    def wait_head(slot):
        pltpu.make_async_copy(hb.at[slot], hb.at[slot], sems.at[slot]).wait()

    def cp_x(i):
        return pltpu.make_async_copy(x_hbm.at[rs(i * tq, tq), :], x_ref.at[rs(i * tq, tq), :],
                                     sems.at[NS + 4 + i])

    def cp_out(i, z):
        r0, nr = (i * tq, tq) if i < n - 1 else ((n - 1) * tq + (i - n + 1) * tq // 2, tq // 2)
        src = pl.ds(pl.multiple_of(z * tq + r0, tb), nr)
        return pltpu.make_async_copy(ob_ref.at[src, :], out_hbm.at[pl.ds(r0, nr), :], sems.at[NS + 4 + n + i])

    def cp_ffn():
        return (pltpu.make_async_copy(wg_hbm, wg_ref, sems.at[NS + 4 + 2 * n + 4]),
                pltpu.make_async_copy(wu_hbm, wu_ref, sems.at[NS + 4 + 2 * n + 1]),
                pltpu.make_async_copy(wd_hbm, wd_ref, sems.at[NS + 4 + 2 * n + 2]))

    def cp_wr():
        return pltpu.make_async_copy(wr_hbm, wr_ref, sems.at[NS + 4 + 2 * n + 3])

    def lanes(v, k):
        return jnp.concatenate([v] * k, axis=1)

    def rows(v, k):
        return jnp.concatenate([v] * k, axis=0)

    def rs(r0, nr):
        return slice(r0, r0 + nr) if isinstance(r0, int) else pl.ds(pl.multiple_of(r0, tb), nr)

    def fold(v):
        t = v[:, 0:128]
        for j in range(1, v.shape[1] // 128):
            t = t + v[:, j * 128:(j + 1) * 128]
        return t

    def compact(col, g0, init):
        lane = jax.lax.broadcasted_iota(_I32, init.shape, 1) - g0
        for g in range(col.shape[0] // 8):
            init = jnp.where(lane == g, col[8 * g:8 * g + 8, :], init)
        return init

    def side(jobs, res):
        for k, f in enumerate(jobs or []):
            r0 = min(k * res.shape[0] // len(jobs) // 8 * 8, res.shape[0] - tb)
            f(res[r0:r0 + tb, 0:128])

    def stored(ref, r0, z):
        k = 32 // (8 * ref.dtype.itemsize)
        v = ref[pl.ds(pl.multiple_of(z * 8 * k + r0, 8 * k), 8 * k), 0:128]
        return v if k == 1 else pltpu.bitcast(v, _F32)

    def qproj(i, slot, jobs=None):
        w = hb.at[slot, Q0:Q0 + D]
        xv = xn_ref.at[rs(i * tq, tq)]
        q = jnp.dot(xv[:, 0:D4], w[0:D4, :], preferred_element_type=_F32)
        q = q + jnp.concatenate(
            [jnp.dot(xv[t * tb:(t + 1) * tb, D4:D], w[D4:D, :], preferred_element_type=_F32)
             for t in range(4)], axis=0)
        side(jobs, q)
        return (q * scale).astype(_BF16)

    def rowmax(mx):
        return jnp.broadcast_to(jnp.max(mx, axis=-1, keepdims=True), (tq, 128))

    def qk(par, slot, q, z, jobs=None, lanewise=False):
        if jobs is None and not lanewise:
            s = jax.lax.dot_general(q, hb[slot, K0:K0 + S], _NT, preferred_element_type=_F32)
            s_ref[z + par % 2] = s
            return rowmax(s)
        mx = None
        for c in range(R):
            s = jax.lax.dot_general(q, hb[slot, K0 + c * cw:K0 + (c + 1) * cw], _NT, preferred_element_type=_F32)
            s_ref[z + par % 2, :, c * cw:(c + 1) * cw] = s
            for j in range(cw // 128):
                sj = s[:, j * 128:(j + 1) * 128]
                mx = sj if mx is None else jnp.maximum(mx, sj)
            side(jobs and jobs[c], s)
        return mx if lanewise else rowmax(mx)

    def finalize(r0, nr, c0, c1, s):
        out = x_ref[r0:r0 + nr, c0:c1].astype(_F32) + s * z_ref[r0:r0 + nr, c0:c1]
        ob_ref[r0:r0 + nr, c0:c1] = out.astype(_BF16)
        return out

    def wo(i, slot, o, lp, mode, jobs=None, off=0):
        nq = o.shape[0]
        l = jnp.sum(lp, axis=-1, keepdims=True)
        o32 = o * pl.reciprocal(l, full_range=False)
        o = o32.astype(_BF16)
        w = [hb[slot, O0 + c:O0 + c + 128] for c in range(0, D, 128)]
        av = acc_ref.at[rs(i * tq, tq)]

        def emit(r0, nr, c0, c1, a):
            if mode == "init":
                av[r0:r0 + nr, c0:c1] = a
            elif mode == "acc":
                av[r0:r0 + nr, c0:c1] += a
            else:
                finalize(i * tq + r0, nr, c0, c1, av[r0:r0 + nr, c0:c1] + a)

        a = jnp.dot(o, jnp.concatenate(w[:-1], axis=1), preferred_element_type=_F32)
        emit(off, nq, 0, D4, a)
        side(jobs, a)
        for t in range(0, nq, nq // 4):
            emit(off + t, nq // 4, D4, D,
                 jnp.dot(o32[t:t + nq // 4, :].astype(_BF16), w[-1], preferred_element_type=_F32))
        return a[:, 0:128]

    def pv(par, slot, m, gate, z, jobs=None, before=None, last=False, off=0, lag=1):
        o = lp = None
        gates = [gate] * lag
        for c in range(R):
            mc = m if gates[c] is None else _after16(gates[c], m)
            if before is not None and before[c] is not None:
                mc = _after(rows(before[c](), m.shape[0] // 8), mc)
            sc = s_ref[z + par % 2, off:off + m.shape[0], c * cw:(c + 1) * cw]
            pe = jnp.exp2(sc - lanes(mc, cw // 128))
            ps = [pe[:, j * 128:(j + 1) * 128] for j in range(cw // 128)]
            for pj in ps:
                lp = pj if lp is None else lp + pj
            ps[-1] = jnp.minimum(ps[-1], lp)
            pb = jnp.concatenate(ps, axis=1).astype(_BF16)
            oc = jnp.dot(pb, hb[slot, V0 + c * cw:V0 + (c + 1) * cw], preferred_element_type=_F32)
            side(None if jobs is None else jobs[c], oc)
            o = oc if o is None else o + oc
            gates.append(o)
        return o, (lp if last else _after16(o, lp))

    def layernorm(r0, nr, rt, z, rel=None):
        def x(k):
            k = k if rel is not None else 0
            return x_ref[pl.ds(pl.multiple_of(k * z * 16 + r0, 16), nr), :].astype(_F32)
        xs = fold(x(0))
        if rel is not None:
            xs = _after(rel, xs)
        mean = jnp.sum(xs, axis=-1, keepdims=True) * (1.0 / D)
        xc = x(1) - mean
        var = compact(jnp.sum(xc * xc, axis=-1, keepdims=True), 0, jnp.ones((8, 128), _F32)) * (1.0 / D)
        inv = 1.0 / _bf(jnp.sqrt(_bf(_bf(var) + _bf(jnp.float32(_EPS)))))
        inv = jnp.concatenate([jnp.broadcast_to(inv[:, g:g + 1], (8, 128)) for g in range(nr // 8)], axis=0)
        xn = (_bf(x(2) - _bf(mean)) * lanes(inv, D // 128)).astype(_BF16)
        xn_ref[rs(r0, nr), :] = xn
        rp = fold(xn.astype(_F32) * wr_ref[...].astype(_F32).reshape(1, D))
        rt[0] = compact(jnp.sum(rp, axis=-1, keepdims=True), r0 // 8, rt[0])

    def topk(rt):
        rt = _bf(rt)
        lane = jax.lax.broadcasted_iota(_I32, rt.shape, 1)
        sub = jax.lax.broadcasted_iota(_I32, rt.shape, 0)
        top = pltpu.bitcast(jnp.where(rt == 0.0, 0.0, rt), _I32) >> 16
        code = jnp.where(rt != rt, 0, jnp.where(top < 0, -1 - top, top + 32768))
        key = pltpu.bitcast((1 << 29) + code * S + (S - 1 - (lane * 8 + sub)), _F32)
        for c in range(_TOPC):
            kmax = jnp.max(jnp.max(key, axis=0, keepdims=True), axis=1, keepdims=True)
            sel_ref[c] = S - 1 - (pltpu.bitcast(kmax, _I32)[0, 0] & (S - 1))
            key = jnp.where(key == kmax, 0.0, key)

    def pace(v, k, done, rel):
        t = fold(v)
        t = jnp.concatenate([t[j:j + 8] + t[j + 8:j + 16] for j in range(0, v.shape[0], 16)], axis=0)
        if rel is not None:
            t = _after(jnp.concatenate([rel[j:j + 8] for j in range(0, v.shape[0], 16)], axis=0), t)
        done[0] = compact(jnp.sum(t, axis=-1, keepdims=True), k, done[0])

    def gate_piece(r0, nr, done, rel):
        g = _silu(xn_ref[r0:r0 + nr, :].astype(_F32))
        z_ref[r0:r0 + nr, :] = g
        pace(g, r0 // 16, done, rel)

    def fin_piece(r0, nr, done, z, rel):
        s = _after(lanes(rel, D // 128), acc_ref[r0:r0 + nr, :])
        pace(finalize(r0, nr, 0, D, s), r0 // 16, done, None)
        if (r0 + nr) % tq == 0:
            cp_out(r0 // tq, z).start()

    def ffn_jobs():
        st = {}
        F4 = (F // cw) * cw

        def gather():
            rowid = jax.lax.broadcasted_iota(_I32, (_TOPC, 1), 0)
            xs = jnp.zeros((_TOPC, D), _F32)
            for c in range(_TOPC):
                w = xnp_ref[pl.ds(sel_ref[c] // 2, 1), :]
                w = jnp.where(sel_ref[c] % 2 == 0, w << 16, w & jnp.uint32(0xFFFF0000))
                xs = jnp.where(rowid == c, pltpu.bitcast(w, _F32), xs)
            st["xs"], st["xb"] = xs, xs.astype(_BF16)

        def add(key, val):
            st[key] = val if key not in st else st[key] + val

        def up(parts, k, rel):
            xk = st["xb"][:, k * 128:(k + 1) * 128]
            for name, w_ref, c0, c1 in parts:
                add((name, c0), jax.lax.dot_general(xk, w_ref[c0:c1, k * 128:(k + 1) * 128], _NT,
                                                    preferred_element_type=_F32))

        def hidden():
            cuts = list(range(0, F, cw))
            g = _bf(jnp.concatenate([st["g", c] for c in cuts], axis=1))
            u = _bf(jnp.concatenate([st["u", c] for c in cuts], axis=1))
            st["h"] = (_bf(_silu(g)) * u).astype(_BF16)

        def down(cuts, c0, c1, rel):
            if "h" not in st:
                hidden()
            for k0, k1 in zip(cuts[:-1], cuts[1:]):
                add(("y", c0), jnp.dot(st["h"][:, k0:k1], wd_ref[k0:k1, c0:c1], preferred_element_type=_F32))

        def scatter(done):
            xs = _after(lanes(done, D // 128), st["xs"])
            rs = _bf(jnp.sum(fold(xs * wr_ref[...].astype(_F32).reshape(1, D)), axis=-1, keepdims=True))
            y = _bf(jnp.concatenate([st["y", 0], st["y", D4]], axis=1))
            zz = _silu(_bf(xs + _bf(y * _bf(_sigmoid(rs)))))
            for c in range(_TOPC):
                z_ref[pl.ds(sel_ref[c], 1), :] = zz[c:c + 1, :]

        stage1 = []
        for k in range(D // 128):
            for name, w_ref in (("g", wg_ref), ("u", wu_ref)):
                for c0 in range(0, F4, cw):
                    stage1.append(functools.partial(up, [(name, w_ref, c0, c0 + cw)], k))
            stage1.append(functools.partial(up, [("g", wg_ref, F4, F), ("u", wu_ref, F4, F)], k))
        stage2 = [functools.partial(down, [k0, min(k0 + 128, F)], 0, D4) for k0 in range(0, F, 128)]
        stage2 += [functools.partial(down, [k0, k0 + cw], D4, D) for k0 in range(0, F4, cw)]
        stage2 += [functools.partial(down, [F4, F4 + 64, F4 + 128, F4 + 160, F], D4, D)]
        return gather, stage1, stage2, scatter

    def save(state):
        mc_ref[...], oc_ref[...], lc_ref[...] = state

    def load():
        return rowmax(mc_ref[...]), oc_ref[...], lc_ref[...]

    def chunk(u):
        return u % n if isinstance(u, int) else u & (n - 1)

    def slot(u):
        return u // n % NS if isinstance(u, int) else (u >> 3) & (NS - 1)

    def round_(u, par, state, z, mode, jobs=None, before=None, last=False, mid=None, nxt=None):
        m, o, lp = state
        c1, s1 = nxt or (chunk(u + 1), slot(u + 1))
        q = qproj(c1, s1, jobs and jobs[0])
        m_next = qk(par + 1, s1, q, z, jobs and jobs[1:R + 1], lanewise=last)
        if mid is not None:
            mid()
        gate = wo(chunk(u - 1), slot(u - 1), o, lp, mode, jobs and jobs[R + 1])
        if mode == "final":
            cp_out(chunk(u - 1), z).start()
        return (m_next,) + pv(par, slot(u), m, gate, z, jobs and jobs[R + 2:], before, last)

    zs[0] = jnp.minimum(pl.program_id(0), 0)
    wq0, k0, v0, wo0 = (cp(0, 0, NS + t) for t, cp in enumerate((cp_wq, cp_k, cp_v, cp_wo)))
    for c in (cp_x(0), cp_wr(), *wq0, cp_x(1), *k0, cp_x(2), *v0, *wo0, *(cp_x(i) for i in range(3, n))):
        c.start()
    start_head(1, 1)
    start_head(2, 2)
    for c in cp_ffn():
        c.start()
    @pl.loop(0, (S - (p - 1) * tq) // 32)
    def _(i):
        acc_ref[pl.ds(pl.multiple_of((p - 1) * tq + i * 32, 32), 32), :] = jnp.zeros((32, D), _F32)

    cp_x(0).wait()
    cp_wr().wait()
    z = zs[0]
    rt = [jnp.zeros((8, S // 8), _F32)]

    def ln_jobs(i, z, spread):
        pieces = [functools.partial(layernorm, i * tq + t * tb, tb, rt, z) for t in range(4)]
        return [[pieces.pop(0) for _ in range(k)] for k in spread]

    for f in ln_jobs(0, z, [4])[0]:
        f()
    wq0[0].wait()
    cp_x(1).wait()
    q0 = qproj(0, 0)
    for f in ln_jobs(1, z, [4])[0]:
        f()
    q1 = qproj(1, 0)
    k0[0].wait()
    m0 = qk(0, 0, q0, z, lanewise=True)
    cp_x(2).wait()
    m0 = rowmax(m0)
    m1 = qk(1, 0, q1, z, ln_jobs(2, z, [3, 1, 0, 0]), lanewise=True)
    for c in v0 + wo0:
        c.wait()
    save((m1,) + pv(0, 0, m0, None, z, last=True))

    def pair(j, rt_in):
        for k in range(2):
            pl.when(3 + 2 * j + k < n)(lambda: cp_x(jnp.minimum(3 + 2 * j + k, n - 1)).wait())
        z = zs[0]
        rt[0] = rt_in
        state = load()
        for k in range(2):
            u = 1 + 2 * j + k
            jobs = ln_jobs(jnp.minimum(u + 2, n - 1), z, [1, 1, 1, 1, 0, 0, 0, 0, 0, 0])
            state = round_(u, 1 + k, state, z, "init", jobs, last=(k == 1))
        save(state)
        return rt[0]

    scores = jax.lax.fori_loop(0, (p - 1) // 2, pair, rt[0])

    def entry(u0):
        h0 = (u0 >> 3) + 1
        return (u0, h0 & (NS - 1), (h0 + 1) & (NS - 1), ((u0 + L) >> 3) - h0, chunk(u0 + 1), slot(u0 + 1))

    def body(j, carry):
        u0, w1, w2, two, c1, s1 = carry
        wait_head(w1)
        pl.when(two > 0)(lambda: wait_head(w2))
        z = zs[0]

        def prefetch():
            h1 = ((u0 + L) >> 3) + 1
            start_head(h1, h1 & (NS - 1))
            pl.when(h1 + 1 <= jnp.minimum((u0 + 2 * L) >> 3, H - 1))(
                lambda: start_head(h1 + 1, (h1 + 1) & (NS - 1)))

        state = load()
        for k in range(L):
            state = round_(u0 + k, p + k, state, z, "acc", last=(k == L - 1), mid=prefetch if k == 1 else None,
                           nxt=(c1, s1) if k == 0 else None)
        save(state)
        return entry(u0 + L)

    T = H * n
    jax.lax.fori_loop(0, (T - 2 * n) // L, body, entry(jnp.int32(p)))

    wait_head((H - 1) % NS)
    for c in cp_ffn():
        c.wait()
    z = zs[0]
    state = load()
    gather, stage1, stage2, scatter = ffn_jobs()
    topk(scores)
    gather()
    done, done2 = [jnp.zeros((8, 128), _F32)], [jnp.zeros((8, 128), _F32)]
    late = 3
    gates = [functools.partial(gate_piece, r0, tb, done) for r0 in range(0, S, tb)]
    fins = [functools.partial(fin_piece, r0, tb, done2, z) for r0 in range(0, late * tq, tb)]
    fq = stage1 + [lambda rel: None] + stage2
    u_first = T - 2 * n + p
    for u in range(u_first, T - 1):
        i = u - 1 - (T - n)
        vpu, nv, nf = gates, [1, 1, 0, 0, 0, 0, 1, 1, 1, 1], [1] * 6 + [1 if i < late - 2 else 2] * 4
        if u == u_first:
            nv, nf = [0, 0, 0, 0, 0, 2, 2, 2, 2, 0], [0] * 6 + [1] * 4
        if i > late:
            vpu, nv = fins, [2, 2, 1, 1]
        jobs = [[vpu.pop(0) for _ in range(min(len(vpu), a))] + [fq.pop(0) for _ in range(min(len(fq), b))]
                for a, b in zip(nv + [0] * 10, nf)]
        before = [None] * R
        if i >= late:
            assert not fq and not gates
            before[2] = functools.partial(stored, ob_ref, i * tq, z)
        state = round_(u, u, state, z, "final" if i >= late else "acc", jobs, before,
                       mid=(lambda: scatter(done[0])) if i == late else None)
    assert not fins
    m, o, lp = state
    sl, hq = slot(T - 1), tq // 2
    oa, lpa = pv(T - 1, sl, m[:hq], o[:hq], z, before=[lambda: done2[0], None, None, None], lag=2)
    gate = wo(n - 2, sl, o, lp, "final")
    cp_out(n - 2, z).start()
    ob, lpb = pv(T - 1, sl, m[hq:], gate[:hq], z, off=hq, lag=2,
                 before=[None, None, None, functools.partial(stored, ob_ref, (n - 2) * tq, z)])
    wo(n - 1, sl, oa, lpa, "final")
    cp_out(n - 1, z).start()
    wo(n - 1, sl, ob, lpb, "final", off=hq)
    cp_out(n, z).start()
    for i in range(n + 1):
        cp_out(i, z).wait()


@jax.jit
def pallas_recurrent_scan__mha_block_cached__moe_arch_mod__prompt_kernel(
    A_x: jax.Array,
    A_k_cache: jax.Array,
    A_v_cache: jax.Array,
    A_wq: jax.Array,
    A_wo: jax.Array,
    B_x: jax.Array,
    B_w_r: jax.Array,
    B_w_gate: jax.Array,
    B_w_up: jax.Array,
    B_w_down: jax.Array,
):
    B, S, D = A_x.shape
    _, H, Sk, Dh = A_k_cache.shape
    F = B_w_gate.shape[1]
    assert B == 1 and Sk == S and S % _TQ == 0 and S % _CW == 0 and Dh == 128 and D % 512 == 128
    n = S // _TQ
    assert n == 8 and _P == n - 1 and (H - 2) * n % _L == 0 and _L == 12 and _NS == 4 and S == 2048 and F % _CW == 192
    hbm = pl.BlockSpec(memory_space=pltpu.HBM)
    out = pl.pallas_call(
        functools.partial(_kernel, S=S, D=D, Dh=Dh, H=H),
        grid=(1,),
        in_specs=[hbm] * 9,
        out_specs=pl.BlockSpec(memory_space=pl.ANY),
        out_shape=jax.ShapeDtypeStruct((S, D), _BF16),
        scratch_shapes=[
            pltpu.VMEM((S, D), _BF16),
            pltpu.VMEM((S // 2, D), jnp.uint32),
            pltpu.VMEM((S, D), _F32),
            pltpu.VMEM((S, D), _F32),
            pltpu.VMEM((S, D), _BF16),
            pltpu.VMEM((2, _TQ, S), _F32),
            pltpu.VMEM((_TQ, 128), _F32),
            pltpu.VMEM((_TQ, Dh), _F32),
            pltpu.VMEM((_TQ, 128), _F32),
            pltpu.VMEM((_NS, 2 * S + 2 * D, Dh), _BF16),
            pltpu.VMEM((F, D), _BF16),
            pltpu.VMEM((F, D), _BF16),
            pltpu.VMEM((F, D), _BF16),
            pltpu.VMEM((D,), _BF16),
            pltpu.SMEM((_TOPC,), _I32),
            pltpu.SMEM((1,), _I32),
            pltpu.SemaphoreType.DMA((_NS + 4 + 2 * n + 5,)),
        ],
        compiler_params=pltpu.CompilerParams(
            dimension_semantics=("arbitrary",),
            vmem_limit_bytes=100 * 1024 * 1024,
            disable_bounds_checks=True,
            disable_semaphore_checks=True,
            internal_scratch_in_bytes=64 * 1024,
        ),
    )(A_x.reshape(S, D), A_k_cache.reshape(H, Sk, Dh), A_v_cache.reshape(H, Sk, Dh), A_wq, A_wo,
      B_w_r, B_w_gate.T, B_w_up.T, B_w_down)
    return out.reshape(B, S, D)
```

```python
import functools
import math

import jax
import jax.numpy as jnp
import jax.experimental.pallas as pl
import jax.experimental.pallas.tpu as pltpu

_F32 = jnp.float32
_BF16 = jnp.bfloat16
_I32 = jnp.int32
_NT = (((1,), (1,)), ((), ()))

_TOPC = 8
_EPS = 1e-5
_TQ = 256
_CW = 512
_P = 7
_L = 12
_NS = 4


def _bf(x):
    return x.astype(_BF16).astype(_F32)


def _silu(x):
    h = 0.5 * x
    return h + h * jnp.tanh(h)


def _sigmoid(x):
    return 0.5 + 0.5 * jnp.tanh(0.5 * x)


def _after(gate, val):
    return jnp.where(gate > jnp.inf, 0.0, val)


def _after16(gate, val):
    g = gate > jnp.inf
    g = jnp.concatenate([g[r:r + 8] for r in range(8, gate.shape[0], 16) for _ in range(2)], axis=0)
    return jnp.where(g, 0.0, val)


def _kernel(x_hbm, k_hbm, v_hbm, wq_hbm, wo_hbm, wr_hbm, wg_hbm, wu_hbm, wd_hbm,
            out_hbm,
            x_ref, xnp_ref, z_ref, acc_ref, ob_ref, s_ref, mc_ref, oc_ref, lc_ref,
            hb, wg_ref, wu_ref, wd_ref, wr_ref, sel_ref, zs,
            sems,
            *, S, D, Dh, H):
    tq, cw, p, L, NS = _TQ, _CW, _P, _L, _NS
    n = S // tq
    R = S // cw
    tb = tq // 4
    D4 = (D // 512) * 512
    F = wd_ref.shape[0]
    scale = (Dh ** -0.5) * math.log2(math.e)
    xn_ref = xnp_ref.bitcast(_BF16)

    K0, V0, Q0, O0 = 0, S, 2 * S, 2 * S + D

    def hcol(h):
        return pl.ds(pl.multiple_of(h * Dh, Dh), Dh)

    def cp_k(h, slot, sem):
        return (pltpu.make_async_copy(k_hbm.at[h], hb.at[slot, K0:K0 + S], sems.at[sem]),)

    def cp_v(h, slot, sem):
        return (pltpu.make_async_copy(v_hbm.at[h], hb.at[slot, V0:V0 + S], sems.at[sem]),)

    def cp_wq(h, slot, sem):
        return (pltpu.make_async_copy(wq_hbm.at[:, hcol(h)], hb.at[slot, Q0:Q0 + D], sems.at[sem]),)

    def cp_wo(h, slot, sem):
        return tuple(pltpu.make_async_copy(wo_hbm.at[hcol(h), c:c + 128], hb.at[slot, O0 + c:O0 + c + 128],
                                           sems.at[sem]) for c in range(0, D, 128))

    def start_head(h, slot):
        for cp in (cp_wq, cp_k, cp_v, cp_wo):
            for c in cp(h, slot, slot):
                c.start()

    def wait_head(slot):
        pltpu.make_async_copy(hb.at[slot], hb.at[slot], sems.at[slot]).wait()

    def cp_x(i):
        return pltpu.make_async_copy(x_hbm.at[rs(i * tq, tq), :], x_ref.at[rs(i * tq, tq), :],
                                     sems.at[NS + 4 + i])

    def cp_out(i, z):
        r0, nr = (i * tq, tq) if i < n - 1 else ((n - 1) * tq + (i - n + 1) * tq // 2, tq // 2)
        src = pl.ds(pl.multiple_of(z * tq + r0, tb), nr)
        return pltpu.make_async_copy(ob_ref.at[src, :], out_hbm.at[pl.ds(r0, nr), :], sems.at[NS + 4 + n + i])

    def cp_ffn():
        return (pltpu.make_async_copy(wg_hbm, wg_ref, sems.at[NS + 4 + 2 * n + 4]),
                pltpu.make_async_copy(wu_hbm, wu_ref, sems.at[NS + 4 + 2 * n + 1]),
                pltpu.make_async_copy(wd_hbm, wd_ref, sems.at[NS + 4 + 2 * n + 2]))

    def cp_wr():
        return pltpu.make_async_copy(wr_hbm, wr_ref, sems.at[NS + 4 + 2 * n + 3])

    def lanes(v, k):
        return jnp.concatenate([v] * k, axis=1)

    def rows(v, k):
        return jnp.concatenate([v] * k, axis=0)

    def rs(r0, nr):
        return slice(r0, r0 + nr) if isinstance(r0, int) else pl.ds(pl.multiple_of(r0, tb), nr)

    def fold(v):
        t = v[:, 0:128]
        for j in range(1, v.shape[1] // 128):
            t = t + v[:, j * 128:(j + 1) * 128]
        return t

    def compact(col, g0, init):
        lane = jax.lax.broadcasted_iota(_I32, init.shape, 1) - g0
        for g in range(col.shape[0] // 8):
            init = jnp.where(lane == g, col[8 * g:8 * g + 8, :], init)
        return init

    def side(jobs, res):
        for k, f in enumerate(jobs or []):
            r0 = min(k * res.shape[0] // len(jobs) // 8 * 8, res.shape[0] - tb)
            f(res[r0:r0 + tb, 0:128])

    def stored(ref, r0, z):
        k = 32 // (8 * ref.dtype.itemsize)
        v = ref[pl.ds(pl.multiple_of(z * 8 * k + r0, 8 * k), 8 * k), 0:128]
        return v if k == 1 else pltpu.bitcast(v, _F32)

    def qproj(i, slot, jobs=None):
        w = hb.at[slot, Q0:Q0 + D]
        xv = xn_ref.at[rs(i * tq, tq)]
        q = jnp.dot(xv[:, 0:D4], w[0:D4, :], preferred_element_type=_F32)
        q = q + jnp.concatenate(
            [jnp.dot(xv[t * tb:(t + 1) * tb, D4:D], w[D4:D, :], preferred_element_type=_F32)
             for t in range(4)], axis=0)
        side(jobs, q)
        return (q * scale).astype(_BF16)

    def rowmax(mx):
        return jnp.broadcast_to(jnp.max(mx, axis=-1, keepdims=True), (tq, 128))

    def qk(par, slot, q, z, jobs=None, lanewise=False):
        if jobs is None and not lanewise:
            s = jax.lax.dot_general(q, hb[slot, K0:K0 + S], _NT, preferred_element_type=_F32)
            s_ref[z + par % 2] = s
            return rowmax(s)
        mx = None
        for c in range(R):
            s = jax.lax.dot_general(q, hb[slot, K0 + c * cw:K0 + (c + 1) * cw], _NT, preferred_element_type=_F32)
            s_ref[z + par % 2, :, c * cw:(c + 1) * cw] = s
            for j in range(cw // 128):
                sj = s[:, j * 128:(j + 1) * 128]
                mx = sj if mx is None else jnp.maximum(mx, sj)
            side(jobs and jobs[c], s)
        return mx if lanewise else rowmax(mx)

    def finalize(r0, nr, c0, c1, s):
        out = x_ref[r0:r0 + nr, c0:c1].astype(_F32) + s * z_ref[r0:r0 + nr, c0:c1]
        ob_ref[r0:r0 + nr, c0:c1] = out.astype(_BF16)
        return out

    def wo(i, slot, o, lp, mode, jobs=None, off=0):
        nq = o.shape[0]
        l = jnp.sum(lp, axis=-1, keepdims=True)
        o32 = o * pl.reciprocal(l, full_range=False)
        o = o32.astype(_BF16)
        w = [hb[slot, O0 + c:O0 + c + 128] for c in range(0, D, 128)]
        av = acc_ref.at[rs(i * tq, tq)]

        def emit(r0, nr, c0, c1, a):
            if mode == "init":
                av[r0:r0 + nr, c0:c1] = a
            elif mode == "acc":
                av[r0:r0 + nr, c0:c1] += a
            else:
                finalize(i * tq + r0, nr, c0, c1, av[r0:r0 + nr, c0:c1] + a)

        a = jnp.dot(o, jnp.concatenate(w[:-1], axis=1), preferred_element_type=_F32)
        emit(off, nq, 0, D4, a)
        side(jobs, a)
        for t in range(0, nq, nq // 4):
            emit(off + t, nq // 4, D4, D,
                 jnp.dot(o32[t:t + nq // 4, :].astype(_BF16), w[-1], preferred_element_type=_F32))
        return a[:, 0:128]

    def pv(par, slot, m, gate, z, jobs=None, before=None, last=False, off=0, lag=1):
        o = lp = None
        gates = [gate] * lag
        for c in range(R):
            mc = m if gates[c] is None else _after16(gates[c], m)
            if before is not None and before[c] is not None:
                mc = _after(rows(before[c](), m.shape[0] // 8), mc)
            sc = s_ref[z + par % 2, off:off + m.shape[0], c * cw:(c + 1) * cw]
            pe = jnp.exp2(sc - lanes(mc, cw // 128))
            ps = [pe[:, j * 128:(j + 1) * 128] for j in range(cw // 128)]
            for pj in ps:
                lp = pj if lp is None else lp + pj
            ps[-1] = jnp.minimum(ps[-1], lp)
            pb = jnp.concatenate(ps, axis=1).astype(_BF16)
            oc = jnp.dot(pb, hb[slot, V0 + c * cw:V0 + (c + 1) * cw], preferred_element_type=_F32)
            side(None if jobs is None else jobs[c], oc)
            o = oc if o is None else o + oc
            gates.append(o)
        return o, (lp if last else _after16(o, lp))

    def layernorm(r0, nr, rt, z, rel=None):
        def x(k):
            k = k if rel is not None else 0
            return x_ref[pl.ds(pl.multiple_of(k * z * tb + r0, tb), nr), :].astype(_F32)
        xs = fold(x(0))
        if rel is not None:
            xs = _after(rel, xs)
        mean = jnp.sum(xs, axis=-1, keepdims=True) * (1.0 / D)
        xc = x(1) - mean
        var = compact(jnp.sum(xc * xc, axis=-1, keepdims=True), 0, jnp.ones((8, 128), _F32)) * (1.0 / D)
        inv = 1.0 / _bf(jnp.sqrt(_bf(_bf(var) + _bf(jnp.float32(_EPS)))))
        inv = jnp.concatenate([jnp.broadcast_to(inv[:, g:g + 1], (8, 128)) for g in range(nr // 8)], axis=0)
        xn = (_bf(x(2) - _bf(mean)) * lanes(inv, D // 128)).astype(_BF16)
        xn_ref[rs(r0, nr), :] = xn
        rp = fold(xn.astype(_F32) * wr_ref[...].astype(_F32).reshape(1, D))
        rt[0] = compact(jnp.sum(rp, axis=-1, keepdims=True), r0 // 8, rt[0])

    def topk(rt):
        rt = _bf(rt)
        lane = jax.lax.broadcasted_iota(_I32, rt.shape, 1)
        sub = jax.lax.broadcasted_iota(_I32, rt.shape, 0)
        top = pltpu.bitcast(jnp.where(rt == 0.0, 0.0, rt), _I32) >> 16
        code = jnp.where(rt != rt, 0, jnp.where(top < 0, -1 - top, top + 32768))
        key = pltpu.bitcast((1 << 29) + code * S + (S - 1 - (lane * 8 + sub)), _F32)
        for c in range(_TOPC):
            kmax = jnp.max(jnp.max(key, axis=0, keepdims=True), axis=1, keepdims=True)
            sel_ref[c] = S - 1 - (pltpu.bitcast(kmax, _I32)[0, 0] & (S - 1))
            key = jnp.where(key == kmax, 0.0, key)

    def pace(v, k, done, rel):
        t = fold(v)
        t = jnp.concatenate([t[j:j + 8] + t[j + 8:j + 16] for j in range(0, v.shape[0], 16)], axis=0)
        if rel is not None:
            t = _after(jnp.concatenate([rel[j:j + 8] for j in range(0, v.shape[0], 16)], axis=0), t)
        done[0] = compact(jnp.sum(t, axis=-1, keepdims=True), k, done[0])

    def gate_piece(r0, nr, done, rel):
        g = _silu(xn_ref[r0:r0 + nr, :].astype(_F32))
        z_ref[r0:r0 + nr, :] = g
        pace(g, r0 // 16, done, rel)

    def fin_piece(r0, nr, done, z, rel):
        s = _after(lanes(rel, D // 128), acc_ref[r0:r0 + nr, :])
        pace(finalize(r0, nr, 0, D, s), r0 // 16, done, None)
        if (r0 + nr) % tq == 0:
            cp_out(r0 // tq, z).start()

    def ffn_jobs():
        st = {}
        F4 = (F // cw) * cw

        def gather():
            rowid = jax.lax.broadcasted_iota(_I32, (_TOPC, 1), 0)
            xs = jnp.zeros((_TOPC, D), _F32)
            for c in range(_TOPC):
                w = xnp_ref[pl.ds(sel_ref[c] // 2, 1), :]
                w = jnp.where(sel_ref[c] % 2 == 0, w << 16, w & jnp.uint32(0xFFFF0000))
                xs = jnp.where(rowid == c, pltpu.bitcast(w, _F32), xs)
            st["xs"], st["xb"] = xs, xs.astype(_BF16)

        def add(key, val):
            st[key] = val if key not in st else st[key] + val

        def up(parts, k, rel):
            xk = st["xb"][:, k * 128:(k + 1) * 128]
            for name, w_ref, c0, c1 in parts:
                add((name, c0), jax.lax.dot_general(xk, w_ref[c0:c1, k * 128:(k + 1) * 128], _NT,
                                                    preferred_element_type=_F32))

        def hidden():
            cuts = list(range(0, F, cw))
            g = _bf(jnp.concatenate([st["g", c] for c in cuts], axis=1))
            u = _bf(jnp.concatenate([st["u", c] for c in cuts], axis=1))
            st["h"] = (_bf(_silu(g)) * u).astype(_BF16)

        def down(cuts, c0, c1, rel):
            if "h" not in st:
                hidden()
            for k0, k1 in zip(cuts[:-1], cuts[1:]):
                add(("y", c0), jnp.dot(st["h"][:, k0:k1], wd_ref[k0:k1, c0:c1], preferred_element_type=_F32))

        def scatter(done):
            xs = _after(lanes(done, D // 128), st["xs"])
            rs = _bf(jnp.sum(fold(xs * wr_ref[...].astype(_F32).reshape(1, D)), axis=-1, keepdims=True))
            y = _bf(jnp.concatenate([st["y", 0], st["y", D4]], axis=1))
            zz = _silu(_bf(xs + _bf(y * _bf(_sigmoid(rs)))))
            for c in range(_TOPC):
                z_ref[pl.ds(sel_ref[c], 1), :] = zz[c:c + 1, :]

        stage1 = []
        for k in range(D // 128):
            for name, w_ref in (("g", wg_ref), ("u", wu_ref)):
                for c0 in range(0, F4, cw):
                    stage1.append(functools.partial(up, [(name, w_ref, c0, c0 + cw)], k))
            stage1.append(functools.partial(up, [("g", wg_ref, F4, F), ("u", wu_ref, F4, F)], k))
        stage2 = [functools.partial(down, [k0, min(k0 + 128, F)], 0, D4) for k0 in range(0, F, 128)]
        stage2 += [functools.partial(down, [k0, k0 + cw], D4, D) for k0 in range(0, F4, cw)]
        stage2 += [functools.partial(down, [F4, F4 + 64, F4 + 128, F4 + 160, F], D4, D)]
        return gather, stage1, stage2, scatter

    def save(state):
        mc_ref[...], oc_ref[...], lc_ref[...] = state

    def load():
        return rowmax(mc_ref[...]), oc_ref[...], lc_ref[...]

    def chunk(u):
        return u % n if isinstance(u, int) else u & (n - 1)

    def slot(u):
        return u // n % NS if isinstance(u, int) else (u >> 3) & (NS - 1)

    def round_(u, par, state, z, mode, jobs=None, before=None, last=False, mid=None, nxt=None):
        m, o, lp = state
        c1, s1 = nxt or (chunk(u + 1), slot(u + 1))
        q = qproj(c1, s1, jobs and jobs[0])
        m_next = qk(par + 1, s1, q, z, jobs and jobs[1:R + 1], lanewise=last)
        if mid is not None:
            mid()
        gate = wo(chunk(u - 1), slot(u - 1), o, lp, mode, jobs and jobs[R + 1])
        if mode == "final":
            cp_out(chunk(u - 1), z).start()
        return (m_next,) + pv(par, slot(u), m, gate, z, jobs and jobs[R + 2:], before, last)

    zs[0] = jnp.minimum(pl.program_id(0), 0)
    wq0, k0, v0, wo0 = (cp(0, 0, NS + t) for t, cp in enumerate((cp_wq, cp_k, cp_v, cp_wo)))
    for c in (cp_wr(), cp_x(0), *wq0, cp_x(1), *k0, cp_x(2), *v0, *wo0, *(cp_x(i) for i in range(3, n))):
        c.start()
    start_head(1, 1)
    start_head(2, 2)
    for c in cp_ffn():
        c.start()
    @pl.loop(0, (S - (p - 1) * tq) // 32)
    def _(i):
        acc_ref[pl.ds(pl.multiple_of((p - 1) * tq + i * 32, 32), 32), :] = jnp.zeros((32, D), _F32)

    cp_x(0).wait()
    cp_wr().wait()
    z = zs[0]
    rt = [jnp.zeros((8, S // 8), _F32)]

    def ln_jobs(i, z, spread):
        pieces = [functools.partial(layernorm, i * tq + t * tb, tb, rt, z) for t in range(4)]
        return [[pieces.pop(0) for _ in range(k)] for k in spread]

    for f in ln_jobs(0, z, [4])[0]:
        f()
    wq0[0].wait()
    cp_x(1).wait()
    q0 = qproj(0, 0)
    for f in ln_jobs(1, z, [4])[0]:
        f()
    q1 = qproj(1, 0)
    k0[0].wait()
    m0 = qk(0, 0, q0, z, lanewise=True)
    cp_x(2).wait()
    m0 = rowmax(m0)
    m1 = qk(1, 0, q1, z, ln_jobs(2, z, [3, 1, 0, 0]), lanewise=True)
    v0[0].wait()
    save((m1,) + pv(0, 0, m0, None, z, last=True))
    for c in wo0:
        c.wait()

    def pair(j, rt_in):
        for k in range(2):
            pl.when(3 + 2 * j + k < n)(lambda: cp_x(jnp.minimum(3 + 2 * j + k, n - 1)).wait())
        z = zs[0]
        rt[0] = rt_in
        state = load()
        for k in range(2):
            u = 1 + 2 * j + k
            jobs = ln_jobs(jnp.minimum(u + 2, n - 1), z, [1, 1, 1, 1, 0, 0, 0, 0, 0, 0])
            state = round_(u, 1 + k, state, z, "init", jobs, last=(k == 1))
        save(state)
        return rt[0]

    scores = jax.lax.fori_loop(0, (p - 1) // 2, pair, rt[0])

    def entry(u0):
        h0 = (u0 >> 3) + 1
        return (u0, h0 & (NS - 1), (h0 + 1) & (NS - 1), ((u0 + L) >> 3) - h0, chunk(u0 + 1), slot(u0 + 1))

    def body(j, carry):
        u0, w1, w2, two, c1, s1 = carry
        wait_head(w1)
        pl.when(two > 0)(lambda: wait_head(w2))
        z = zs[0]

        def prefetch():
            h1 = ((u0 + L) >> 3) + 1
            start_head(h1, h1 & (NS - 1))
            pl.when(h1 + 1 <= jnp.minimum((u0 + 2 * L) >> 3, H - 1))(
                lambda: start_head(h1 + 1, (h1 + 1) & (NS - 1)))

        state = load()
        for k in range(L):
            state = round_(u0 + k, p + k, state, z, "acc", last=(k == L - 1), mid=prefetch if k == 1 else None,
                           nxt=(c1, s1) if k == 0 else None)
        save(state)
        return entry(u0 + L)

    T = H * n
    jax.lax.fori_loop(0, (T - 2 * n) // L, body, entry(jnp.int32(p)))

    wait_head((H - 1) % NS)
    for c in cp_ffn():
        c.wait()
    z = zs[0]
    state = load()
    gather, stage1, stage2, scatter = ffn_jobs()
    topk(scores)
    gather()
    done, done2 = [jnp.zeros((8, 128), _F32)], [jnp.zeros((8, 128), _F32)]
    late = 3
    gates = [functools.partial(gate_piece, r0, tb, done) for r0 in range(0, S, tb)]
    fins = [functools.partial(fin_piece, r0, tb, done2, z) for r0 in range(0, late * tq, tb)]
    fq = stage1 + [lambda rel: None] + stage2
    u_first = T - 2 * n + p
    for u in range(u_first, T - 1):
        i = u - 1 - (T - n)
        vpu, nv, nf = gates, [1, 1, 0, 0, 0, 0, 1, 1, 1, 1], [1] * 6 + [1 if i < late - 2 else 2] * 4
        if u == u_first:
            nv, nf = [0, 0, 0, 0, 0, 2, 2, 2, 2, 0], [0] * 6 + [1] * 4
        if i > late:
            vpu, nv = fins, [2, 2, 1, 1]
        jobs = [[vpu.pop(0) for _ in range(min(len(vpu), a))] + [fq.pop(0) for _ in range(min(len(fq), b))]
                for a, b in zip(nv + [0] * 10, nf)]
        before = [None] * R
        if i >= late:
            assert not fq and not gates
            before[2] = functools.partial(stored, ob_ref, i * tq, z)
        state = round_(u, u, state, z, "final" if i >= late else "acc", jobs, before,
                       mid=(lambda: scatter(done[0])) if i == late else None)
    assert not fins
    m, o, lp = state
    sl, hq = slot(T - 1), tq // 2
    oa, lpa = pv(T - 1, sl, m[:hq], o[:hq], z, before=[lambda: done2[0], None, None, None], lag=2)
    gate = wo(n - 2, sl, o, lp, "final")
    cp_out(n - 2, z).start()
    ob, lpb = pv(T - 1, sl, m[hq:], gate[:hq], z, off=hq, lag=2,
                 before=[None, None, None, functools.partial(stored, ob_ref, (n - 2) * tq, z)])
    wo(n - 1, sl, oa, lpa, "final")
    cp_out(n - 1, z).start()
    wo(n - 1, sl, ob, lpb, "final", off=hq)
    cp_out(n, z).start()
    for i in range(n + 1):
        cp_out(i, z).wait()


@jax.jit
def pallas_recurrent_scan__mha_block_cached__moe_arch_mod__prompt_kernel(
    A_x: jax.Array,
    A_k_cache: jax.Array,
    A_v_cache: jax.Array,
    A_wq: jax.Array,
    A_wo: jax.Array,
    B_x: jax.Array,
    B_w_r: jax.Array,
    B_w_gate: jax.Array,
    B_w_up: jax.Array,
    B_w_down: jax.Array,
):
    B, S, D = A_x.shape
    _, H, Sk, Dh = A_k_cache.shape
    F = B_w_gate.shape[1]
    assert B == 1 and Sk == S and S % _TQ == 0 and S % _CW == 0 and Dh == 128 and D % 512 == 128
    n = S // _TQ
    assert n == 8 and _P == n - 1 and (H - 2) * n % _L == 0 and _L == 12 and _NS == 4 and S == 2048 and F % _CW == 192
    hbm = pl.BlockSpec(memory_space=pltpu.HBM)
    out = pl.pallas_call(
        functools.partial(_kernel, S=S, D=D, Dh=Dh, H=H),
        grid=(1,),
        in_specs=[hbm] * 9,
        out_specs=pl.BlockSpec(memory_space=pl.ANY),
        out_shape=jax.ShapeDtypeStruct((S, D), _BF16),
        scratch_shapes=[
            pltpu.VMEM((S, D), _BF16),
            pltpu.VMEM((S // 2, D), jnp.uint32),
            pltpu.VMEM((S, D), _F32),
            pltpu.VMEM((S, D), _F32),
            pltpu.VMEM((S, D), _BF16),
            pltpu.VMEM((2, _TQ, S), _F32),
            pltpu.VMEM((_TQ, 128), _F32),
            pltpu.VMEM((_TQ, Dh), _F32),
            pltpu.VMEM((_TQ, 128), _F32),
            pltpu.VMEM((_NS, 2 * S + 2 * D, Dh), _BF16),
            pltpu.VMEM((F, D), _BF16),
            pltpu.VMEM((F, D), _BF16),
            pltpu.VMEM((F, D), _BF16),
            pltpu.VMEM((D,), _BF16),
            pltpu.SMEM((_TOPC,), _I32),
            pltpu.SMEM((1,), _I32),
            pltpu.SemaphoreType.DMA((_NS + 4 + 2 * n + 5,)),
        ],
        compiler_params=pltpu.CompilerParams(
            dimension_semantics=("arbitrary",),
            vmem_limit_bytes=100 * 1024 * 1024,
            disable_bounds_checks=True,
            disable_semaphore_checks=True,
            internal_scratch_in_bytes=64 * 1024,
        ),
    )(A_x.reshape(S, D), A_k_cache.reshape(H, Sk, Dh), A_v_cache.reshape(H, Sk, Dh), A_wq, A_wo,
      B_w_r, B_w_gate.T, B_w_up.T, B_w_down)
    return out.reshape(B, S, D)
```

```python
import functools
import math

import jax
import jax.numpy as jnp
import jax.experimental.pallas as pl
import jax.experimental.pallas.tpu as pltpu

_F32 = jnp.float32
_BF16 = jnp.bfloat16
_I32 = jnp.int32
_NT = (((1,), (1,)), ((), ()))

_TOPC = 8
_EPS = 1e-5
_TQ = 256
_CW = 512
_P = 7
_L = 12
_NS = 4


def _bf(x):
    return x.astype(_BF16).astype(_F32)


def _silu(x):
    h = 0.5 * x
    return h + h * jnp.tanh(h)


def _sigmoid(x):
    return 0.5 + 0.5 * jnp.tanh(0.5 * x)


def _after(gate, val):
    return jnp.where(gate > jnp.inf, 0.0, val)


def _after16(gate, val):
    g = gate > jnp.inf
    g = jnp.concatenate([g[r:r + 8] for r in range(8, gate.shape[0], 16) for _ in range(2)], axis=0)
    return jnp.where(g, 0.0, val)


def _kernel(x_hbm, k_hbm, v_hbm, wq_hbm, wo_hbm, wr_hbm, wg_hbm, wu_hbm, wd_hbm,
            out_hbm,
            x_ref, xnp_ref, z_ref, acc_ref, ob_ref, s_ref, mc_ref, oc_ref, lc_ref,
            hb, wg_ref, wu_ref, wd_ref, wr_ref, sel_ref, zs,
            sems,
            *, S, D, Dh, H):
    tq, cw, p, L, NS = _TQ, _CW, _P, _L, _NS
    n = S // tq
    R = S // cw
    tb = tq // 4
    D4 = (D // 512) * 512
    F = wd_ref.shape[0]
    scale = (Dh ** -0.5) * math.log2(math.e)

    K0, V0, Q0, O0 = 0, S, 2 * S, 2 * S + D

    def hcol(h):
        return pl.ds(pl.multiple_of(h * Dh, Dh), Dh)

    def cp_k(h, slot, sem):
        return (pltpu.make_async_copy(k_hbm.at[h], hb.at[slot, K0:K0 + S], sems.at[sem]),)

    def cp_v(h, slot, sem):
        return (pltpu.make_async_copy(v_hbm.at[h], hb.at[slot, V0:V0 + S], sems.at[sem]),)

    def cp_wq(h, slot, sem):
        return (pltpu.make_async_copy(wq_hbm.at[:, hcol(h)], hb.at[slot, Q0:Q0 + D], sems.at[sem]),)

    def cp_wo(h, slot, sem):
        return tuple(pltpu.make_async_copy(wo_hbm.at[hcol(h), c:c + 128], hb.at[slot, O0 + c:O0 + c + 128],
                                           sems.at[sem]) for c in range(0, D, 128))

    def start_head(h, slot):
        for cp in (cp_wq, cp_k, cp_v, cp_wo):
            for c in cp(h, slot, slot):
                c.start()

    def wait_head(slot):
        pltpu.make_async_copy(hb.at[slot], hb.at[slot], sems.at[slot]).wait()

    def cp_x(i):
        return pltpu.make_async_copy(x_hbm.at[rs(i * tq, tq), :], x_ref.at[rs(i * tq, tq), :],
                                     sems.at[NS + 4 + i])

    def cp_out(i, z):
        r0, nr = (i * tq, tq) if i < n - 1 else ((n - 1) * tq + (i - n + 1) * tq // 2, tq // 2)
        src = pl.ds(pl.multiple_of(z * tq + r0, tb), nr)
        return pltpu.make_async_copy(ob_ref.at[src, :], out_hbm.at[pl.ds(r0, nr), :], sems.at[NS + 4 + n + i])

    def cp_ffn():
        return (pltpu.make_async_copy(wg_hbm, wg_ref, sems.at[NS + 4 + 2 * n + 4]),
                pltpu.make_async_copy(wu_hbm, wu_ref, sems.at[NS + 4 + 2 * n + 1]),
                pltpu.make_async_copy(wd_hbm, wd_ref, sems.at[NS + 4 + 2 * n + 2]))

    def cp_wr():
        return pltpu.make_async_copy(wr_hbm, wr_ref, sems.at[NS + 4 + 2 * n + 3])

    def lanes(v, k):
        return jnp.concatenate([v] * k, axis=1)

    def rows(v, k):
        return jnp.concatenate([v] * k, axis=0)

    def rs(r0, nr):
        return slice(r0, r0 + nr) if isinstance(r0, int) else pl.ds(pl.multiple_of(r0, tb), nr)

    def rs2(r0, nr):
        return slice(r0 // 2, (r0 + nr) // 2) if isinstance(r0, int) else pl.ds(pl.multiple_of(r0 // 2, tb // 2), nr // 2)

    def fold(v):
        t = v[:, 0:128]
        for j in range(1, v.shape[1] // 128):
            t = t + v[:, j * 128:(j + 1) * 128]
        return t

    def compact(col, g0, init):
        lane = jax.lax.broadcasted_iota(_I32, init.shape, 1) - g0
        for g in range(col.shape[0] // 8):
            init = jnp.where(lane == g, col[8 * g:8 * g + 8, :], init)
        return init

    def side(jobs, res):
        for k, f in enumerate(jobs or []):
            r0 = min(k * res.shape[0] // len(jobs) // 8 * 8, res.shape[0] - tb)
            f(res[r0:r0 + tb, 0:128])

    def stored(ref, r0, z):
        k = 32 // (8 * ref.dtype.itemsize)
        v = ref[pl.ds(pl.multiple_of(z * 8 * k + r0, 8 * k), 8 * k), 0:128]
        return v if k == 1 else pltpu.bitcast(v, _F32)

    def qproj(i, slot, jobs=None):
        w = hb.at[slot, Q0:Q0 + D]
        xv = xnp_ref.at[rs2(i * tq, tq)]
        q = jnp.dot(pltpu.bitcast(xv[:, 0:D4], _BF16), w[0:D4, :], preferred_element_type=_F32)
        q = q + jnp.concatenate(
            [jnp.dot(pltpu.bitcast(xv[t * tb // 2:(t + 1) * tb // 2, D4:D], _BF16), w[D4:D, :],
                     preferred_element_type=_F32)
             for t in range(4)], axis=0)
        side(jobs, q)
        return (q * scale).astype(_BF16)

    def rowmax(mx):
        return jnp.broadcast_to(jnp.max(mx, axis=-1, keepdims=True), (tq, 128))

    def qk(par, slot, q, z, jobs=None, lanewise=False):
        if jobs is None and not lanewise:
            s = jax.lax.dot_general(q, hb[slot, K0:K0 + S], _NT, preferred_element_type=_F32)
            s_ref[z + par % 2] = s
            return rowmax(s)
        mx = None
        for c in range(R):
            s = jax.lax.dot_general(q, hb[slot, K0 + c * cw:K0 + (c + 1) * cw], _NT, preferred_element_type=_F32)
            s_ref[z + par % 2, :, c * cw:(c + 1) * cw] = s
            for j in range(cw // 128):
                sj = s[:, j * 128:(j + 1) * 128]
                mx = sj if mx is None else jnp.maximum(mx, sj)
            side(jobs and jobs[c], s)
        return mx if lanewise else rowmax(mx)

    def finalize(r0, nr, c0, c1, s):
        out = x_ref[r0:r0 + nr, c0:c1].astype(_F32) + s * z_ref[r0:r0 + nr, c0:c1]
        ob_ref[r0:r0 + nr, c0:c1] = out.astype(_BF16)
        return out

    def wo(i, slot, o, lp, mode, jobs=None, off=0):
        nq = o.shape[0]
        l = jnp.sum(lp, axis=-1, keepdims=True)
        o32 = o * pl.reciprocal(l, full_range=False)
        o = o32.astype(_BF16)
        w = [hb[slot, O0 + c:O0 + c + 128] for c in range(0, D, 128)]
        av = acc_ref.at[rs(i * tq, tq)]

        def emit(r0, nr, c0, c1, a):
            if mode == "init":
                av[r0:r0 + nr, c0:c1] = a
            elif mode == "acc":
                av[r0:r0 + nr, c0:c1] += a
            else:
                finalize(i * tq + r0, nr, c0, c1, av[r0:r0 + nr, c0:c1] + a)

        a = jnp.dot(o, jnp.concatenate(w[:-1], axis=1), preferred_element_type=_F32)
        emit(off, nq, 0, D4, a)
        side(jobs, a)
        for t in range(0, nq, nq // 4):
            emit(off + t, nq // 4, D4, D,
                 jnp.dot(o32[t:t + nq // 4, :].astype(_BF16), w[-1], preferred_element_type=_F32))
        return a[:, 0:128]

    def pv(par, slot, m, gate, z, jobs=None, before=None, last=False, off=0, lag=1):
        o = lp = None
        gates = [gate] * lag
        for c in range(R):
            mc = m if gates[c] is None else _after16(gates[c], m)
            if before is not None and before[c] is not None:
                mc = _after(rows(before[c](), m.shape[0] // 8), mc)
            sc = s_ref[z + par % 2, off:off + m.shape[0], c * cw:(c + 1) * cw]
            pe = jnp.exp2(sc - lanes(mc, cw // 128))
            ps = [pe[:, j * 128:(j + 1) * 128] for j in range(cw // 128)]
            for pj in ps:
                lp = pj if lp is None else lp + pj
            ps[-1] = jnp.minimum(ps[-1], lp)
            pb = jnp.concatenate(ps, axis=1).astype(_BF16)
            oc = jnp.dot(pb, hb[slot, V0 + c * cw:V0 + (c + 1) * cw], preferred_element_type=_F32)
            side(None if jobs is None else jobs[c], oc)
            o = oc if o is None else o + oc
            gates.append(o)
        return o, (lp if last else _after16(o, lp))

    def layernorm(r0, nr, rt, z, rel=None):
        def x(k):
            k = k if rel is not None else 0
            return x_ref[pl.ds(pl.multiple_of(k * z * tb + r0, tb), nr), :].astype(_F32)
        xs = fold(x(0))
        if rel is not None:
            xs = _after(rel, xs)
        mean = jnp.sum(xs, axis=-1, keepdims=True) * (1.0 / D)
        xc = x(1) - mean
        var = compact(jnp.sum(xc * xc, axis=-1, keepdims=True), 0, jnp.ones((8, 128), _F32)) * (1.0 / D)
        inv = 1.0 / _bf(jnp.sqrt(_bf(_bf(var) + _bf(jnp.float32(_EPS)))))
        inv = jnp.concatenate([jnp.broadcast_to(inv[:, g:g + 1], (8, 128)) for g in range(nr // 8)], axis=0)
        xn = (_bf(x(2) - _bf(mean)) * lanes(inv, D // 128)).astype(_BF16)
        xnp_ref[rs2(r0, nr), :] = pltpu.bitcast(xn, jnp.uint32)
        rp = fold(xn.astype(_F32) * wr_ref[...].astype(_F32).reshape(1, D))
        rt[0] = compact(jnp.sum(rp, axis=-1, keepdims=True), r0 // 8, rt[0])

    def topk(rt):
        rt = _bf(rt)
        lane = jax.lax.broadcasted_iota(_I32, rt.shape, 1)
        sub = jax.lax.broadcasted_iota(_I32, rt.shape, 0)
        top = pltpu.bitcast(jnp.where(rt == 0.0, 0.0, rt), _I32) >> 16
        code = jnp.where(rt != rt, 0, jnp.where(top < 0, -1 - top, top + 32768))
        key = pltpu.bitcast((1 << 29) + code * S + (S - 1 - (lane * 8 + sub)), _F32)
        for c in range(_TOPC):
            kmax = jnp.max(jnp.max(key, axis=0, keepdims=True), axis=1, keepdims=True)
            sel_ref[c] = S - 1 - (pltpu.bitcast(kmax, _I32)[0, 0] & (S - 1))
            key = jnp.where(key == kmax, 0.0, key)

    def pace(v, k, done, rel):
        t = fold(v)
        t = jnp.concatenate([t[j:j + 8] + t[j + 8:j + 16] for j in range(0, v.shape[0], 16)], axis=0)
        if rel is not None:
            t = _after(jnp.concatenate([rel[j:j + 8] for j in range(0, v.shape[0], 16)], axis=0), t)
        done[0] = compact(jnp.sum(t, axis=-1, keepdims=True), k, done[0])

    def gate_piece(r0, nr, done, rel):
        g = _silu(pltpu.bitcast(xnp_ref[rs2(r0, nr), :], _BF16).astype(_F32))
        z_ref[r0:r0 + nr, :] = g
        pace(g, r0 // 16, done, rel)

    def fin_piece(r0, nr, done, z, rel):
        s = _after(lanes(rel, D // 128), acc_ref[r0:r0 + nr, :])
        pace(finalize(r0, nr, 0, D, s), r0 // 16, done, None)
        if (r0 + nr) % tq == 0:
            cp_out(r0 // tq, z).start()

    def ffn_jobs():
        st = {}
        F4 = (F // cw) * cw

        def gather():
            rowid = jax.lax.broadcasted_iota(_I32, (_TOPC, 1), 0)
            xs = jnp.zeros((_TOPC, D), _F32)
            for c in range(_TOPC):
                w = xnp_ref[pl.ds(sel_ref[c] // 2, 1), :]
                w = jnp.where(sel_ref[c] % 2 == 0, w << 16, w & jnp.uint32(0xFFFF0000))
                xs = jnp.where(rowid == c, pltpu.bitcast(w, _F32), xs)
            st["xs"], st["xb"] = xs, xs.astype(_BF16)

        def add(key, val):
            st[key] = val if key not in st else st[key] + val

        def up(parts, k, rel):
            xk = st["xb"][:, k * 128:(k + 1) * 128]
            for name, w_ref, c0, c1 in parts:
                add((name, c0), jax.lax.dot_general(xk, w_ref[c0:c1, k * 128:(k + 1) * 128], _NT,
                                                    preferred_element_type=_F32))

        def hidden():
            cuts = list(range(0, F, cw))
            g = _bf(jnp.concatenate([st["g", c] for c in cuts], axis=1))
            u = _bf(jnp.concatenate([st["u", c] for c in cuts], axis=1))
            st["h"] = (_bf(_silu(g)) * u).astype(_BF16)

        def down(cuts, c0, c1, rel):
            if "h" not in st:
                hidden()
            for k0, k1 in zip(cuts[:-1], cuts[1:]):
                add(("y", c0), jnp.dot(st["h"][:, k0:k1], wd_ref[k0:k1, c0:c1], preferred_element_type=_F32))

        def scatter(done):
            xs = _after(lanes(done, D // 128), st["xs"])
            rs = _bf(jnp.sum(fold(xs * wr_ref[...].astype(_F32).reshape(1, D)), axis=-1, keepdims=True))
            y = _bf(jnp.concatenate([st["y", 0], st["y", D4]], axis=1))
            zz = _silu(_bf(xs + _bf(y * _bf(_sigmoid(rs)))))
            for c in range(_TOPC):
                z_ref[pl.ds(sel_ref[c], 1), :] = zz[c:c + 1, :]

        stage1 = []
        for k in range(D // 128):
            for name, w_ref in (("g", wg_ref), ("u", wu_ref)):
                for c0 in range(0, F4, cw):
                    stage1.append(functools.partial(up, [(name, w_ref, c0, c0 + cw)], k))
            stage1.append(functools.partial(up, [("g", wg_ref, F4, F), ("u", wu_ref, F4, F)], k))
        stage2 = [functools.partial(down, [k0, min(k0 + 128, F)], 0, D4) for k0 in range(0, F, 128)]
        stage2 += [functools.partial(down, [k0, k0 + cw], D4, D) for k0 in range(0, F4, cw)]
        stage2 += [functools.partial(down, [F4, F4 + 64, F4 + 128, F4 + 160, F], D4, D)]
        return gather, stage1, stage2, scatter

    def save(state):
        mc_ref[...], oc_ref[...], lc_ref[...] = state

    def load():
        return rowmax(mc_ref[...]), oc_ref[...], lc_ref[...]

    def chunk(u):
        return u % n if isinstance(u, int) else u & (n - 1)

    def slot(u):
        return u // n % NS if isinstance(u, int) else (u >> 3) & (NS - 1)

    def round_(u, par, state, z, mode, jobs=None, before=None, last=False, mid=None, nxt=None):
        m, o, lp = state
        c1, s1 = nxt or (chunk(u + 1), slot(u + 1))
        q = qproj(c1, s1, jobs and jobs[0])
        m_next = qk(par + 1, s1, q, z, jobs and jobs[1:R + 1], lanewise=last)
        if mid is not None:
            mid()
        gate = wo(chunk(u - 1), slot(u - 1), o, lp, mode, jobs and jobs[R + 1])
        if mode == "final":
            cp_out(chunk(u - 1), z).start()
        return (m_next,) + pv(par, slot(u), m, gate, z, jobs and jobs[R + 2:], before, last)

    zs[0] = jnp.minimum(pl.program_id(0), 0)
    wq0, k0, v0, wo0 = (cp(0, 0, NS + t) for t, cp in enumerate((cp_wq, cp_k, cp_v, cp_wo)))
    for c in (cp_wr(), cp_x(0), *wq0, cp_x(1), *k0, cp_x(2), *v0, *wo0, *(cp_x(i) for i in range(3, n))):
        c.start()
    start_head(1, 1)
    start_head(2, 2)
    for c in cp_ffn():
        c.start()
    @pl.loop(0, (S - (p - 1) * tq) // 32)
    def _(i):
        acc_ref[pl.ds(pl.multiple_of((p - 1) * tq + i * 32, 32), 32), :] = jnp.zeros((32, D), _F32)

    cp_x(0).wait()
    cp_wr().wait()
    z = zs[0]
    rt = [jnp.zeros((8, S // 8), _F32)]

    def ln_jobs(i, z, spread):
        pieces = [functools.partial(layernorm, i * tq + t * tb, tb, rt, z) for t in range(4)]
        return [[pieces.pop(0) for _ in range(k)] for k in spread]

    for f in ln_jobs(0, z, [4])[0]:
        f()
    wq0[0].wait()
    cp_x(1).wait()
    q0 = qproj(0, 0)
    for f in ln_jobs(1, z, [4])[0]:
        f()
    q1 = qproj(1, 0)
    k0[0].wait()
    m0 = qk(0, 0, q0, z, lanewise=True)
    cp_x(2).wait()
    m0 = rowmax(m0)
    m1 = qk(1, 0, q1, z, ln_jobs(2, z, [3, 1, 0, 0]), lanewise=True)
    v0[0].wait()
    save((m1,) + pv(0, 0, m0, None, z, last=True))
    for c in wo0:
        c.wait()

    def pair(j, rt_in):
        for k in range(2):
            pl.when(3 + 2 * j + k < n)(lambda: cp_x(jnp.minimum(3 + 2 * j + k, n - 1)).wait())
        z = zs[0]
        rt[0] = rt_in
        state = load()
        for k in range(2):
            u = 1 + 2 * j + k
            jobs = ln_jobs(jnp.minimum(u + 2, n - 1), z, [1, 1, 1, 1, 0, 0, 0, 0, 0, 0])
            state = round_(u, 1 + k, state, z, "init", jobs, last=(k == 1))
        save(state)
        return rt[0]

    scores = jax.lax.fori_loop(0, (p - 1) // 2, pair, rt[0])

    def entry(u0):
        h0 = (u0 >> 3) + 1
        return (u0, h0 & (NS - 1), (h0 + 1) & (NS - 1), ((u0 + L) >> 3) - h0, chunk(u0 + 1), slot(u0 + 1))

    def body(j, carry):
        u0, w1, w2, two, c1, s1 = carry
        wait_head(w1)
        pl.when(two > 0)(lambda: wait_head(w2))
        z = zs[0]

        def prefetch():
            h1 = ((u0 + L) >> 3) + 1
            start_head(h1, h1 & (NS - 1))
            pl.when(h1 + 1 <= jnp.minimum((u0 + 2 * L) >> 3, H - 1))(
                lambda: start_head(h1 + 1, (h1 + 1) & (NS - 1)))

        state = load()
        for k in range(L):
            state = round_(u0 + k, p + k, state, z, "acc", last=(k == L - 1), mid=prefetch if k == 1 else None,
                           nxt=(c1, s1) if k == 0 else None)
        save(state)
        return entry(u0 + L)

    T = H * n
    jax.lax.fori_loop(0, (T - 2 * n) // L, body, entry(jnp.int32(p)))

    wait_head((H - 1) % NS)
    for c in cp_ffn():
        c.wait()
    z = zs[0]
    state = load()
    gather, stage1, stage2, scatter = ffn_jobs()
    topk(scores)
    gather()
    done, done2 = [jnp.zeros((8, 128), _F32)], [jnp.zeros((8, 128), _F32)]
    late = 3
    gates = [functools.partial(gate_piece, r0, tb, done) for r0 in range(0, S, tb)]
    fins = [functools.partial(fin_piece, r0, tb, done2, z) for r0 in range(0, late * tq, tb)]
    fq = stage1 + [lambda rel: None] + stage2
    u_first = T - 2 * n + p
    for u in range(u_first, T - 1):
        i = u - 1 - (T - n)
        vpu, nv, nf = gates, [1, 1, 0, 0, 0, 0, 1, 1, 1, 1], [1] * 6 + [1 if i < late - 2 else 2] * 4
        if u == u_first:
            nv, nf = [0, 0, 0, 0, 0, 2, 2, 2, 2, 0], [0] * 6 + [1] * 4
        if i > late:
            vpu, nv = fins, [2, 2, 1, 1]
        jobs = [[vpu.pop(0) for _ in range(min(len(vpu), a))] + [fq.pop(0) for _ in range(min(len(fq), b))]
                for a, b in zip(nv + [0] * 10, nf)]
        before = [None] * R
        if i >= late:
            assert not fq and not gates
            before[2] = functools.partial(stored, ob_ref, i * tq, z)
        state = round_(u, u, state, z, "final" if i >= late else "acc", jobs, before,
                       mid=(lambda: scatter(done[0])) if i == late else None)
    assert not fins
    m, o, lp = state
    sl, hq = slot(T - 1), tq // 2
    oa, lpa = pv(T - 1, sl, m[:hq], o[:hq], z, before=[lambda: done2[0], None, None, None], lag=2)
    gate = wo(n - 2, sl, o, lp, "final")
    cp_out(n - 2, z).start()
    ob, lpb = pv(T - 1, sl, m[hq:], gate[:hq], z, off=hq, lag=2,
                 before=[None, None, None, functools.partial(stored, ob_ref, (n - 2) * tq, z)])
    wo(n - 1, sl, oa, lpa, "final")
    cp_out(n - 1, z).start()
    wo(n - 1, sl, ob, lpb, "final", off=hq)
    cp_out(n, z).start()
    for i in range(n + 1):
        cp_out(i, z).wait()


@jax.jit
def pallas_recurrent_scan__mha_block_cached__moe_arch_mod__prompt_kernel(
    A_x: jax.Array,
    A_k_cache: jax.Array,
    A_v_cache: jax.Array,
    A_wq: jax.Array,
    A_wo: jax.Array,
    B_x: jax.Array,
    B_w_r: jax.Array,
    B_w_gate: jax.Array,
    B_w_up: jax.Array,
    B_w_down: jax.Array,
):
    B, S, D = A_x.shape
    _, H, Sk, Dh = A_k_cache.shape
    F = B_w_gate.shape[1]
    assert B == 1 and Sk == S and S % _TQ == 0 and S % _CW == 0 and Dh == 128 and D % 512 == 128
    n = S // _TQ
    assert n == 8 and _P == n - 1 and (H - 2) * n % _L == 0 and _L == 12 and _NS == 4 and S == 2048 and F % _CW == 192
    hbm = pl.BlockSpec(memory_space=pltpu.HBM)
    out = pl.pallas_call(
        functools.partial(_kernel, S=S, D=D, Dh=Dh, H=H),
        grid=(1,),
        in_specs=[hbm] * 9,
        out_specs=pl.BlockSpec(memory_space=pl.ANY),
        out_shape=jax.ShapeDtypeStruct((S, D), _BF16),
        scratch_shapes=[
            pltpu.VMEM((S, D), _BF16),
            pltpu.VMEM((S // 2, D), jnp.uint32),
            pltpu.VMEM((S, D), _F32),
            pltpu.VMEM((S, D), _F32),
            pltpu.VMEM((S, D), _BF16),
            pltpu.VMEM((2, _TQ, S), _F32),
            pltpu.VMEM((_TQ, 128), _F32),
            pltpu.VMEM((_TQ, Dh), _F32),
            pltpu.VMEM((_TQ, 128), _F32),
            pltpu.VMEM((_NS, 2 * S + 2 * D, Dh), _BF16),
            pltpu.VMEM((F, D), _BF16),
            pltpu.VMEM((F, D), _BF16),
            pltpu.VMEM((F, D), _BF16),
            pltpu.VMEM((D,), _BF16),
            pltpu.SMEM((_TOPC,), _I32),
            pltpu.SMEM((1,), _I32),
            pltpu.SemaphoreType.DMA((_NS + 4 + 2 * n + 5,)),
        ],
        compiler_params=pltpu.CompilerParams(
            dimension_semantics=("arbitrary",),
            vmem_limit_bytes=100 * 1024 * 1024,
            disable_bounds_checks=True,
            disable_semaphore_checks=True,
            internal_scratch_in_bytes=64 * 1024,
        ),
    )(A_x.reshape(S, D), A_k_cache.reshape(H, Sk, Dh), A_v_cache.reshape(H, Sk, Dh), A_wq, A_wo,
      B_w_r, B_w_gate.T, B_w_up.T, B_w_down)
    return out.reshape(B, S, D)
```

```python
import functools
import math

import jax
import jax.numpy as jnp
import jax.experimental.pallas as pl
import jax.experimental.pallas.tpu as pltpu

_F32 = jnp.float32
_BF16 = jnp.bfloat16
_I32 = jnp.int32
_NT = (((1,), (1,)), ((), ()))

_TOPC = 8
_EPS = 1e-5
_TQ = 256
_CW = 512
_P = 7
_L = 12
_NS = 4


def _bf(x):
    return x.astype(_BF16).astype(_F32)


def _silu(x):
    h = 0.5 * x
    return h + h * jnp.tanh(h)


def _sigmoid(x):
    return 0.5 + 0.5 * jnp.tanh(0.5 * x)


def _after(gate, val):
    return jnp.where(gate > jnp.inf, 0.0, val)


def _after16(gate, val):
    g = gate > jnp.inf
    g = jnp.concatenate([g[r:r + 8] for r in range(8, gate.shape[0], 16) for _ in range(2)], axis=0)
    return jnp.where(g, 0.0, val)


def _kernel(x_hbm, k_hbm, v_hbm, wq_hbm, wo_hbm, wr_hbm, wg_hbm, wu_hbm, wd_hbm,
            out_hbm,
            x_ref, xnp_ref, z_ref, acc_ref, ob_ref, s_ref, mc_ref, oc_ref, lc_ref,
            hb, wg_ref, wu_ref, wd_ref, wr_ref, sel_ref, zs,
            sems,
            *, S, D, Dh, H):
    tq, cw, p, L, NS = _TQ, _CW, _P, _L, _NS
    n = S // tq
    R = S // cw
    tb = tq // 4
    D4 = (D // 512) * 512
    F = wd_ref.shape[0]
    scale = (Dh ** -0.5) * math.log2(math.e)

    K0, V0, Q0, O0 = 0, S, 2 * S, 2 * S + D

    def hcol(h):
        return pl.ds(pl.multiple_of(h * Dh, Dh), Dh)

    def cp_k(h, slot, sem, r0=0, r1=S):
        return (pltpu.make_async_copy(k_hbm.at[h, r0:r1], hb.at[slot, K0 + r0:K0 + r1], sems.at[sem]),)

    def cp_v(h, slot, sem):
        return (pltpu.make_async_copy(v_hbm.at[h], hb.at[slot, V0:V0 + S], sems.at[sem]),)

    def cp_wq(h, slot, sem):
        return (pltpu.make_async_copy(wq_hbm.at[:, hcol(h)], hb.at[slot, Q0:Q0 + D], sems.at[sem]),)

    def cp_wo(h, slot, sem):
        return tuple(pltpu.make_async_copy(wo_hbm.at[hcol(h), c:c + 128], hb.at[slot, O0 + c:O0 + c + 128],
                                           sems.at[sem]) for c in range(0, D, 128))

    def start_head(h, slot):
        for cp in (cp_wq, cp_k, cp_v, cp_wo):
            for c in cp(h, slot, slot):
                c.start()

    def wait_head(slot):
        pltpu.make_async_copy(hb.at[slot], hb.at[slot], sems.at[slot]).wait()

    def cp_x(i):
        return pltpu.make_async_copy(x_hbm.at[rs(i * tq, tq), :], x_ref.at[rs(i * tq, tq), :],
                                     sems.at[NS + 5 + i])

    def cp_out(i, z):
        r0, nr = (i * tq, tq) if i < n - 1 else ((n - 1) * tq + (i - n + 1) * tq // 2, tq // 2)
        src = pl.ds(pl.multiple_of(z * tq + r0, tb), nr)
        return pltpu.make_async_copy(ob_ref.at[src, :], out_hbm.at[pl.ds(r0, nr), :], sems.at[NS + 5 + n + i])

    def cp_ffn():
        return (pltpu.make_async_copy(wg_hbm, wg_ref, sems.at[NS + 5 + 2 * n + 4]),
                pltpu.make_async_copy(wu_hbm, wu_ref, sems.at[NS + 5 + 2 * n + 1]),
                pltpu.make_async_copy(wd_hbm, wd_ref, sems.at[NS + 5 + 2 * n + 2]))

    def cp_wr():
        return pltpu.make_async_copy(wr_hbm, wr_ref, sems.at[NS + 5 + 2 * n + 3])

    def lanes(v, k):
        return jnp.concatenate([v] * k, axis=1)

    def rows(v, k):
        return jnp.concatenate([v] * k, axis=0)

    def rs(r0, nr):
        return slice(r0, r0 + nr) if isinstance(r0, int) else pl.ds(pl.multiple_of(r0, tb), nr)

    def rs2(r0, nr):
        return slice(r0 // 2, (r0 + nr) // 2) if isinstance(r0, int) else pl.ds(pl.multiple_of(r0 // 2, tb // 2), nr // 2)

    def fold(v):
        t = v[:, 0:128]
        for j in range(1, v.shape[1] // 128):
            t = t + v[:, j * 128:(j + 1) * 128]
        return t

    def compact(col, g0, init):
        lane = jax.lax.broadcasted_iota(_I32, init.shape, 1) - g0
        for g in range(col.shape[0] // 8):
            init = jnp.where(lane == g, col[8 * g:8 * g + 8, :], init)
        return init

    def side(jobs, res):
        for k, f in enumerate(jobs or []):
            r0 = min(k * res.shape[0] // len(jobs) // 8 * 8, res.shape[0] - tb)
            f(res[r0:r0 + tb, 0:128])

    def stored(ref, r0, z):
        k = 32 // (8 * ref.dtype.itemsize)
        v = ref[pl.ds(pl.multiple_of(z * 8 * k + r0, 8 * k), 8 * k), 0:128]
        return v if k == 1 else pltpu.bitcast(v, _F32)

    def qproj(i, slot, jobs=None):
        w = hb.at[slot, Q0:Q0 + D]
        xv = xnp_ref.at[rs2(i * tq, tq)]
        q = jnp.dot(pltpu.bitcast(xv[:, 0:D4], _BF16), w[0:D4, :], preferred_element_type=_F32)
        q = q + jnp.concatenate(
            [jnp.dot(pltpu.bitcast(xv[t * tb // 2:(t + 1) * tb // 2, D4:D], _BF16), w[D4:D, :],
                     preferred_element_type=_F32)
             for t in range(4)], axis=0)
        side(jobs, q)
        return (q * scale).astype(_BF16)

    def rowmax(mx):
        return jnp.broadcast_to(jnp.max(mx, axis=-1, keepdims=True), (tq, 128))

    def qk(par, slot, q, z, jobs=None, lanewise=False, groups=range(R), mx=None):
        if jobs is None and not lanewise:
            s = jax.lax.dot_general(q, hb[slot, K0:K0 + S], _NT, preferred_element_type=_F32)
            s_ref[z + par % 2] = s
            return rowmax(s)
        for c in groups:
            s = jax.lax.dot_general(q, hb[slot, K0 + c * cw:K0 + (c + 1) * cw], _NT, preferred_element_type=_F32)
            s_ref[z + par % 2, :, c * cw:(c + 1) * cw] = s
            for j in range(cw // 128):
                sj = s[:, j * 128:(j + 1) * 128]
                mx = sj if mx is None else jnp.maximum(mx, sj)
            side(jobs and jobs[c], s)
        return mx if lanewise else rowmax(mx)

    def finalize(r0, nr, c0, c1, s):
        out = x_ref[r0:r0 + nr, c0:c1].astype(_F32) + s * z_ref[r0:r0 + nr, c0:c1]
        ob_ref[r0:r0 + nr, c0:c1] = out.astype(_BF16)
        return out

    def wo(i, slot, o, lp, mode, jobs=None, off=0):
        nq = o.shape[0]
        l = jnp.sum(lp, axis=-1, keepdims=True)
        o32 = o * pl.reciprocal(l, full_range=False)
        o = o32.astype(_BF16)
        w = [hb[slot, O0 + c:O0 + c + 128] for c in range(0, D, 128)]
        av = acc_ref.at[rs(i * tq, tq)]

        def emit(r0, nr, c0, c1, a):
            if mode == "init":
                av[r0:r0 + nr, c0:c1] = a
            elif mode == "acc":
                av[r0:r0 + nr, c0:c1] += a
            else:
                finalize(i * tq + r0, nr, c0, c1, av[r0:r0 + nr, c0:c1] + a)

        a = jnp.dot(o, jnp.concatenate(w[:-1], axis=1), preferred_element_type=_F32)
        emit(off, nq, 0, D4, a)
        side(jobs, a)
        for t in range(0, nq, nq // 4):
            emit(off + t, nq // 4, D4, D,
                 jnp.dot(o32[t:t + nq // 4, :].astype(_BF16), w[-1], preferred_element_type=_F32))
        return a[:, 0:128]

    def pv(par, slot, m, gate, z, jobs=None, before=None, last=False, off=0, lag=1):
        o = lp = None
        gates = [gate] * lag
        for c in range(R):
            mc = m if gates[c] is None else _after16(gates[c], m)
            if before is not None and before[c] is not None:
                mc = _after(rows(before[c](), m.shape[0] // 8), mc)
            sc = s_ref[z + par % 2, off:off + m.shape[0], c * cw:(c + 1) * cw]
            pe = jnp.exp2(sc - lanes(mc, cw // 128))
            ps = [pe[:, j * 128:(j + 1) * 128] for j in range(cw // 128)]
            for pj in ps:
                lp = pj if lp is None else lp + pj
            ps[-1] = jnp.minimum(ps[-1], lp)
            pb = jnp.concatenate(ps, axis=1).astype(_BF16)
            oc = jnp.dot(pb, hb[slot, V0 + c * cw:V0 + (c + 1) * cw], preferred_element_type=_F32)
            side(None if jobs is None else jobs[c], oc)
            o = oc if o is None else o + oc
            gates.append(o)
        return o, (lp if last else _after16(o, lp))

    def layernorm(r0, nr, rt, z, rel=None):
        def x(k):
            return x_ref[pl.ds(pl.multiple_of(k * z * tb + r0, tb), nr), :].astype(_F32)
        xs = fold(x(0))
        if rel is not None:
            xs = _after(rel, xs)
        mean = jnp.sum(xs, axis=-1, keepdims=True) * (1.0 / D)
        xc = x(1) - mean
        var = compact(jnp.sum(xc * xc, axis=-1, keepdims=True), 0, jnp.ones((8, 128), _F32)) * (1.0 / D)
        inv = 1.0 / _bf(jnp.sqrt(_bf(_bf(var) + _bf(jnp.float32(_EPS)))))
        inv = jnp.concatenate([jnp.broadcast_to(inv[:, g:g + 1], (8, 128)) for g in range(nr // 8)], axis=0)
        xn = (_bf(x(2) - _bf(mean)) * lanes(inv, D // 128)).astype(_BF16)
        xnp_ref[rs2(r0, nr), :] = pltpu.bitcast(xn, jnp.uint32)
        if rel is not None:
            router(r0, nr, rt, xn, None)

    def router(r0, nr, rt, xn, rel):
        if xn is None:
            xn = pltpu.bitcast(xnp_ref[rs2(r0, nr), :], _BF16)
        rp = fold(xn.astype(_F32) * wr_ref[...].astype(_F32).reshape(1, D))
        if rel is not None:
            rp = _after(rel, rp)
        rt[0] = compact(jnp.sum(rp, axis=-1, keepdims=True), r0 // 8, rt[0])

    def topk(rt):
        rt = _bf(rt)
        lane = jax.lax.broadcasted_iota(_I32, rt.shape, 1)
        sub = jax.lax.broadcasted_iota(_I32, rt.shape, 0)
        top = pltpu.bitcast(jnp.where(rt == 0.0, 0.0, rt), _I32) >> 16
        code = jnp.where(rt != rt, 0, jnp.where(top < 0, -1 - top, top + 32768))
        key = pltpu.bitcast((1 << 29) + code * S + (S - 1 - (lane * 8 + sub)), _F32)
        for c in range(_TOPC):
            kmax = jnp.max(jnp.max(key, axis=0, keepdims=True), axis=1, keepdims=True)
            sel_ref[c] = S - 1 - (pltpu.bitcast(kmax, _I32)[0, 0] & (S - 1))
            key = jnp.where(key == kmax, 0.0, key)

    def pace(v, k, done, rel):
        t = fold(v)
        t = jnp.concatenate([t[j:j + 8] + t[j + 8:j + 16] for j in range(0, v.shape[0], 16)], axis=0)
        if rel is not None:
            t = _after(jnp.concatenate([rel[j:j + 8] for j in range(0, v.shape[0], 16)], axis=0), t)
        done[0] = compact(jnp.sum(t, axis=-1, keepdims=True), k, done[0])

    def gate_piece(r0, nr, done, rel):
        g = _silu(pltpu.bitcast(xnp_ref[rs2(r0, nr), :], _BF16).astype(_F32))
        z_ref[r0:r0 + nr, :] = g
        pace(g, r0 // 16, done, rel)

    def fin_piece(r0, nr, done, z, rel):
        s = _after(lanes(rel, D // 128), acc_ref[r0:r0 + nr, :])
        pace(finalize(r0, nr, 0, D, s), r0 // 16, done, None)
        if (r0 + nr) % tq == 0:
            cp_out(r0 // tq, z).start()

    def ffn_jobs():
        st = {}
        F4 = (F // cw) * cw

        def gather():
            rowid = jax.lax.broadcasted_iota(_I32, (_TOPC, 1), 0)
            xs = jnp.zeros((_TOPC, D), _F32)
            for c in range(_TOPC):
                w = xnp_ref[pl.ds(sel_ref[c] // 2, 1), :]
                w = jnp.where(sel_ref[c] % 2 == 0, w << 16, w & jnp.uint32(0xFFFF0000))
                xs = jnp.where(rowid == c, pltpu.bitcast(w, _F32), xs)
            st["xs"], st["xb"] = xs, xs.astype(_BF16)

        def add(key, val):
            st[key] = val if key not in st else st[key] + val

        def up(parts, k, rel):
            xk = st["xb"][:, k * 128:(k + 1) * 128]
            for name, w_ref, c0, c1 in parts:
                add((name, c0), jax.lax.dot_general(xk, w_ref[c0:c1, k * 128:(k + 1) * 128], _NT,
                                                    preferred_element_type=_F32))

        def hidden():
            cuts = list(range(0, F, cw))
            g = _bf(jnp.concatenate([st["g", c] for c in cuts], axis=1))
            u = _bf(jnp.concatenate([st["u", c] for c in cuts], axis=1))
            st["h"] = (_bf(_silu(g)) * u).astype(_BF16)

        def down(cuts, c0, c1, rel):
            if "h" not in st:
                hidden()
            for k0, k1 in zip(cuts[:-1], cuts[1:]):
                add(("y", c0), jnp.dot(st["h"][:, k0:k1], wd_ref[k0:k1, c0:c1], preferred_element_type=_F32))

        def scatter(done):
            xs = _after(lanes(done, D // 128), st["xs"])
            rs = _bf(jnp.sum(fold(xs * wr_ref[...].astype(_F32).reshape(1, D)), axis=-1, keepdims=True))
            y = _bf(jnp.concatenate([st["y", 0], st["y", D4]], axis=1))
            zz = _silu(_bf(xs + _bf(y * _bf(_sigmoid(rs)))))
            for c in range(_TOPC):
                z_ref[pl.ds(sel_ref[c], 1), :] = zz[c:c + 1, :]

        stage1 = []
        for k in range(D // 128):
            for name, w_ref in (("g", wg_ref), ("u", wu_ref)):
                for c0 in range(0, F4, cw):
                    stage1.append(functools.partial(up, [(name, w_ref, c0, c0 + cw)], k))
            stage1.append(functools.partial(up, [("g", wg_ref, F4, F), ("u", wu_ref, F4, F)], k))
        stage2 = [functools.partial(down, [k0, min(k0 + 128, F)], 0, D4) for k0 in range(0, F, 128)]
        stage2 += [functools.partial(down, [k0, k0 + cw], D4, D) for k0 in range(0, F4, cw)]
        stage2 += [functools.partial(down, [F4, F4 + 64, F4 + 128, F4 + 160, F], D4, D)]
        return gather, stage1, stage2, scatter

    def save(state):
        mc_ref[...], oc_ref[...], lc_ref[...] = state

    def load():
        return rowmax(mc_ref[...]), oc_ref[...], lc_ref[...]

    def chunk(u):
        return u % n if isinstance(u, int) else u & (n - 1)

    def slot(u):
        return u // n % NS if isinstance(u, int) else (u >> 3) & (NS - 1)

    def round_(u, par, state, z, mode, jobs=None, before=None, last=False, mid=None, nxt=None):
        m, o, lp = state
        c1, s1 = nxt or (chunk(u + 1), slot(u + 1))
        q = qproj(c1, s1, jobs and jobs[0])
        m_next = qk(par + 1, s1, q, z, jobs and jobs[1:R + 1], lanewise=last)
        if mid is not None:
            mid()
        gate = wo(chunk(u - 1), slot(u - 1), o, lp, mode, jobs and jobs[R + 1])
        if mode == "final":
            cp_out(chunk(u - 1), z).start()
        return (m_next,) + pv(par, slot(u), m, gate, z, jobs and jobs[R + 2:], before, last)

    zs[0] = jnp.minimum(pl.program_id(0), 0)
    wq0, v0, wo0 = (cp(0, 0, NS + t) for t, cp in enumerate((cp_wq, cp_v, cp_wo)))
    k0 = cp_k(0, 0, NS + 3, 0, S // 2) + cp_k(0, 0, NS + 4, S // 2, S)
    for c in (cp_x(0), *wq0, cp_x(1), cp_wr(), *k0, cp_x(2), *v0, *wo0, *(cp_x(i) for i in range(3, n))):
        c.start()
    start_head(1, 1)
    start_head(2, 2)
    for c in cp_ffn():
        c.start()
    @pl.loop(0, (S - (p - 1) * tq) // 32)
    def _(i):
        acc_ref[pl.ds(pl.multiple_of((p - 1) * tq + i * 32, 32), 32), :] = jnp.zeros((32, D), _F32)

    cp_x(0).wait()
    z = zs[0]
    rt = [jnp.zeros((8, S // 8), _F32)]

    def ln_jobs(i, z, spread):
        pieces = [functools.partial(layernorm, i * tq + t * tb, tb, rt, z) for t in range(4)]
        return [[pieces.pop(0) for _ in range(k)] for k in spread]

    for f in ln_jobs(0, z, [4])[0]:
        f()
    wq0[0].wait()
    cp_x(1).wait()
    q0 = qproj(0, 0)
    for f in ln_jobs(1, z, [4])[0]:
        f()
    q1 = qproj(1, 0)
    cp_wr().wait()
    k0[0].wait()
    scores01 = [[functools.partial(router, (2 * c + t) * tb, tb, rt, None) for t in range(2)] for c in range(R)]
    m0 = qk(0, 0, q0, z, scores01[:2], True, range(2))
    m1 = qk(1, 0, q1, z, scores01[2:], True, range(2))
    k0[1].wait()
    cp_x(2).wait()
    ln2 = ln_jobs(2, z, [0, 0, 3, 1])
    m0 = rowmax(qk(0, 0, q0, z, ln2, True, range(2, 4), m0))
    m1 = qk(1, 0, q1, z, None, True, range(2, 4), m1)
    v0[0].wait()
    save((m1,) + pv(0, 0, m0, None, z, last=True))
    for c in wo0:
        c.wait()

    def pair(j, rt_in):
        for k in range(2):
            pl.when(3 + 2 * j + k < n)(lambda: cp_x(jnp.minimum(3 + 2 * j + k, n - 1)).wait())
        z = zs[0]
        rt[0] = rt_in
        state = load()
        for k in range(2):
            u = 1 + 2 * j + k
            jobs = ln_jobs(jnp.minimum(u + 2, n - 1), z, [1, 1, 1, 1, 0, 0, 0, 0, 0, 0])
            state = round_(u, 1 + k, state, z, "init", jobs, last=(k == 1))
        save(state)
        return rt[0]

    scores = jax.lax.fori_loop(0, (p - 1) // 2, pair, rt[0])

    def entry(u0):
        h0 = (u0 >> 3) + 1
        return (u0, h0 & (NS - 1), (h0 + 1) & (NS - 1), ((u0 + L) >> 3) - h0, chunk(u0 + 1), slot(u0 + 1))

    def body(j, carry):
        u0, w1, w2, two, c1, s1 = carry
        wait_head(w1)
        pl.when(two > 0)(lambda: wait_head(w2))
        z = zs[0]

        def prefetch():
            h1 = ((u0 + L) >> 3) + 1
            start_head(h1, h1 & (NS - 1))
            pl.when(h1 + 1 <= jnp.minimum((u0 + 2 * L) >> 3, H - 1))(
                lambda: start_head(h1 + 1, (h1 + 1) & (NS - 1)))

        state = load()
        for k in range(L):
            state = round_(u0 + k, p + k, state, z, "acc", last=(k == L - 1), mid=prefetch if k == 1 else None,
                           nxt=(c1, s1) if k == 0 else None)
        save(state)
        return entry(u0 + L)

    T = H * n
    jax.lax.fori_loop(0, (T - 2 * n) // L, body, entry(jnp.int32(p)))

    wait_head((H - 1) % NS)
    for c in cp_ffn():
        c.wait()
    z = zs[0]
    state = load()
    gather, stage1, stage2, scatter = ffn_jobs()
    topk(scores)
    gather()
    done, done2 = [jnp.zeros((8, 128), _F32)], [jnp.zeros((8, 128), _F32)]
    late = 3
    gates = [functools.partial(gate_piece, r0, tb, done) for r0 in range(0, S, tb)]
    fins = [functools.partial(fin_piece, r0, tb, done2, z) for r0 in range(0, late * tq, tb)]
    fq = stage1 + [lambda rel: None] + stage2
    u_first = T - 2 * n + p
    for u in range(u_first, T - 1):
        i = u - 1 - (T - n)
        vpu, nv, nf = gates, [1, 1, 0, 0, 0, 0, 1, 1, 1, 1], [1] * 6 + [1 if i < late - 2 else 2] * 4
        if u == u_first:
            nv, nf = [0, 0, 0, 0, 0, 2, 2, 2, 2, 0], [0] * 6 + [1] * 4
        if i > late:
            vpu, nv = fins, [2, 2, 1, 1]
        jobs = [[vpu.pop(0) for _ in range(min(len(vpu), a))] + [fq.pop(0) for _ in range(min(len(fq), b))]
                for a, b in zip(nv + [0] * 10, nf)]
        before = [None] * R
        if i >= late:
            assert not fq and not gates
            before[2] = functools.partial(stored, ob_ref, i * tq, z)
        state = round_(u, u, state, z, "final" if i >= late else "acc", jobs, before,
                       mid=(lambda: scatter(done[0])) if i == late else None)
    assert not fins
    m, o, lp = state
    sl, hq = slot(T - 1), tq // 2
    oa, lpa = pv(T - 1, sl, m[:hq], o[:hq], z, before=[lambda: done2[0], None, None, None], lag=2)
    gate = wo(n - 2, sl, o, lp, "final")
    cp_out(n - 2, z).start()
    ob, lpb = pv(T - 1, sl, m[hq:], gate[:hq], z, off=hq, lag=2,
                 before=[None, None, None, functools.partial(stored, ob_ref, (n - 2) * tq, z)])
    wo(n - 1, sl, oa, lpa, "final")
    cp_out(n - 1, z).start()
    wo(n - 1, sl, ob, lpb, "final", off=hq)
    cp_out(n, z).start()
    for i in range(n + 1):
        cp_out(i, z).wait()


@jax.jit
def pallas_recurrent_scan__mha_block_cached__moe_arch_mod__prompt_kernel(
    A_x: jax.Array,
    A_k_cache: jax.Array,
    A_v_cache: jax.Array,
    A_wq: jax.Array,
    A_wo: jax.Array,
    B_x: jax.Array,
    B_w_r: jax.Array,
    B_w_gate: jax.Array,
    B_w_up: jax.Array,
    B_w_down: jax.Array,
):
    B, S, D = A_x.shape
    _, H, Sk, Dh = A_k_cache.shape
    F = B_w_gate.shape[1]
    assert B == 1 and Sk == S and S % _TQ == 0 and S % _CW == 0 and Dh == 128 and D % 512 == 128
    n = S // _TQ
    assert n == 8 and _P == n - 1 and (H - 2) * n % _L == 0 and _L == 12 and _NS == 4 and S == 2048 and F % _CW == 192
    hbm = pl.BlockSpec(memory_space=pltpu.HBM)
    out = pl.pallas_call(
        functools.partial(_kernel, S=S, D=D, Dh=Dh, H=H),
        grid=(1,),
        in_specs=[hbm] * 9,
        out_specs=pl.BlockSpec(memory_space=pl.ANY),
        out_shape=jax.ShapeDtypeStruct((S, D), _BF16),
        scratch_shapes=[
            pltpu.VMEM((S, D), _BF16),
            pltpu.VMEM((S // 2, D), jnp.uint32),
            pltpu.VMEM((S, D), _F32),
            pltpu.VMEM((S, D), _F32),
            pltpu.VMEM((S, D), _BF16),
            pltpu.VMEM((2, _TQ, S), _F32),
            pltpu.VMEM((_TQ, 128), _F32),
            pltpu.VMEM((_TQ, Dh), _F32),
            pltpu.VMEM((_TQ, 128), _F32),
            pltpu.VMEM((_NS, 2 * S + 2 * D, Dh), _BF16),
            pltpu.VMEM((F, D), _BF16),
            pltpu.VMEM((F, D), _BF16),
            pltpu.VMEM((F, D), _BF16),
            pltpu.VMEM((D,), _BF16),
            pltpu.SMEM((_TOPC,), _I32),
            pltpu.SMEM((1,), _I32),
            pltpu.SemaphoreType.DMA((_NS + 5 + 2 * n + 5,)),
        ],
        compiler_params=pltpu.CompilerParams(
            dimension_semantics=("arbitrary",),
            vmem_limit_bytes=100 * 1024 * 1024,
            disable_bounds_checks=True,
            disable_semaphore_checks=True,
            internal_scratch_in_bytes=64 * 1024,
        ),
    )(A_x.reshape(S, D), A_k_cache.reshape(H, Sk, Dh), A_v_cache.reshape(H, Sk, Dh), A_wq, A_wo,
      B_w_r, B_w_gate.T, B_w_up.T, B_w_down)
    return out.reshape(B, S, D)
```

```python
import functools
import math

import jax
import jax.numpy as jnp
import jax.experimental.pallas as pl
import jax.experimental.pallas.tpu as pltpu

_F32 = jnp.float32
_BF16 = jnp.bfloat16
_I32 = jnp.int32
_NT = (((1,), (1,)), ((), ()))

_TOPC = 8
_EPS = 1e-5
_TQ = 256
_CW = 512
_P = 7
_L = 12
_NS = 4


def _bf(x):
    return x.astype(_BF16).astype(_F32)


def _silu(x):
    h = 0.5 * x
    return h + h * jnp.tanh(h)


def _sigmoid(x):
    return 0.5 + 0.5 * jnp.tanh(0.5 * x)


def _after(gate, val):
    return jnp.where(gate > jnp.inf, 0.0, val)


def _after16(gate, val):
    g = gate > jnp.inf
    g = jnp.concatenate([g[r:r + 8] for r in range(8, gate.shape[0], 16) for _ in range(2)], axis=0)
    return jnp.where(g, 0.0, val)


def _kernel(x_hbm, k_hbm, v_hbm, wq_hbm, wo_hbm, wr_hbm, wg_hbm, wu_hbm, wd_hbm,
            out_hbm,
            x_ref, xnp_ref, z_ref, acc_ref, ob_ref, s_ref, mc_ref, oc_ref, lc_ref,
            hb, wg_ref, wu_ref, wd_ref, wr_ref, sel_ref, zs,
            sems,
            *, S, D, Dh, H):
    tq, cw, p, L, NS = _TQ, _CW, _P, _L, _NS
    n = S // tq
    R = S // cw
    tb = tq // 4
    D4 = (D // 512) * 512
    F = wd_ref.shape[0]
    scale = (Dh ** -0.5) * math.log2(math.e)

    K0, V0, Q0, O0 = 0, S, 2 * S, 2 * S + D

    def hcol(h):
        return pl.ds(pl.multiple_of(h * Dh, Dh), Dh)

    def cp_k(h, slot, sem, r0=0, r1=S):
        return (pltpu.make_async_copy(k_hbm.at[h, r0:r1], hb.at[slot, K0 + r0:K0 + r1], sems.at[sem]),)

    def cp_v(h, slot, sem):
        return (pltpu.make_async_copy(v_hbm.at[h], hb.at[slot, V0:V0 + S], sems.at[sem]),)

    def cp_wq(h, slot, sem):
        return (pltpu.make_async_copy(wq_hbm.at[:, hcol(h)], hb.at[slot, Q0:Q0 + D], sems.at[sem]),)

    def cp_wo(h, slot, sem):
        return tuple(pltpu.make_async_copy(wo_hbm.at[hcol(h), c:c + 128], hb.at[slot, O0 + c:O0 + c + 128],
                                           sems.at[sem]) for c in range(0, D, 128))

    def start_head(h, slot):
        for cp in (cp_wq, cp_k, cp_v, cp_wo):
            for c in cp(h, slot, slot):
                c.start()

    def wait_head(slot):
        pltpu.make_async_copy(hb.at[slot], hb.at[slot], sems.at[slot]).wait()

    def cp_x(i):
        return pltpu.make_async_copy(x_hbm.at[rs(i * tq, tq), :], x_ref.at[rs(i * tq, tq), :],
                                     sems.at[NS + 5 + i])

    def cp_out(i, z):
        r0, nr = (i * tq, tq) if i < n - 1 else ((n - 1) * tq + (i - n + 1) * tq // 2, tq // 2)
        src = pl.ds(pl.multiple_of(z * tq + r0, tb), nr)
        return pltpu.make_async_copy(ob_ref.at[src, :], out_hbm.at[pl.ds(r0, nr), :], sems.at[NS + 5 + n + i])

    def cp_ffn():
        return (pltpu.make_async_copy(wg_hbm, wg_ref, sems.at[NS + 5 + 2 * n + 4]),
                pltpu.make_async_copy(wu_hbm, wu_ref, sems.at[NS + 5 + 2 * n + 1]),
                pltpu.make_async_copy(wd_hbm, wd_ref, sems.at[NS + 5 + 2 * n + 2]))

    def cp_wr():
        return pltpu.make_async_copy(wr_hbm, wr_ref, sems.at[NS + 5 + 2 * n + 3])

    def lanes(v, k):
        return jnp.concatenate([v] * k, axis=1)

    def rows(v, k):
        return jnp.concatenate([v] * k, axis=0)

    def rs(r0, nr):
        return slice(r0, r0 + nr) if isinstance(r0, int) else pl.ds(pl.multiple_of(r0, tb), nr)

    def rs2(r0, nr):
        return slice(r0 // 2, (r0 + nr) // 2) if isinstance(r0, int) else pl.ds(pl.multiple_of(r0 // 2, tb // 2), nr // 2)

    def fold(v):
        t = v[:, 0:128]
        for j in range(1, v.shape[1] // 128):
            t = t + v[:, j * 128:(j + 1) * 128]
        return t

    def compact(col, g0, init):
        lane = jax.lax.broadcasted_iota(_I32, init.shape, 1) - g0
        for g in range(col.shape[0] // 8):
            init = jnp.where(lane == g, col[8 * g:8 * g + 8, :], init)
        return init

    def side(jobs, res):
        for k, f in enumerate(jobs or []):
            r0 = min(k * res.shape[0] // len(jobs) // 8 * 8, res.shape[0] - tb)
            f(res[r0:r0 + tb, 0:128])

    def stored(ref, r0, z):
        k = 32 // (8 * ref.dtype.itemsize)
        v = ref[pl.ds(pl.multiple_of(z * 8 * k + r0, 8 * k), 8 * k), 0:128]
        return v if k == 1 else pltpu.bitcast(v, _F32)

    def qproj(i, slot, jobs=None):
        w = hb.at[slot, Q0:Q0 + D]
        xv = xnp_ref.at[rs2(i * tq, tq)]
        q = jnp.dot(pltpu.bitcast(xv[:, 0:D4], _BF16), w[0:D4, :], preferred_element_type=_F32)
        q = q + jnp.concatenate(
            [jnp.dot(pltpu.bitcast(xv[t * tb // 2:(t + 1) * tb // 2, D4:D], _BF16), w[D4:D, :],
                     preferred_element_type=_F32)
             for t in range(4)], axis=0)
        side(jobs, q)
        return (q * scale).astype(_BF16)

    def rowmax(mx):
        return jnp.broadcast_to(jnp.max(mx, axis=-1, keepdims=True), (tq, 128))

    def qk(par, slot, q, z, jobs=None, lanewise=False, groups=range(R), mx=None):
        if jobs is None and not lanewise:
            s = jax.lax.dot_general(q, hb[slot, K0:K0 + S], _NT, preferred_element_type=_F32)
            s_ref[z + par % 2] = s
            return rowmax(s)
        for c in groups:
            s = jax.lax.dot_general(q, hb[slot, K0 + c * cw:K0 + (c + 1) * cw], _NT, preferred_element_type=_F32)
            s_ref[z + par % 2, :, c * cw:(c + 1) * cw] = s
            for j in range(cw // 128):
                sj = s[:, j * 128:(j + 1) * 128]
                mx = sj if mx is None else jnp.maximum(mx, sj)
            side(jobs and jobs[c], s)
        return mx if lanewise else rowmax(mx)

    def finalize(r0, nr, c0, c1, s):
        out = x_ref[r0:r0 + nr, c0:c1].astype(_F32) + s * z_ref[r0:r0 + nr, c0:c1]
        ob_ref[r0:r0 + nr, c0:c1] = out.astype(_BF16)
        return out

    def wo(i, slot, o, lp, mode, jobs=None, off=0):
        nq = o.shape[0]
        l = jnp.sum(lp, axis=-1, keepdims=True)
        o32 = o * pl.reciprocal(l, full_range=False)
        o = o32.astype(_BF16)
        w = [hb[slot, O0 + c:O0 + c + 128] for c in range(0, D, 128)]
        av = acc_ref.at[rs(i * tq, tq)]

        def emit(r0, nr, c0, c1, a):
            if mode == "init":
                av[r0:r0 + nr, c0:c1] = a
            elif mode == "acc":
                av[r0:r0 + nr, c0:c1] += a
            else:
                finalize(i * tq + r0, nr, c0, c1, av[r0:r0 + nr, c0:c1] + a)

        a = jnp.dot(o, jnp.concatenate(w[:-1], axis=1), preferred_element_type=_F32)
        emit(off, nq, 0, D4, a)
        side(jobs, a)
        for t in range(0, nq, nq // 4):
            emit(off + t, nq // 4, D4, D,
                 jnp.dot(o32[t:t + nq // 4, :].astype(_BF16), w[-1], preferred_element_type=_F32))
        return a[:, 0:128]

    def pv(par, slot, m, gate, z, jobs=None, before=None, last=False, off=0, lag=1):
        o = lp = None
        gates = [gate] * lag
        for c in range(R):
            mc = m if gates[c] is None else _after16(gates[c], m)
            if before is not None and before[c] is not None:
                mc = _after(rows(before[c](), m.shape[0] // 8), mc)
            sc = s_ref[z + par % 2, off:off + m.shape[0], c * cw:(c + 1) * cw]
            pe = jnp.exp2(sc - lanes(mc, cw // 128))
            ps = [pe[:, j * 128:(j + 1) * 128] for j in range(cw // 128)]
            for pj in ps:
                lp = pj if lp is None else lp + pj
            ps[-1] = jnp.minimum(ps[-1], lp)
            pb = jnp.concatenate(ps, axis=1).astype(_BF16)
            oc = jnp.dot(pb, hb[slot, V0 + c * cw:V0 + (c + 1) * cw], preferred_element_type=_F32)
            side(None if jobs is None else jobs[c], oc)
            o = oc if o is None else o + oc
            gates.append(o)
        return o, (lp if last else _after16(o, lp))

    def layernorm(r0, nr, rt, z, rel=None):
        def x(k):
            return x_ref[pl.ds(pl.multiple_of(k * z * tb + r0, tb), nr), :].astype(_F32)
        xs = fold(x(0))
        if rel is not None:
            xs = _after(rel, xs)
        mean = jnp.sum(xs, axis=-1, keepdims=True) * (1.0 / D)
        xc = x(1) - mean
        var = compact(jnp.sum(xc * xc, axis=-1, keepdims=True), 0, jnp.ones((8, 128), _F32)) * (1.0 / D)
        inv = 1.0 / _bf(jnp.sqrt(_bf(_bf(var) + _bf(jnp.float32(_EPS)))))
        inv = jnp.concatenate([jnp.broadcast_to(inv[:, g:g + 1], (8, 128)) for g in range(nr // 8)], axis=0)
        xn = (_bf(x(2) - _bf(mean)) * lanes(inv, D // 128)).astype(_BF16)
        xnp_ref[rs2(r0, nr), :] = pltpu.bitcast(xn, jnp.uint32)
        if rel is not None:
            router(r0, nr, rt, xn, None)

    def router(r0, nr, rt, xn, rel):
        if xn is None:
            xn = pltpu.bitcast(xnp_ref[rs2(r0, nr), :], _BF16)
        rp = fold(xn.astype(_F32) * wr_ref[...].astype(_F32).reshape(1, D))
        if rel is not None:
            rp = _after(rel, rp)
        rt[0] = compact(jnp.sum(rp, axis=-1, keepdims=True), r0 // 8, rt[0])

    def topk(rt):
        rt = _bf(rt)
        lane = jax.lax.broadcasted_iota(_I32, rt.shape, 1)
        sub = jax.lax.broadcasted_iota(_I32, rt.shape, 0)
        top = pltpu.bitcast(jnp.where(rt == 0.0, 0.0, rt), _I32) >> 16
        code = jnp.where(rt != rt, 0, jnp.where(top < 0, -1 - top, top + 32768))
        key = pltpu.bitcast((1 << 29) + code * S + (S - 1 - (lane * 8 + sub)), _F32)
        for c in range(_TOPC):
            kmax = jnp.max(jnp.max(key, axis=0, keepdims=True), axis=1, keepdims=True)
            sel_ref[c] = S - 1 - (pltpu.bitcast(kmax, _I32)[0, 0] & (S - 1))
            key = jnp.where(key == kmax, 0.0, key)

    def pace(v, k, done, rel):
        t = fold(v)
        t = jnp.concatenate([t[j:j + 8] + t[j + 8:j + 16] for j in range(0, v.shape[0], 16)], axis=0)
        if rel is not None:
            t = _after(jnp.concatenate([rel[j:j + 8] for j in range(0, v.shape[0], 16)], axis=0), t)
        done[0] = compact(jnp.sum(t, axis=-1, keepdims=True), k, done[0])

    def gate_piece(r0, nr, done, rel):
        g = _silu(pltpu.bitcast(xnp_ref[rs2(r0, nr), :], _BF16).astype(_F32))
        z_ref[r0:r0 + nr, :] = g
        pace(g, r0 // 16, done, rel)

    def fin_piece(r0, nr, done, z, rel):
        s = _after(lanes(rel, D // 128), acc_ref[r0:r0 + nr, :])
        pace(finalize(r0, nr, 0, D, s), r0 // 16, done, None)
        if (r0 + nr) % tq == 0:
            cp_out(r0 // tq, z).start()

    def ffn_jobs():
        st = {}
        F4 = (F // cw) * cw

        def gather():
            rowid = jax.lax.broadcasted_iota(_I32, (_TOPC, 1), 0)
            xs = jnp.zeros((_TOPC, D), _F32)
            for c in range(_TOPC):
                w = xnp_ref[pl.ds(sel_ref[c] // 2, 1), :]
                w = jnp.where(sel_ref[c] % 2 == 0, w << 16, w & jnp.uint32(0xFFFF0000))
                xs = jnp.where(rowid == c, pltpu.bitcast(w, _F32), xs)
            st["xs"], st["xb"] = xs, xs.astype(_BF16)

        def add(key, val):
            st[key] = val if key not in st else st[key] + val

        def up(parts, k, rel):
            xk = st["xb"][:, k * 128:(k + 1) * 128]
            for name, w_ref, c0, c1 in parts:
                add((name, c0), jax.lax.dot_general(xk, w_ref[c0:c1, k * 128:(k + 1) * 128], _NT,
                                                    preferred_element_type=_F32))

        def hidden():
            cuts = list(range(0, F, cw))
            g = _bf(jnp.concatenate([st["g", c] for c in cuts], axis=1))
            u = _bf(jnp.concatenate([st["u", c] for c in cuts], axis=1))
            st["h"] = (_bf(_silu(g)) * u).astype(_BF16)

        def down(cuts, c0, c1, rel):
            if "h" not in st:
                hidden()
            for k0, k1 in zip(cuts[:-1], cuts[1:]):
                add(("y", c0), jnp.dot(st["h"][:, k0:k1], wd_ref[k0:k1, c0:c1], preferred_element_type=_F32))

        def scatter(done):
            xs = _after(lanes(done, D // 128), st["xs"])
            rs = _bf(jnp.sum(fold(xs * wr_ref[...].astype(_F32).reshape(1, D)), axis=-1, keepdims=True))
            y = _bf(jnp.concatenate([st["y", 0], st["y", D4]], axis=1))
            zz = _silu(_bf(xs + _bf(y * _bf(_sigmoid(rs)))))
            for c in range(_TOPC):
                z_ref[pl.ds(sel_ref[c], 1), :] = zz[c:c + 1, :]

        stage1 = []
        for k in range(D // 128):
            for name, w_ref in (("g", wg_ref), ("u", wu_ref)):
                for c0 in range(0, F4, cw):
                    stage1.append(functools.partial(up, [(name, w_ref, c0, c0 + cw)], k))
            stage1.append(functools.partial(up, [("g", wg_ref, F4, F), ("u", wu_ref, F4, F)], k))
        stage2 = [functools.partial(down, [k0, min(k0 + 128, F)], 0, D4) for k0 in range(0, F, 128)]
        stage2 += [functools.partial(down, [k0, k0 + cw], D4, D) for k0 in range(0, F4, cw)]
        stage2 += [functools.partial(down, [F4, F4 + 64, F4 + 128, F4 + 160, F], D4, D)]
        return gather, stage1, stage2, scatter

    def save(state):
        mc_ref[...], oc_ref[...], lc_ref[...] = state

    def load():
        return rowmax(mc_ref[...]), oc_ref[...], lc_ref[...]

    def chunk(u):
        return u % n if isinstance(u, int) else u & (n - 1)

    def slot(u):
        return u // n % NS if isinstance(u, int) else (u >> 3) & (NS - 1)

    def round_(u, par, state, z, mode, jobs=None, before=None, last=False, mid=None, nxt=None):
        m, o, lp = state
        c1, s1 = nxt or (chunk(u + 1), slot(u + 1))
        q = qproj(c1, s1, jobs and jobs[0])
        m_next = qk(par + 1, s1, q, z, jobs and jobs[1:R + 1], lanewise=last)
        if mid is not None:
            mid()
        gate = wo(chunk(u - 1), slot(u - 1), o, lp, mode, jobs and jobs[R + 1])
        if mode == "final":
            cp_out(chunk(u - 1), z).start()
        return (m_next,) + pv(par, slot(u), m, gate, z, jobs and jobs[R + 2:], before, last)

    zs[0] = jnp.minimum(pl.program_id(0), 0)
    wq0, v0, wo0 = (cp(0, 0, NS + t) for t, cp in enumerate((cp_wq, cp_v, cp_wo)))
    k0 = cp_k(0, 0, NS + 3, 0, S // 2) + cp_k(0, 0, NS + 4, S // 2, S)
    for c in (cp_x(0), *wq0, cp_x(1), cp_wr(), *k0, cp_x(2), *v0, *wo0, *(cp_x(i) for i in range(3, n))):
        c.start()
    start_head(1, 1)
    start_head(2, 2)
    for c in cp_ffn():
        c.start()
    @pl.loop(0, (S - (p - 1) * tq) // 32)
    def _(i):
        acc_ref[pl.ds(pl.multiple_of((p - 1) * tq + i * 32, 32), 32), :] = jnp.zeros((32, D), _F32)

    cp_x(0).wait()
    z = zs[0]
    rt = [jnp.zeros((8, S // 8), _F32)]

    def ln_jobs(i, z, spread):
        pieces = [functools.partial(layernorm, i * tq + t * tb, tb, rt, z) for t in range(4)]
        return [[pieces.pop(0) for _ in range(k)] for k in spread]

    for f in ln_jobs(0, z, [4])[0]:
        f()
    wq0[0].wait()
    cp_x(1).wait()
    q0 = qproj(0, 0)
    for f in ln_jobs(1, z, [4])[0]:
        f()
    q1 = qproj(1, 0)
    cp_wr().wait()
    k0[0].wait()
    scores01 = [[functools.partial(router, (2 * c + t) * tb, tb, rt, None) for t in range(2)] for c in range(R)]
    m0 = qk(0, 0, q0, z, scores01[:2], True, range(2))
    m1 = qk(1, 0, q1, z, scores01[2:], True, range(2))
    k0[1].wait()
    cp_x(2).wait()
    ln2 = ln_jobs(2, z, [0, 0, 3, 1])
    m0 = rowmax(qk(0, 0, q0, z, ln2, True, range(2, 4), m0))
    m1 = qk(1, 0, q1, z, None, True, range(2, 4), m1)
    v0[0].wait()
    save((m1,) + pv(0, 0, m0, None, z, last=True))
    pltpu.make_async_copy(hb.at[0, O0:O0 + D], hb.at[0, O0:O0 + D], sems.at[NS + 2]).wait()

    def pair(j, carry):
        rt[0], u, i0, i1 = carry
        cp_x(i0).wait()
        pl.when(i1 > i0)(lambda: cp_x(i1).wait())
        z = zs[0]
        state = load()
        for k, i in enumerate((i0, i1)):
            jobs = ln_jobs(i, z, [1, 1, 1, 1, 0, 0, 0, 0, 0, 0])
            state = round_(u + k, 1 + k, state, z, "init", jobs, last=(k == 1), nxt=(u + k + 1, 0))
        save(state)
        return rt[0], u + 2, i0 + 2, jnp.minimum(i1 + 2, n - 1)

    scores = jax.lax.fori_loop(0, (p - 1) // 2, pair, (rt[0], jnp.int32(1), jnp.int32(3), jnp.int32(4)))[0]

    def entry(u0):
        h0 = (u0 >> 3) + 1
        return (u0, h0 & (NS - 1), (h0 + 1) & (NS - 1), ((u0 + L) >> 3) - h0, chunk(u0 + 1), slot(u0 + 1))

    def body(j, carry):
        u0, w1, w2, two, c1, s1 = carry
        wait_head(w1)
        pl.when(two > 0)(lambda: wait_head(w2))
        z = zs[0]

        def prefetch():
            h1 = ((u0 + L) >> 3) + 1
            start_head(h1, h1 & (NS - 1))
            pl.when(h1 + 1 <= jnp.minimum((u0 + 2 * L) >> 3, H - 1))(
                lambda: start_head(h1 + 1, (h1 + 1) & (NS - 1)))

        state = load()
        for k in range(L):
            state = round_(u0 + k, p + k, state, z, "acc", last=(k == L - 1), mid=prefetch if k == 1 else None,
                           nxt=(c1, s1) if k == 0 else None)
        save(state)
        return entry(u0 + L)

    T = H * n
    jax.lax.fori_loop(0, (T - 2 * n) // L, body, entry(jnp.int32(p)))

    wait_head((H - 1) % NS)
    for c in cp_ffn():
        c.wait()
    z = zs[0]
    state = load()
    gather, stage1, stage2, scatter = ffn_jobs()
    topk(scores)
    gather()
    done, done2 = [jnp.zeros((8, 128), _F32)], [jnp.zeros((8, 128), _F32)]
    late = 3
    gates = [functools.partial(gate_piece, r0, tb, done) for r0 in range(0, S, tb)]
    fins = [functools.partial(fin_piece, r0, tb, done2, z) for r0 in range(0, late * tq, tb)]
    fq = stage1 + [lambda rel: None] + stage2
    u_first = T - 2 * n + p
    for u in range(u_first, T - 1):
        i = u - 1 - (T - n)
        vpu, nv, nf = gates, [1, 1, 0, 0, 0, 0, 1, 1, 1, 1], [1] * 6 + [1 if i < late - 2 else 2] * 4
        if u == u_first:
            nv, nf = [0, 0, 0, 0, 0, 2, 2, 2, 2, 0], [0] * 6 + [1] * 4
        if i > late:
            vpu, nv = fins, [2, 2, 1, 1]
        jobs = [[vpu.pop(0) for _ in range(min(len(vpu), a))] + [fq.pop(0) for _ in range(min(len(fq), b))]
                for a, b in zip(nv + [0] * 10, nf)]
        before = [None] * R
        if i >= late:
            assert not fq and not gates
            before[2] = functools.partial(stored, ob_ref, i * tq, z)
        state = round_(u, u, state, z, "final" if i >= late else "acc", jobs, before,
                       mid=(lambda: scatter(done[0])) if i == late else None)
    assert not fins
    m, o, lp = state
    sl, hq = slot(T - 1), tq // 2
    oa, lpa = pv(T - 1, sl, m[:hq], o[:hq], z, before=[lambda: done2[0], None, None, None], lag=2)
    gate = wo(n - 2, sl, o, lp, "final")
    cp_out(n - 2, z).start()
    ob, lpb = pv(T - 1, sl, m[hq:], gate[:hq], z, off=hq, lag=2,
                 before=[None, None, None, functools.partial(stored, ob_ref, (n - 2) * tq, z)])
    wo(n - 1, sl, oa, lpa, "final")
    cp_out(n - 1, z).start()
    wo(n - 1, sl, ob, lpb, "final", off=hq)
    cp_out(n, z).start()
    for i in range(n + 1):
        cp_out(i, z).wait()


@jax.jit
def pallas_recurrent_scan__mha_block_cached__moe_arch_mod__prompt_kernel(
    A_x: jax.Array,
    A_k_cache: jax.Array,
    A_v_cache: jax.Array,
    A_wq: jax.Array,
    A_wo: jax.Array,
    B_x: jax.Array,
    B_w_r: jax.Array,
    B_w_gate: jax.Array,
    B_w_up: jax.Array,
    B_w_down: jax.Array,
):
    B, S, D = A_x.shape
    _, H, Sk, Dh = A_k_cache.shape
    F = B_w_gate.shape[1]
    assert B == 1 and Sk == S and S % _TQ == 0 and S % _CW == 0 and Dh == 128 and D % 512 == 128
    n = S // _TQ
    assert n == 8 and _P == n - 1 and (H - 2) * n % _L == 0 and _L == 12 and _NS == 4 and S == 2048 and F % _CW == 192
    hbm = pl.BlockSpec(memory_space=pltpu.HBM)
    out = pl.pallas_call(
        functools.partial(_kernel, S=S, D=D, Dh=Dh, H=H),
        grid=(1,),
        in_specs=[hbm] * 9,
        out_specs=pl.BlockSpec(memory_space=pl.ANY),
        out_shape=jax.ShapeDtypeStruct((S, D), _BF16),
        scratch_shapes=[
            pltpu.VMEM((S, D), _BF16),
            pltpu.VMEM((S // 2, D), jnp.uint32),
            pltpu.VMEM((S, D), _F32),
            pltpu.VMEM((S, D), _F32),
            pltpu.VMEM((S, D), _BF16),
            pltpu.VMEM((2, _TQ, S), _F32),
            pltpu.VMEM((_TQ, 128), _F32),
            pltpu.VMEM((_TQ, Dh), _F32),
            pltpu.VMEM((_TQ, 128), _F32),
            pltpu.VMEM((_NS, 2 * S + 2 * D, Dh), _BF16),
            pltpu.VMEM((F, D), _BF16),
            pltpu.VMEM((F, D), _BF16),
            pltpu.VMEM((F, D), _BF16),
            pltpu.VMEM((D,), _BF16),
            pltpu.SMEM((_TOPC,), _I32),
            pltpu.SMEM((1,), _I32),
            pltpu.SemaphoreType.DMA((_NS + 5 + 2 * n + 5,)),
        ],
        compiler_params=pltpu.CompilerParams(
            dimension_semantics=("arbitrary",),
            vmem_limit_bytes=100 * 1024 * 1024,
            disable_bounds_checks=True,
            disable_semaphore_checks=True,
            internal_scratch_in_bytes=64 * 1024,
        ),
    )(A_x.reshape(S, D), A_k_cache.reshape(H, Sk, Dh), A_v_cache.reshape(H, Sk, Dh), A_wq, A_wo,
      B_w_r, B_w_gate.T, B_w_up.T, B_w_down)
    return out.reshape(B, S, D)
```

```python
import functools
import math

import jax
import jax.numpy as jnp
import jax.experimental.pallas as pl
import jax.experimental.pallas.tpu as pltpu

_F32 = jnp.float32
_BF16 = jnp.bfloat16
_I32 = jnp.int32
_NT = (((1,), (1,)), ((), ()))

_TOPC = 8
_EPS = 1e-5
_TQ = 256
_CW = 512
_P = 7
_L = 12
_NS = 4


def _bf(x):
    return x.astype(_BF16).astype(_F32)


def _silu(x):
    h = 0.5 * x
    return h + h * jnp.tanh(h)


def _sigmoid(x):
    return 0.5 + 0.5 * jnp.tanh(0.5 * x)


def _after(gate, val):
    return jnp.where(gate > jnp.inf, 0.0, val)


def _after16(gate, val):
    g = gate > jnp.inf
    g = jnp.concatenate([g[r:r + 8] for r in range(8, gate.shape[0], 16) for _ in range(2)], axis=0)
    return jnp.where(g, 0.0, val)


def _kernel(x_hbm, k_hbm, v_hbm, wq_hbm, wo_hbm, wr_hbm, wg_hbm, wu_hbm, wd_hbm,
            out_hbm,
            x_ref, xnp_ref, z_ref, acc_ref, ob_ref, s_ref, mc_ref, oc_ref, lc_ref,
            hb, wg_ref, wu_ref, wd_ref, wr_ref, sel_ref, zs,
            sems,
            *, S, D, Dh, H):
    tq, cw, p, L, NS = _TQ, _CW, _P, _L, _NS
    n = S // tq
    R = S // cw
    tb = tq // 4
    D4 = (D // 512) * 512
    F = wd_ref.shape[0]
    scale = (Dh ** -0.5) * math.log2(math.e)

    K0, V0, Q0, O0 = 0, S, 2 * S, 2 * S + D

    def hcol(h):
        return pl.ds(pl.multiple_of(h * Dh, Dh), Dh)

    def cp_k(h, slot, sem, r0=0, r1=S):
        return (pltpu.make_async_copy(k_hbm.at[h, r0:r1], hb.at[slot, K0 + r0:K0 + r1], sems.at[sem]),)

    def cp_v(h, slot, sem):
        return (pltpu.make_async_copy(v_hbm.at[h], hb.at[slot, V0:V0 + S], sems.at[sem]),)

    def cp_wq(h, slot, sem):
        return (pltpu.make_async_copy(wq_hbm.at[:, hcol(h)], hb.at[slot, Q0:Q0 + D], sems.at[sem]),)

    def cp_wo(h, slot, sem):
        return tuple(pltpu.make_async_copy(wo_hbm.at[hcol(h), c:c + 128], hb.at[slot, O0 + c:O0 + c + 128],
                                           sems.at[sem]) for c in range(0, D, 128))

    def start_head(h, slot):
        for cp in (cp_wq, cp_k, cp_v, cp_wo):
            for c in cp(h, slot, slot):
                c.start()

    def wait_head(slot):
        pltpu.make_async_copy(hb.at[slot], hb.at[slot], sems.at[slot]).wait()

    def cp_x(i):
        return pltpu.make_async_copy(x_hbm.at[rs(i * tq, tq), :], x_ref.at[rs(i * tq, tq), :],
                                     sems.at[NS + 5 + i])

    def cp_out(i, z):
        r0, nr = (i * tq, tq) if i < n - 1 else ((n - 1) * tq + (i - n + 1) * tq // 2, tq // 2)
        src = pl.ds(pl.multiple_of(z * tq + r0, tb), nr)
        return pltpu.make_async_copy(ob_ref.at[src, :], out_hbm.at[pl.ds(r0, nr), :], sems.at[NS + 5 + n + i])

    def cp_ffn():
        return (pltpu.make_async_copy(wg_hbm, wg_ref, sems.at[NS + 5 + 2 * n + 4]),
                pltpu.make_async_copy(wu_hbm, wu_ref, sems.at[NS + 5 + 2 * n + 1]),
                pltpu.make_async_copy(wd_hbm, wd_ref, sems.at[NS + 5 + 2 * n + 2]))

    def cp_wr():
        return pltpu.make_async_copy(wr_hbm, wr_ref, sems.at[NS + 5 + 2 * n + 3])

    def lanes(v, k):
        return jnp.concatenate([v] * k, axis=1)

    def rows(v, k):
        return jnp.concatenate([v] * k, axis=0)

    def rs(r0, nr):
        return slice(r0, r0 + nr) if isinstance(r0, int) else pl.ds(pl.multiple_of(r0, tb), nr)

    def rs2(r0, nr):
        return slice(r0 // 2, (r0 + nr) // 2) if isinstance(r0, int) else pl.ds(pl.multiple_of(r0 // 2, tb // 2), nr // 2)

    def fold(v):
        t = v[:, 0:128]
        for j in range(1, v.shape[1] // 128):
            t = t + v[:, j * 128:(j + 1) * 128]
        return t

    def compact(col, g0, init):
        lane = jax.lax.broadcasted_iota(_I32, init.shape, 1) - g0
        for g in range(col.shape[0] // 8):
            init = jnp.where(lane == g, col[8 * g:8 * g + 8, :], init)
        return init

    def side(jobs, res):
        for k, f in enumerate(jobs or []):
            r0 = min(k * res.shape[0] // len(jobs) // 8 * 8, res.shape[0] - tb)
            f(res[r0:r0 + tb, 0:128])

    def stored(ref, r0, z):
        k = 32 // (8 * ref.dtype.itemsize)
        v = ref[pl.ds(pl.multiple_of(z * 8 * k + r0, 8 * k), 8 * k), 0:128]
        return v if k == 1 else pltpu.bitcast(v, _F32)

    def qproj(i, slot, jobs=None):
        w = hb.at[slot, Q0:Q0 + D]
        xv = xnp_ref.at[rs2(i * tq, tq)]
        q = jnp.dot(pltpu.bitcast(xv[:, 0:D4], _BF16), w[0:D4, :], preferred_element_type=_F32)
        q = q + jnp.concatenate(
            [jnp.dot(pltpu.bitcast(xv[t * tb // 2:(t + 1) * tb // 2, D4:D], _BF16), w[D4:D, :],
                     preferred_element_type=_F32)
             for t in range(4)], axis=0)
        side(jobs, q)
        return (q * scale).astype(_BF16)

    def rowmax(mx):
        return jnp.broadcast_to(jnp.max(mx, axis=-1, keepdims=True), (tq, 128))

    def qk(par, slot, q, z, jobs=None, lanewise=False, groups=range(R), mx=None):
        if jobs is None and not lanewise:
            s = jax.lax.dot_general(q, hb[slot, K0:K0 + S], _NT, preferred_element_type=_F32)
            s_ref[z + par % 2] = s
            return rowmax(s)
        for c in groups:
            s = jax.lax.dot_general(q, hb[slot, K0 + c * cw:K0 + (c + 1) * cw], _NT, preferred_element_type=_F32)
            s_ref[z + par % 2, :, c * cw:(c + 1) * cw] = s
            for j in range(cw // 128):
                sj = s[:, j * 128:(j + 1) * 128]
                mx = sj if mx is None else jnp.maximum(mx, sj)
            side(jobs and jobs[c], s)
        return mx if lanewise else rowmax(mx)

    def finalize(r0, nr, c0, c1, s):
        out = x_ref[r0:r0 + nr, c0:c1].astype(_F32) + s * z_ref[r0:r0 + nr, c0:c1]
        ob_ref[r0:r0 + nr, c0:c1] = out.astype(_BF16)
        return out

    def wo(i, slot, o, lp, mode, jobs=None, off=0):
        nq = o.shape[0]
        l = jnp.sum(lp, axis=-1, keepdims=True)
        o32 = o * pl.reciprocal(l, full_range=False)
        o = o32.astype(_BF16)
        w = [hb[slot, O0 + c:O0 + c + 128] for c in range(0, D, 128)]
        av = acc_ref.at[rs(i * tq, tq)]

        def emit(r0, nr, c0, c1, a):
            if mode == "init":
                av[r0:r0 + nr, c0:c1] = a
            elif mode == "acc":
                av[r0:r0 + nr, c0:c1] += a
            else:
                finalize(i * tq + r0, nr, c0, c1, av[r0:r0 + nr, c0:c1] + a)

        a = jnp.dot(o, jnp.concatenate(w[:-1], axis=1), preferred_element_type=_F32)
        emit(off, nq, 0, D4, a)
        side(jobs, a)
        for t in range(0, nq, nq // 4):
            emit(off + t, nq // 4, D4, D,
                 jnp.dot(o32[t:t + nq // 4, :].astype(_BF16), w[-1], preferred_element_type=_F32))
        return a[:, 0:128]

    def pv(par, slot, m, gate, z, jobs=None, before=None, last=False, off=0, lag=1):
        o = lp = None
        gates = [gate] * lag
        for c in range(R):
            mc = m if gates[c] is None else _after16(gates[c], m)
            if before is not None and before[c] is not None:
                mc = _after(rows(before[c](), m.shape[0] // 8), mc)
            sc = s_ref[z + par % 2, off:off + m.shape[0], c * cw:(c + 1) * cw]
            pe = jnp.exp2(sc - lanes(mc, cw // 128))
            ps = [pe[:, j * 128:(j + 1) * 128] for j in range(cw // 128)]
            for pj in ps:
                lp = pj if lp is None else lp + pj
            ps[-1] = jnp.minimum(ps[-1], lp)
            pb = jnp.concatenate(ps, axis=1).astype(_BF16)
            oc = jnp.dot(pb, hb[slot, V0 + c * cw:V0 + (c + 1) * cw], preferred_element_type=_F32)
            side(None if jobs is None else jobs[c], oc)
            o = oc if o is None else o + oc
            gates.append(o)
        return o, (lp if last else _after16(o, lp))

    def layernorm(r0, nr, z, rel=None):
        def x(k):
            return x_ref[pl.ds(pl.multiple_of(k * z * tb + r0, tb), nr), :].astype(_F32)
        xs = fold(x(0))
        if rel is not None:
            xs = _after(rel, xs)
        mean = jnp.sum(xs, axis=-1, keepdims=True) * (1.0 / D)
        xc = x(1) - mean
        var = compact(jnp.sum(xc * xc, axis=-1, keepdims=True), 0, jnp.ones((8, 128), _F32)) * (1.0 / D)
        inv = 1.0 / _bf(jnp.sqrt(_bf(_bf(var) + _bf(jnp.float32(_EPS)))))
        lane = jax.lax.broadcasted_iota(_I32, (8, 128), 1)
        inv = jnp.concatenate([jnp.where(lane == g, inv, 0.0) for g in range(nr // 8)], axis=0)
        inv = jnp.sum(inv, axis=-1, keepdims=True)
        xn = (_bf(x(2) - _bf(mean)) * inv).astype(_BF16)
        xnp_ref[rs2(r0, nr), :] = pltpu.bitcast(xn, jnp.uint32)

    def router(r0, nr, rt, rel):
        xn = pltpu.bitcast(xnp_ref[rs2(r0, nr), :], _BF16)
        rp = _after(rel, fold(xn.astype(_F32) * wr_ref[...].astype(_F32).reshape(1, D)))
        rt[0] = compact(jnp.sum(rp, axis=-1, keepdims=True), r0 // 8, rt[0])

    def topk(rt):
        rt = _bf(rt)
        lane = jax.lax.broadcasted_iota(_I32, rt.shape, 1)
        sub = jax.lax.broadcasted_iota(_I32, rt.shape, 0)
        top = pltpu.bitcast(jnp.where(rt == 0.0, 0.0, rt), _I32) >> 16
        code = jnp.where(rt != rt, 0, jnp.where(top < 0, -1 - top, top + 32768))
        key = pltpu.bitcast((1 << 29) + code * S + (S - 1 - (lane * 8 + sub)), _F32)
        for c in range(_TOPC):
            kmax = jnp.max(jnp.max(key, axis=0, keepdims=True), axis=1, keepdims=True)
            sel_ref[c] = S - 1 - (pltpu.bitcast(kmax, _I32)[0, 0] & (S - 1))
            key = jnp.where(key == kmax, 0.0, key)

    def pace(v, k, done, rel):
        t = fold(v)
        t = jnp.concatenate([t[j:j + 8] + t[j + 8:j + 16] for j in range(0, v.shape[0], 16)], axis=0)
        if rel is not None:
            t = _after(jnp.concatenate([rel[j:j + 8] for j in range(0, v.shape[0], 16)], axis=0), t)
        done[0] = compact(jnp.sum(t, axis=-1, keepdims=True), k, done[0])

    def gate_piece(r0, nr, done, rel):
        g = _silu(pltpu.bitcast(xnp_ref[rs2(r0, nr), :], _BF16).astype(_F32))
        z_ref[r0:r0 + nr, :] = g
        pace(g, r0 // 16, done, rel)

    def fin_piece(r0, nr, done, z, rel):
        s = _after(lanes(rel, D // 128), acc_ref[r0:r0 + nr, :])
        pace(finalize(r0, nr, 0, D, s), r0 // 16, done, None)
        if (r0 + nr) % tq == 0:
            cp_out(r0 // tq, z).start()

    def ffn_jobs():
        st = {}
        F4 = (F // cw) * cw

        def gather():
            rowid = jax.lax.broadcasted_iota(_I32, (_TOPC, 1), 0)
            xs = jnp.zeros((_TOPC, D), _F32)
            for c in range(_TOPC):
                w = xnp_ref[pl.ds(sel_ref[c] // 2, 1), :]
                w = jnp.where(sel_ref[c] % 2 == 0, w << 16, w & jnp.uint32(0xFFFF0000))
                xs = jnp.where(rowid == c, pltpu.bitcast(w, _F32), xs)
            st["xs"], st["xb"] = xs, xs.astype(_BF16)

        def add(key, val):
            st[key] = val if key not in st else st[key] + val

        def up(parts, k, rel):
            xk = st["xb"][:, k * 128:(k + 1) * 128]
            for name, w_ref, c0, c1 in parts:
                add((name, c0), jax.lax.dot_general(xk, w_ref[c0:c1, k * 128:(k + 1) * 128], _NT,
                                                    preferred_element_type=_F32))

        def hidden():
            cuts = list(range(0, F, cw))
            g = _bf(jnp.concatenate([st["g", c] for c in cuts], axis=1))
            u = _bf(jnp.concatenate([st["u", c] for c in cuts], axis=1))
            st["h"] = (_bf(_silu(g)) * u).astype(_BF16)

        def down(cuts, c0, c1, rel):
            if "h" not in st:
                hidden()
            for k0, k1 in zip(cuts[:-1], cuts[1:]):
                add(("y", c0), jnp.dot(st["h"][:, k0:k1], wd_ref[k0:k1, c0:c1], preferred_element_type=_F32))

        def scatter(done):
            xs = _after(lanes(done, D // 128), st["xs"])
            rs = _bf(jnp.sum(fold(xs * wr_ref[...].astype(_F32).reshape(1, D)), axis=-1, keepdims=True))
            y = _bf(jnp.concatenate([st["y", 0], st["y", D4]], axis=1))
            zz = _silu(_bf(xs + _bf(y * _bf(_sigmoid(rs)))))
            for c in range(_TOPC):
                z_ref[pl.ds(sel_ref[c], 1), :] = zz[c:c + 1, :]

        stage1 = []
        for k in range(D // 128):
            for name, w_ref in (("g", wg_ref), ("u", wu_ref)):
                for c0 in range(0, F4, cw):
                    stage1.append(functools.partial(up, [(name, w_ref, c0, c0 + cw)], k))
            stage1.append(functools.partial(up, [("g", wg_ref, F4, F), ("u", wu_ref, F4, F)], k))
        stage2 = [functools.partial(down, [k0, min(k0 + 128, F)], 0, D4) for k0 in range(0, F, 128)]
        stage2 += [functools.partial(down, [k0, k0 + cw], D4, D) for k0 in range(0, F4, cw)]
        stage2 += [functools.partial(down, [F4, F4 + 64, F4 + 128, F4 + 160, F], D4, D)]
        return gather, stage1, stage2, scatter

    def save(state):
        mc_ref[...], oc_ref[...], lc_ref[...] = state

    def load():
        return rowmax(mc_ref[...]), oc_ref[...], lc_ref[...]

    def chunk(u):
        return u % n if isinstance(u, int) else u & (n - 1)

    def slot(u):
        return u // n % NS if isinstance(u, int) else (u >> 3) & (NS - 1)

    def round_(u, par, state, z, mode, jobs=None, before=None, last=False, mid=None, nxt=None):
        m, o, lp = state
        c1, s1 = nxt or (chunk(u + 1), slot(u + 1))
        q = qproj(c1, s1, jobs and jobs[0])
        m_next = qk(par + 1, s1, q, z, jobs and jobs[1:R + 1], lanewise=last)
        if mid is not None:
            mid()
        gate = wo(chunk(u - 1), slot(u - 1), o, lp, mode, jobs and jobs[R + 1])
        if mode == "final":
            cp_out(chunk(u - 1), z).start()
        return (m_next,) + pv(par, slot(u), m, gate, z, jobs and jobs[R + 2:], before, last)

    zs[0] = jnp.minimum(pl.program_id(0), 0)
    wq0, v0, wo0 = (cp(0, 0, NS + t) for t, cp in enumerate((cp_wq, cp_v, cp_wo)))
    k0 = cp_k(0, 0, NS + 3, 0, S // 2) + cp_k(0, 0, NS + 4, S // 2, S)
    for c in (cp_x(0), *wq0, cp_x(1), cp_wr(), *k0, cp_x(2), *v0, *wo0, *(cp_x(i) for i in range(3, n))):
        c.start()
    start_head(1, 1)
    start_head(2, 2)
    for c in cp_ffn():
        c.start()
    @pl.loop(0, (S - (p - 1) * tq) // 32)
    def _(i):
        acc_ref[pl.ds(pl.multiple_of((p - 1) * tq + i * 32, 32), 32), :] = jnp.zeros((32, D), _F32)

    cp_x(0).wait()
    z = zs[0]
    rt = [jnp.zeros((8, S // 8), _F32)]

    def ln_jobs(i, z, spread):
        pieces = [functools.partial(layernorm, i * tq + t * tb, tb, z) for t in range(4)]
        return [[pieces.pop(0) for _ in range(k)] for k in spread]

    def score_jobs(i, spread):
        pieces = [functools.partial(router, i * tq + t * tb, tb, rt) for t in range(4)]
        return [[pieces.pop(0) for _ in range(k)] for k in spread]

    for f in ln_jobs(0, z, [4])[0]:
        f()
    wq0[0].wait()
    cp_x(1).wait()
    q0 = qproj(0, 0)
    for f in ln_jobs(1, z, [4])[0]:
        f()
    q1 = qproj(1, 0)
    cp_wr().wait()
    k0[0].wait()
    scores01 = [[functools.partial(router, (2 * c + t) * tb, tb, rt) for t in range(2)] for c in range(R)]
    m0 = qk(0, 0, q0, z, scores01[:2], True, range(2))
    m1 = qk(1, 0, q1, z, scores01[2:], True, range(2))
    k0[1].wait()
    cp_x(2).wait()
    ln2 = ln_jobs(2, z, [0, 0, 3, 1])
    m0 = rowmax(qk(0, 0, q0, z, ln2, True, range(2, 4), m0))
    m1 = qk(1, 0, q1, z, None, True, range(2, 4), m1)
    v0[0].wait()
    save((m1,) + pv(0, 0, m0, None, z, score_jobs(2, [2, 2, 0, 0]), last=True))
    pltpu.make_async_copy(hb.at[0, O0:O0 + D], hb.at[0, O0:O0 + D], sems.at[NS + 2]).wait()

    def pair(j, carry):
        rt[0], u, i0, i1 = carry
        cp_x(i0).wait()
        pl.when(i1 > i0)(lambda: cp_x(i1).wait())
        z = zs[0]
        state = load()
        for k, i in enumerate((i0, i1)):
            jobs = ln_jobs(i, z, [1, 1, 1, 1, 0, 0]) + score_jobs(i, [1, 1, 1, 1])
            state = round_(u + k, 1 + k, state, z, "init", jobs, last=(k == 1), nxt=(u + k + 1, 0))
        save(state)
        return rt[0], u + 2, i0 + 2, jnp.minimum(i1 + 2, n - 1)

    scores = jax.lax.fori_loop(0, (p - 1) // 2, pair, (rt[0], jnp.int32(1), jnp.int32(3), jnp.int32(4)))[0]

    def entry(u0):
        h0 = (u0 >> 3) + 1
        return (u0, h0 & (NS - 1), (h0 + 1) & (NS - 1), ((u0 + L) >> 3) - h0, chunk(u0 + 1), slot(u0 + 1))

    def body(j, carry):
        u0, w1, w2, two, c1, s1 = carry
        wait_head(w1)
        pl.when(two > 0)(lambda: wait_head(w2))
        z = zs[0]

        def prefetch():
            h1 = ((u0 + L) >> 3) + 1
            start_head(h1, h1 & (NS - 1))
            pl.when(h1 + 1 <= jnp.minimum((u0 + 2 * L) >> 3, H - 1))(
                lambda: start_head(h1 + 1, (h1 + 1) & (NS - 1)))

        state = load()
        for k in range(L):
            state = round_(u0 + k, p + k, state, z, "acc", last=(k == L - 1), mid=prefetch if k == 1 else None,
                           nxt=(c1, s1) if k == 0 else None)
        save(state)
        return entry(u0 + L)

    T = H * n
    jax.lax.fori_loop(0, (T - 2 * n) // L, body, entry(jnp.int32(p)))

    wait_head((H - 1) % NS)
    for c in cp_ffn():
        c.wait()
    z = zs[0]
    state = load()
    gather, stage1, stage2, scatter = ffn_jobs()
    topk(scores)
    gather()
    done, done2 = [jnp.zeros((8, 128), _F32)], [jnp.zeros((8, 128), _F32)]
    late = 3
    gates = [functools.partial(gate_piece, r0, tb, done) for r0 in range(0, S, tb)]
    fins = [functools.partial(fin_piece, r0, tb, done2, z) for r0 in range(0, late * tq, tb)]
    fq = stage1 + [lambda rel: None] + stage2
    u_first = T - 2 * n + p
    for u in range(u_first, T - 1):
        i = u - 1 - (T - n)
        vpu, nv, nf = gates, [1, 1, 0, 0, 0, 0, 1, 1, 1, 1], [1] * 6 + [1 if i < late - 2 else 2] * 4
        if u == u_first:
            nv, nf = [0, 0, 0, 0, 0, 2, 2, 2, 2, 0], [0] * 6 + [1] * 4
        if i > late:
            vpu, nv = fins, [2, 2, 1, 1]
        jobs = [[vpu.pop(0) for _ in range(min(len(vpu), a))] + [fq.pop(0) for _ in range(min(len(fq), b))]
                for a, b in zip(nv + [0] * 10, nf)]
        before = [None] * R
        if i >= late:
            assert not fq and not gates
            before[2] = functools.partial(stored, ob_ref, i * tq, z)
        state = round_(u, u, state, z, "final" if i >= late else "acc", jobs, before,
                       mid=(lambda: scatter(done[0])) if i == late else None)
    assert not fins
    m, o, lp = state
    sl, hq = slot(T - 1), tq // 2
    oa, lpa = pv(T - 1, sl, m[:hq], o[:hq], z, before=[lambda: done2[0], None, None, None], lag=2)
    gate = wo(n - 2, sl, o, lp, "final")
    cp_out(n - 2, z).start()
    ob, lpb = pv(T - 1, sl, m[hq:], gate[:hq], z, off=hq, lag=2,
                 before=[None, None, None, functools.partial(stored, ob_ref, (n - 2) * tq, z)])
    wo(n - 1, sl, oa, lpa, "final")
    cp_out(n - 1, z).start()
    wo(n - 1, sl, ob, lpb, "final", off=hq)
    cp_out(n, z).start()
    for i in range(n + 1):
        cp_out(i, z).wait()


@jax.jit
def pallas_recurrent_scan__mha_block_cached__moe_arch_mod__prompt_kernel(
    A_x: jax.Array,
    A_k_cache: jax.Array,
    A_v_cache: jax.Array,
    A_wq: jax.Array,
    A_wo: jax.Array,
    B_x: jax.Array,
    B_w_r: jax.Array,
    B_w_gate: jax.Array,
    B_w_up: jax.Array,
    B_w_down: jax.Array,
):
    B, S, D = A_x.shape
    _, H, Sk, Dh = A_k_cache.shape
    F = B_w_gate.shape[1]
    assert B == 1 and Sk == S and S % _TQ == 0 and S % _CW == 0 and Dh == 128 and D % 512 == 128
    n = S // _TQ
    assert n == 8 and _P == n - 1 and (H - 2) * n % _L == 0 and _L == 12 and _NS == 4 and S == 2048 and F % _CW == 192
    hbm = pl.BlockSpec(memory_space=pltpu.HBM)
    out = pl.pallas_call(
        functools.partial(_kernel, S=S, D=D, Dh=Dh, H=H),
        grid=(1,),
        in_specs=[hbm] * 9,
        out_specs=pl.BlockSpec(memory_space=pl.ANY),
        out_shape=jax.ShapeDtypeStruct((S, D), _BF16),
        scratch_shapes=[
            pltpu.VMEM((S, D), _BF16),
            pltpu.VMEM((S // 2, D), jnp.uint32),
            pltpu.VMEM((S, D), _F32),
            pltpu.VMEM((S, D), _F32),
            pltpu.VMEM((S, D), _BF16),
            pltpu.VMEM((2, _TQ, S), _F32),
            pltpu.VMEM((_TQ, 128), _F32),
            pltpu.VMEM((_TQ, Dh), _F32),
            pltpu.VMEM((_TQ, 128), _F32),
            pltpu.VMEM((_NS, 2 * S + 2 * D, Dh), _BF16),
            pltpu.VMEM((F, D), _BF16),
            pltpu.VMEM((F, D), _BF16),
            pltpu.VMEM((F, D), _BF16),
            pltpu.VMEM((D,), _BF16),
            pltpu.SMEM((_TOPC,), _I32),
            pltpu.SMEM((1,), _I32),
            pltpu.SemaphoreType.DMA((_NS + 5 + 2 * n + 5,)),
        ],
        compiler_params=pltpu.CompilerParams(
            dimension_semantics=("arbitrary",),
            vmem_limit_bytes=100 * 1024 * 1024,
            disable_bounds_checks=True,
            disable_semaphore_checks=True,
            internal_scratch_in_bytes=64 * 1024,
        ),
    )(A_x.reshape(S, D), A_k_cache.reshape(H, Sk, Dh), A_v_cache.reshape(H, Sk, Dh), A_wq, A_wo,
      B_w_r, B_w_gate.T, B_w_up.T, B_w_down)
    return out.reshape(B, S, D)
```

```python
import functools
import math

import jax
import jax.numpy as jnp
import jax.experimental.pallas as pl
import jax.experimental.pallas.tpu as pltpu

_F32 = jnp.float32
_BF16 = jnp.bfloat16
_I32 = jnp.int32
_NT = (((1,), (1,)), ((), ()))

_TOPC = 8
_EPS = 1e-5
_TQ = 256
_CW = 512
_P = 7
_L = 12
_NS = 4


def _bf(x):
    return x.astype(_BF16).astype(_F32)


def _silu(x):
    h = 0.5 * x
    return h + h * jnp.tanh(h)


def _sigmoid(x):
    return 0.5 + 0.5 * jnp.tanh(0.5 * x)


def _after(gate, val):
    return jnp.where(gate > jnp.inf, 0.0, val)


def _after16(gate, val):
    g = gate > jnp.inf
    g = jnp.concatenate([g[r:r + 8] for r in range(8, gate.shape[0], 16) for _ in range(2)], axis=0)
    return jnp.where(g, 0.0, val)


def _kernel(x_hbm, k_hbm, v_hbm, wq_hbm, wo_hbm, wr_hbm, wg_hbm, wu_hbm, wd_hbm,
            out_hbm,
            x_ref, xnp_ref, z_ref, acc_ref, ob_ref, s_ref, mc_ref, oc_ref, lc_ref,
            hb, wg_ref, wu_ref, wd_ref, wr_ref, sel_ref, zs,
            sems,
            *, S, D, Dh, H):
    tq, cw, p, L, NS = _TQ, _CW, _P, _L, _NS
    n = S // tq
    R = S // cw
    tb = tq // 4
    D4 = (D // 512) * 512
    F = wd_ref.shape[0]
    scale = (Dh ** -0.5) * math.log2(math.e)

    K0, V0, Q0, O0 = 0, S, 2 * S, 2 * S + D

    def hcol(h):
        return pl.ds(pl.multiple_of(h * Dh, Dh), Dh)

    def cp_k(h, slot, sem, r0=0, r1=S):
        return (pltpu.make_async_copy(k_hbm.at[h, r0:r1], hb.at[slot, K0 + r0:K0 + r1], sems.at[sem]),)

    def cp_v(h, slot, sem):
        return (pltpu.make_async_copy(v_hbm.at[h], hb.at[slot, V0:V0 + S], sems.at[sem]),)

    def cp_wq(h, slot, sem):
        return (pltpu.make_async_copy(wq_hbm.at[:, hcol(h)], hb.at[slot, Q0:Q0 + D], sems.at[sem]),)

    def cp_wo(h, slot, sem):
        return tuple(pltpu.make_async_copy(wo_hbm.at[hcol(h), c:c + 128], hb.at[slot, O0 + c:O0 + c + 128],
                                           sems.at[sem]) for c in range(0, D, 128))

    def start_head(h, slot):
        for cp in (cp_wq, cp_k, cp_v, cp_wo):
            for c in cp(h, slot, slot):
                c.start()

    def wait_head(slot):
        pltpu.make_async_copy(hb.at[slot], hb.at[slot], sems.at[slot]).wait()

    def cp_x(i):
        return pltpu.make_async_copy(x_hbm.at[rs(i * tq, tq), :], x_ref.at[rs(i * tq, tq), :],
                                     sems.at[NS + 5 + i])

    def cp_out(i, z):
        r0, nr = (i * tq, tq) if i < n - 1 else ((n - 1) * tq + (i - n + 1) * tq // 2, tq // 2)
        src = pl.ds(pl.multiple_of(z * tq + r0, tb), nr)
        return pltpu.make_async_copy(ob_ref.at[src, :], out_hbm.at[pl.ds(r0, nr), :], sems.at[NS + 5 + n + i])

    def cp_ffn():
        return (pltpu.make_async_copy(wg_hbm, wg_ref, sems.at[NS + 5 + 2 * n + 4]),
                pltpu.make_async_copy(wu_hbm, wu_ref, sems.at[NS + 5 + 2 * n + 1]),
                pltpu.make_async_copy(wd_hbm, wd_ref, sems.at[NS + 5 + 2 * n + 2]))

    def cp_wr():
        return pltpu.make_async_copy(wr_hbm, wr_ref, sems.at[NS + 5 + 2 * n + 3])

    def lanes(v, k):
        return jnp.concatenate([v] * k, axis=1)

    def rows(v, k):
        return jnp.concatenate([v] * k, axis=0)

    def rs(r0, nr):
        return slice(r0, r0 + nr) if isinstance(r0, int) else pl.ds(pl.multiple_of(r0, tb), nr)

    def rs2(r0, nr):
        return slice(r0 // 2, (r0 + nr) // 2) if isinstance(r0, int) else pl.ds(pl.multiple_of(r0 // 2, 16), nr // 2)

    def fold(v):
        t = v[:, 0:128]
        for j in range(1, v.shape[1] // 128):
            t = t + v[:, j * 128:(j + 1) * 128]
        return t

    def compact(col, g0, init):
        lane = jax.lax.broadcasted_iota(_I32, init.shape, 1) - g0
        for g in range(col.shape[0] // 8):
            init = jnp.where(lane == g, col[8 * g:8 * g + 8, :], init)
        return init

    def side(jobs, res):
        for k, f in enumerate(jobs or []):
            r0 = min(k * res.shape[0] // len(jobs) // 8 * 8, res.shape[0] - tb)
            f(res[r0:r0 + tb, 0:128])

    def stored(ref, r0, z):
        k = 32 // (8 * ref.dtype.itemsize)
        v = ref[pl.ds(pl.multiple_of(z * 8 * k + r0, 8 * k), 8 * k), 0:128]
        return v if k == 1 else pltpu.bitcast(v, _F32)

    def qproj(i, slot, jobs=None):
        w = hb.at[slot, Q0:Q0 + D]
        xv = xnp_ref.at[rs2(i * tq, tq)]
        q = jnp.dot(pltpu.bitcast(xv[:, 0:D4], _BF16), w[0:D4, :], preferred_element_type=_F32)
        q = q + jnp.concatenate(
            [jnp.dot(pltpu.bitcast(xv[t * tb // 2:(t + 1) * tb // 2, D4:D], _BF16), w[D4:D, :],
                     preferred_element_type=_F32)
             for t in range(4)], axis=0)
        side(jobs, q)
        return (q * scale).astype(_BF16)

    def rowmax(mx):
        return jnp.broadcast_to(jnp.max(mx, axis=-1, keepdims=True), (tq, 128))

    def qk(par, slot, q, z, jobs=None, lanewise=False, groups=range(R), mx=None):
        if jobs is None and not lanewise:
            s = jax.lax.dot_general(q, hb[slot, K0:K0 + S], _NT, preferred_element_type=_F32)
            s_ref[z + par % 2] = s
            return rowmax(s)
        for c in groups:
            s = jax.lax.dot_general(q, hb[slot, K0 + c * cw:K0 + (c + 1) * cw], _NT, preferred_element_type=_F32)
            s_ref[z + par % 2, :, c * cw:(c + 1) * cw] = s
            for j in range(cw // 128):
                sj = s[:, j * 128:(j + 1) * 128]
                mx = sj if mx is None else jnp.maximum(mx, sj)
            side(jobs and jobs[c], s)
        return mx if lanewise else rowmax(mx)

    def finalize(r0, nr, c0, c1, s):
        out = x_ref[r0:r0 + nr, c0:c1].astype(_F32) + s * z_ref[r0:r0 + nr, c0:c1]
        ob_ref[r0:r0 + nr, c0:c1] = out.astype(_BF16)
        return out

    def wo(i, slot, o, lp, mode, jobs=None, off=0):
        nq = o.shape[0]
        l = jnp.sum(lp, axis=-1, keepdims=True)
        o32 = o * pl.reciprocal(l, full_range=False)
        o = o32.astype(_BF16)
        w = [hb[slot, O0 + c:O0 + c + 128] for c in range(0, D, 128)]
        av = acc_ref.at[rs(i * tq, tq)]

        def emit(r0, nr, c0, c1, a):
            if mode == "init":
                av[r0:r0 + nr, c0:c1] = a
            elif mode == "acc":
                av[r0:r0 + nr, c0:c1] += a
            else:
                finalize(i * tq + r0, nr, c0, c1, av[r0:r0 + nr, c0:c1] + a)

        a = jnp.dot(o, jnp.concatenate(w[:-1], axis=1), preferred_element_type=_F32)
        emit(off, nq, 0, D4, a)
        side(jobs, a)
        for t in range(0, nq, nq // 4):
            emit(off + t, nq // 4, D4, D,
                 jnp.dot(o32[t:t + nq // 4, :].astype(_BF16), w[-1], preferred_element_type=_F32))
        return a[:, 0:128]

    def pv(par, slot, m, gate, z, jobs=None, before=None, last=False, off=0, lag=1):
        o = lp = None
        gates = [gate] * lag
        for c in range(R):
            mc = m if gates[c] is None else _after16(gates[c], m)
            if before is not None and before[c] is not None:
                mc = _after(rows(before[c](), m.shape[0] // 8), mc)
            sc = s_ref[z + par % 2, off:off + m.shape[0], c * cw:(c + 1) * cw]
            pe = jnp.exp2(sc - lanes(mc, cw // 128))
            ps = [pe[:, j * 128:(j + 1) * 128] for j in range(cw // 128)]
            for pj in ps:
                lp = pj if lp is None else lp + pj
            ps[-1] = jnp.minimum(ps[-1], lp)
            pb = jnp.concatenate(ps, axis=1).astype(_BF16)
            oc = jnp.dot(pb, hb[slot, V0 + c * cw:V0 + (c + 1) * cw], preferred_element_type=_F32)
            side(None if jobs is None else jobs[c], oc)
            o = oc if o is None else o + oc
            gates.append(o)
        return o, (lp if last else _after16(o, lp))

    def layernorm(r0, nr, z, rel=None):
        def x(k):
            return x_ref[pl.ds(pl.multiple_of(k * z * tb + r0, 32), nr), :].astype(_F32)
        xs = fold(x(0))
        if rel is not None:
            xs = _after(rel[:nr], xs)
        mean = jnp.sum(xs, axis=-1, keepdims=True) * (1.0 / D)
        xc = x(1) - mean
        var = compact(jnp.sum(xc * xc, axis=-1, keepdims=True), 0, jnp.ones((8, 128), _F32)) * (1.0 / D)
        inv = 1.0 / _bf(jnp.sqrt(_bf(_bf(var) + _bf(jnp.float32(_EPS)))))
        lane = jax.lax.broadcasted_iota(_I32, (8, 128), 1)
        inv = jnp.concatenate([jnp.where(lane == g, inv, 0.0) for g in range(nr // 8)], axis=0)
        inv = jnp.sum(inv, axis=-1, keepdims=True)
        xn = (_bf(x(2) - _bf(mean)) * inv).astype(_BF16)
        xnp_ref[rs2(r0, nr), :] = pltpu.bitcast(xn, jnp.uint32)

    def router(r0, nr, rt, rel):
        xn = pltpu.bitcast(xnp_ref[rs2(r0, nr), :], _BF16)
        rp = _after(rel, fold(xn.astype(_F32) * wr_ref[...].astype(_F32).reshape(1, D)))
        rt[0] = compact(jnp.sum(rp, axis=-1, keepdims=True), r0 // 8, rt[0])

    def topk(rt):
        rt = _bf(rt)
        lane = jax.lax.broadcasted_iota(_I32, rt.shape, 1)
        sub = jax.lax.broadcasted_iota(_I32, rt.shape, 0)
        top = pltpu.bitcast(jnp.where(rt == 0.0, 0.0, rt), _I32) >> 16
        code = jnp.where(rt != rt, 0, jnp.where(top < 0, -1 - top, top + 32768))
        key = pltpu.bitcast((1 << 29) + code * S + (S - 1 - (lane * 8 + sub)), _F32)
        for c in range(_TOPC):
            kmax = jnp.max(jnp.max(key, axis=0, keepdims=True), axis=1, keepdims=True)
            sel_ref[c] = S - 1 - (pltpu.bitcast(kmax, _I32)[0, 0] & (S - 1))
            key = jnp.where(key == kmax, 0.0, key)

    def pace(v, k, done, rel):
        t = fold(v)
        t = jnp.concatenate([t[j:j + 8] + t[j + 8:j + 16] for j in range(0, v.shape[0], 16)], axis=0)
        if rel is not None:
            t = _after(jnp.concatenate([rel[j:j + 8] for j in range(0, v.shape[0], 16)], axis=0), t)
        done[0] = compact(jnp.sum(t, axis=-1, keepdims=True), k, done[0])

    def gate_piece(r0, nr, done, rel):
        g = _silu(pltpu.bitcast(xnp_ref[rs2(r0, nr), :], _BF16).astype(_F32))
        z_ref[r0:r0 + nr, :] = g
        pace(g, r0 // 16, done, rel)

    def fin_piece(r0, nr, done, z, rel):
        s = _after(lanes(rel, D // 128), acc_ref[r0:r0 + nr, :])
        pace(finalize(r0, nr, 0, D, s), r0 // 16, done, None)
        if (r0 + nr) % tq == 0:
            cp_out(r0 // tq, z).start()

    def ffn_jobs():
        st = {}
        F4 = (F // cw) * cw

        def gather():
            rowid = jax.lax.broadcasted_iota(_I32, (_TOPC, 1), 0)
            xs = jnp.zeros((_TOPC, D), _F32)
            for c in range(_TOPC):
                w = xnp_ref[pl.ds(sel_ref[c] // 2, 1), :]
                w = jnp.where(sel_ref[c] % 2 == 0, w << 16, w & jnp.uint32(0xFFFF0000))
                xs = jnp.where(rowid == c, pltpu.bitcast(w, _F32), xs)
            st["xs"], st["xb"] = xs, xs.astype(_BF16)

        def add(key, val):
            st[key] = val if key not in st else st[key] + val

        def up(parts, k, rel):
            xk = st["xb"][:, k * 128:(k + 1) * 128]
            for name, w_ref, c0, c1 in parts:
                add((name, c0), jax.lax.dot_general(xk, w_ref[c0:c1, k * 128:(k + 1) * 128], _NT,
                                                    preferred_element_type=_F32))

        def hidden():
            cuts = list(range(0, F, cw))
            g = _bf(jnp.concatenate([st["g", c] for c in cuts], axis=1))
            u = _bf(jnp.concatenate([st["u", c] for c in cuts], axis=1))
            st["h"] = (_bf(_silu(g)) * u).astype(_BF16)

        def down(cuts, c0, c1, rel):
            if "h" not in st:
                hidden()
            for k0, k1 in zip(cuts[:-1], cuts[1:]):
                add(("y", c0), jnp.dot(st["h"][:, k0:k1], wd_ref[k0:k1, c0:c1], preferred_element_type=_F32))

        def scatter(done):
            xs = _after(lanes(done, D // 128), st["xs"])
            rs = _bf(jnp.sum(fold(xs * wr_ref[...].astype(_F32).reshape(1, D)), axis=-1, keepdims=True))
            y = _bf(jnp.concatenate([st["y", 0], st["y", D4]], axis=1))
            zz = _silu(_bf(xs + _bf(y * _bf(_sigmoid(rs)))))
            for c in range(_TOPC):
                z_ref[pl.ds(sel_ref[c], 1), :] = zz[c:c + 1, :]

        stage1 = []
        for k in range(D // 128):
            for name, w_ref in (("g", wg_ref), ("u", wu_ref)):
                for c0 in range(0, F4, cw):
                    stage1.append(functools.partial(up, [(name, w_ref, c0, c0 + cw)], k))
            stage1.append(functools.partial(up, [("g", wg_ref, F4, F), ("u", wu_ref, F4, F)], k))
        stage2 = [functools.partial(down, [k0, min(k0 + 128, F)], 0, D4) for k0 in range(0, F, 128)]
        stage2 += [functools.partial(down, [k0, k0 + cw], D4, D) for k0 in range(0, F4, cw)]
        stage2 += [functools.partial(down, [F4, F4 + 64, F4 + 128, F4 + 160, F], D4, D)]
        return gather, stage1, stage2, scatter

    def save(state):
        mc_ref[...], oc_ref[...], lc_ref[...] = state

    def load():
        return rowmax(mc_ref[...]), oc_ref[...], lc_ref[...]

    def chunk(u):
        return u % n if isinstance(u, int) else u & (n - 1)

    def slot(u):
        return u // n % NS if isinstance(u, int) else (u >> 3) & (NS - 1)

    def round_(u, par, state, z, mode, jobs=None, before=None, last=False, mid=None, nxt=None):
        m, o, lp = state
        c1, s1 = nxt or (chunk(u + 1), slot(u + 1))
        q = qproj(c1, s1, jobs and jobs[0])
        m_next = qk(par + 1, s1, q, z, jobs and jobs[1:R + 1], lanewise=last)
        if mid is not None:
            mid()
        gate = wo(chunk(u - 1), slot(u - 1), o, lp, mode, jobs and jobs[R + 1])
        if mode == "final":
            cp_out(chunk(u - 1), z).start()
        return (m_next,) + pv(par, slot(u), m, gate, z, jobs and jobs[R + 2:], before, last)

    zs[0] = jnp.minimum(pl.program_id(0), 0)
    wq0, v0, wo0 = (cp(0, 0, NS + t) for t, cp in enumerate((cp_wq, cp_v, cp_wo)))
    k0 = cp_k(0, 0, NS + 3, 0, S // 2) + cp_k(0, 0, NS + 4, S // 2, S)
    for c in (cp_x(0), *wq0, cp_x(1), cp_wr(), *k0, cp_x(2), *v0, *wo0, *(cp_x(i) for i in range(3, n))):
        c.start()
    start_head(1, 1)
    start_head(2, 2)
    for c in cp_ffn():
        c.start()
    @pl.loop(0, (S - (p - 1) * tq) // 32)
    def _(i):
        acc_ref[pl.ds(pl.multiple_of((p - 1) * tq + i * 32, 32), 32), :] = jnp.zeros((32, D), _F32)

    cp_x(0).wait()
    z = zs[0]
    rt = [jnp.zeros((8, S // 8), _F32)]

    def ln_jobs(i, z, spread):
        pn = tq // sum(spread)
        pieces = [functools.partial(layernorm, i * tq + t * pn, pn, z) for t in range(sum(spread))]
        return [[pieces.pop(0) for _ in range(k)] for k in spread]

    def score_jobs(i, spread):
        pieces = [functools.partial(router, i * tq + t * tb, tb, rt) for t in range(4)]
        return [[pieces.pop(0) for _ in range(k)] for k in spread]

    for f in ln_jobs(0, z, [8])[0]:
        f()
    wq0[0].wait()
    cp_x(1).wait()
    q0 = qproj(0, 0)
    for f in ln_jobs(1, z, [8])[0]:
        f()
    q1 = qproj(1, 0)
    cp_wr().wait()
    k0[0].wait()
    scores01 = [[functools.partial(router, (2 * c + t) * tb, tb, rt) for t in range(2)] for c in range(R)]
    m0 = qk(0, 0, q0, z, scores01[:2], True, range(2))
    m1 = qk(1, 0, q1, z, scores01[2:], True, range(2))
    k0[1].wait()
    cp_x(2).wait()
    ln2 = ln_jobs(2, z, [0, 0, 3, 1])
    m0 = rowmax(qk(0, 0, q0, z, ln2, True, range(2, 4), m0))
    m1 = qk(1, 0, q1, z, None, True, range(2, 4), m1)
    v0[0].wait()
    save((m1,) + pv(0, 0, m0, None, z, score_jobs(2, [2, 2, 0, 0]), last=True))
    pltpu.make_async_copy(hb.at[0, O0:O0 + D], hb.at[0, O0:O0 + D], sems.at[NS + 2]).wait()

    def pair(j, carry):
        rt[0], u, i0, i1 = carry
        cp_x(i0).wait()
        pl.when(i1 > i0)(lambda: cp_x(i1).wait())
        z = zs[0]
        state = load()
        for k, i in enumerate((i0, i1)):
            jobs = ln_jobs(i, z, [2, 2, 2, 1, 1, 0]) + score_jobs(i, [1, 1, 1, 1])
            state = round_(u + k, 1 + k, state, z, "init", jobs, last=(k == 1), nxt=(u + k + 1, 0))
        save(state)
        return rt[0], u + 2, i0 + 2, jnp.minimum(i1 + 2, n - 1)

    scores = jax.lax.fori_loop(0, (p - 1) // 2, pair, (rt[0], jnp.int32(1), jnp.int32(3), jnp.int32(4)))[0]

    def entry(u0):
        h0 = (u0 >> 3) + 1
        return (u0, h0 & (NS - 1), (h0 + 1) & (NS - 1), ((u0 + L) >> 3) - h0, chunk(u0 + 1), slot(u0 + 1))

    def body(j, carry):
        u0, w1, w2, two, c1, s1 = carry
        wait_head(w1)
        pl.when(two > 0)(lambda: wait_head(w2))
        z = zs[0]

        def prefetch():
            h1 = ((u0 + L) >> 3) + 1
            start_head(h1, h1 & (NS - 1))
            pl.when(h1 + 1 <= jnp.minimum((u0 + 2 * L) >> 3, H - 1))(
                lambda: start_head(h1 + 1, (h1 + 1) & (NS - 1)))

        state = load()
        for k in range(L):
            state = round_(u0 + k, p + k, state, z, "acc", last=(k == L - 1), mid=prefetch if k == 1 else None,
                           nxt=(c1, s1) if k == 0 else None)
        save(state)
        return entry(u0 + L)

    T = H * n
    jax.lax.fori_loop(0, (T - 2 * n) // L, body, entry(jnp.int32(p)))

    wait_head((H - 1) % NS)
    for c in cp_ffn():
        c.wait()
    z = zs[0]
    state = load()
    gather, stage1, stage2, scatter = ffn_jobs()
    topk(scores)
    gather()
    done, done2 = [jnp.zeros((8, 128), _F32)], [jnp.zeros((8, 128), _F32)]
    late = 3
    gates = [functools.partial(gate_piece, r0, tb, done) for r0 in range(0, S, tb)]
    fins = [functools.partial(fin_piece, r0, tb, done2, z) for r0 in range(0, late * tq, tb)]
    fq = stage1 + [lambda rel: None] + stage2
    u_first = T - 2 * n + p
    for u in range(u_first, T - 1):
        i = u - 1 - (T - n)
        vpu, nv, nf = gates, [1, 1, 0, 0, 0, 0, 1, 1, 1, 1], [1] * 6 + [1 if i < late - 2 else 2] * 4
        if u == u_first:
            nv, nf = [0, 0, 0, 0, 0, 2, 2, 2, 2, 0], [0] * 6 + [1] * 4
        if i > late:
            vpu, nv = fins, [2, 2, 1, 1]
        jobs = [[vpu.pop(0) for _ in range(min(len(vpu), a))] + [fq.pop(0) for _ in range(min(len(fq), b))]
                for a, b in zip(nv + [0] * 10, nf)]
        before = [None] * R
        if i >= late:
            assert not fq and not gates
            before[2] = functools.partial(stored, ob_ref, i * tq, z)
        state = round_(u, u, state, z, "final" if i >= late else "acc", jobs, before,
                       mid=(lambda: scatter(done[0])) if i == late else None)
    assert not fins
    m, o, lp = state
    sl, hq = slot(T - 1), tq // 2
    oa, lpa = pv(T - 1, sl, m[:hq], o[:hq], z, before=[lambda: done2[0], None, None, None], lag=2)
    gate = wo(n - 2, sl, o, lp, "final")
    cp_out(n - 2, z).start()
    ob, lpb = pv(T - 1, sl, m[hq:], gate[:hq], z, off=hq, lag=2,
                 before=[None, None, None, functools.partial(stored, ob_ref, (n - 2) * tq, z)])
    wo(n - 1, sl, oa, lpa, "final")
    cp_out(n - 1, z).start()
    wo(n - 1, sl, ob, lpb, "final", off=hq)
    cp_out(n, z).start()
    for i in range(n + 1):
        cp_out(i, z).wait()


@jax.jit
def pallas_recurrent_scan__mha_block_cached__moe_arch_mod__prompt_kernel(
    A_x: jax.Array,
    A_k_cache: jax.Array,
    A_v_cache: jax.Array,
    A_wq: jax.Array,
    A_wo: jax.Array,
    B_x: jax.Array,
    B_w_r: jax.Array,
    B_w_gate: jax.Array,
    B_w_up: jax.Array,
    B_w_down: jax.Array,
):
    B, S, D = A_x.shape
    _, H, Sk, Dh = A_k_cache.shape
    F = B_w_gate.shape[1]
    assert B == 1 and Sk == S and S % _TQ == 0 and S % _CW == 0 and Dh == 128 and D % 512 == 128
    n = S // _TQ
    assert n == 8 and _P == n - 1 and (H - 2) * n % _L == 0 and _L == 12 and _NS == 4 and S == 2048 and F % _CW == 192
    hbm = pl.BlockSpec(memory_space=pltpu.HBM)
    out = pl.pallas_call(
        functools.partial(_kernel, S=S, D=D, Dh=Dh, H=H),
        grid=(1,),
        in_specs=[hbm] * 9,
        out_specs=pl.BlockSpec(memory_space=pl.ANY),
        out_shape=jax.ShapeDtypeStruct((S, D), _BF16),
        scratch_shapes=[
            pltpu.VMEM((S, D), _BF16),
            pltpu.VMEM((S // 2, D), jnp.uint32),
            pltpu.VMEM((S, D), _F32),
            pltpu.VMEM((S, D), _F32),
            pltpu.VMEM((S, D), _BF16),
            pltpu.VMEM((2, _TQ, S), _F32),
            pltpu.VMEM((_TQ, 128), _F32),
            pltpu.VMEM((_TQ, Dh), _F32),
            pltpu.VMEM((_TQ, 128), _F32),
            pltpu.VMEM((_NS, 2 * S + 2 * D, Dh), _BF16),
            pltpu.VMEM((F, D), _BF16),
            pltpu.VMEM((F, D), _BF16),
            pltpu.VMEM((F, D), _BF16),
            pltpu.VMEM((D,), _BF16),
            pltpu.SMEM((_TOPC,), _I32),
            pltpu.SMEM((1,), _I32),
            pltpu.SemaphoreType.DMA((_NS + 5 + 2 * n + 5,)),
        ],
        compiler_params=pltpu.CompilerParams(
            dimension_semantics=("arbitrary",),
            vmem_limit_bytes=100 * 1024 * 1024,
            disable_bounds_checks=True,
            disable_semaphore_checks=True,
            internal_scratch_in_bytes=64 * 1024,
        ),
    )(A_x.reshape(S, D), A_k_cache.reshape(H, Sk, Dh), A_v_cache.reshape(H, Sk, Dh), A_wq, A_wo,
      B_w_r, B_w_gate.T, B_w_up.T, B_w_down)
    return out.reshape(B, S, D)
```
